```python
import jax
import jax.numpy as jnp

def _softmax(x, axis=-1):
    return jax.nn.softmax(x, axis=axis)
def _gelu(x):
    return jax.nn.gelu(x, approximate=True)
def _silu(x):
    return jax.nn.silu(x)
def _sigmoid(x):
    return jax.nn.sigmoid(x)
def _layernorm(x, axis=-1, eps=1e-5):
    m = jnp.mean(x, axis=axis, keepdims=True)
    v = jnp.var(x, axis=axis, keepdims=True)
    return (x - m) / jnp.sqrt(v + eps)
def _scatter_add(tgt, idx, src, axis=0):
    return tgt.at[idx].add(src)
def _segment_sum(src, seg, n):
    return jax.ops.segment_sum(src, seg, n)
class _Rng:
    def __init__(self, key):
        self._k = key
    def _next(self):
        self._k, sub = jax.random.split(self._k)
        return sub
    def normal(self, shape):
        return jax.random.normal(self._next(), shape, dtype=jnp.bfloat16)
    def randint(self, lo, hi, shape):
        return jax.random.randint(self._next(), shape, lo, hi, dtype=jnp.int32)
    def uniform(self, shape, lo=0.0, hi=1.0):
        return jax.random.uniform(self._next(), shape, jnp.bfloat16, lo, hi)
    def permutation(self, n):
        return jax.random.permutation(self._next(), n)


kernel_name = 'interleave_layers__sliding_block_cached__moe_arch_mod__decode'

def setup_inputs():
    _rng = _Rng(jax.random.key(int.from_bytes(__import__("os").urandom(4), "little")))
    _w = (lambda a: (lambda t: t.astype(jnp.bfloat16) if jnp.issubdtype(t.dtype, jnp.floating) else t)(jnp.asarray(a)))
    def _A_setup():
        B, Sq, D = 4, 1, 640
        Hq, Hkv, Sk, Dh = 32, 32, 4096, 192
        assert Hq % Hkv == 0, (Hq, Hkv)
        return {
            "x": _w((lambda *s: _rng.normal(s) * 0.05)(B, Sq, D)),
            "k_cache": _w((lambda *s: _rng.normal(s) * 0.05)(B, Hkv, Sk, Dh)),
            "v_cache": _w((lambda *s: _rng.normal(s) * 0.05)(B, Hkv, Sk, Dh)),
            "wq": _w((lambda *s: _rng.normal(s) * 0.05)(D, Hq * Dh) * (D ** -0.5)),
            "wo": _w((lambda *s: _rng.normal(s) * 0.05)(Hq * Dh, D) * ((Hq * Dh) ** -0.5)),
        }
    _A_in = _A_setup()

    def _B_setup():
        B, S, D, F, C = 4, 1, 640, 1536, 1
        return {
            "x": _w((lambda *s: _rng.normal(s) * 0.05)(B, S, D)),
            "w_r": _w((lambda *s: _rng.normal(s) * 0.05)(D)),
            "w_gate": _w((lambda *s: _rng.normal(s) * 0.05)(D, F)),
            "w_up": _w((lambda *s: _rng.normal(s) * 0.05)(D, F)),
            "w_down": _w((lambda *s: _rng.normal(s) * 0.05)(F, D)),
        }
    _B_in = _B_setup()

    return {
        "A_x": _A_in["x"],
        "A_k_cache": _A_in["k_cache"],
        "A_v_cache": _A_in["v_cache"],
        "A_wq": _A_in["wq"],
        "A_wo": _A_in["wo"],
        "B_x": _B_in["x"],
        "B_w_r": _B_in["w_r"],
        "B_w_gate": _B_in["w_gate"],
        "B_w_up": _B_in["w_up"],
        "B_w_down": _B_in["w_down"],
    }

def reference(A_x, A_k_cache, A_v_cache, A_wq, A_wo, B_x, B_w_r, B_w_gate, B_w_up, B_w_down):
    def _A_ref(x, k_cache, v_cache, wq, wo):
        B, Sq, D = x.shape
        Hq, Dh = 32, 192
        Hkv, Sk = k_cache.shape[1], k_cache.shape[2]
        W = min(4096, max(256, Sk // 4))
        rep = Hq // Hkv
        q = (lambda x, *d: x.transpose(*d))((x @ wq).reshape(B, Sq, Hq, Dh), 0, 2, 1, 3)
        k = jnp.repeat(k_cache[:, :, Sk - W:, :], rep, axis=1)
        v = jnp.repeat(v_cache[:, :, Sk - W:, :], rep, axis=1)
        scores = jnp.einsum("bhqd,bhkd->bhqk", q, k) * (Dh ** -0.5)
        p = _softmax(scores, axis=-1)
        o = jnp.einsum("bhqk,bhkd->bhqd", p, v)
        return (lambda x, *d: x.transpose(*d))(o, 0, 2, 1, 3).reshape(B, Sq, Hq * Dh) @ wo

    def _B_ref(x, w_r, w_gate, w_up, w_down):
        B, S, D = x.shape
        C = 1
        r = x @ w_r
        idx = jnp.argsort(-r, axis=-1)[:, :C]
        idx_e = jnp.repeat(idx.reshape(B, C, 1), D, axis=2)
        x_sel = jnp.take_along_axis(x, idx_e, axis=1)
        g = _silu(x_sel @ w_gate)
        u = x_sel @ w_up
        y = (g * u) @ w_down
        r_sel = _sigmoid(jnp.take_along_axis(r, idx, axis=1))
        y = y * r_sel.reshape(B, C, 1)
        b_off = (jnp.arange(B) * S).reshape(B, 1)
        flat_idx = (idx + b_off).reshape(B * C)
        zero = (x * 0.0).reshape(B * S, D)
        upd = _scatter_add(zero, flat_idx, y.reshape(B * C, D), axis=0)
        return x + upd.reshape(B, S, D)

    x = A_x
    x = x + _A_ref(_layernorm(x, axis=-1), A_k_cache, A_v_cache, A_wq, A_wo)
    x = x + _B_ref(_layernorm(x, axis=-1), B_w_r, B_w_gate, B_w_up, B_w_down)
    x = x + _A_ref(_layernorm(x, axis=-1), A_k_cache, A_v_cache, A_wq, A_wo)
    x = x + _B_ref(_layernorm(x, axis=-1), B_w_r, B_w_gate, B_w_up, B_w_down)
    return x
```

```python
import jax
import jax.numpy as jnp
from jax import lax
import jax.experimental.pallas as pl
import jax.experimental.pallas.tpu as pltpu

_F32 = jnp.float32
_BF16 = jnp.bfloat16
_U32 = jnp.uint32


def _layernorm(x):
    m = jnp.mean(x, axis=-1, keepdims=True)
    xc = x - m
    v = jnp.mean(xc * xc, axis=-1, keepdims=True)
    return xc * lax.rsqrt(v + 1e-5)


def _pack(x):
    return pltpu.bitcast(x, _U32)


def _unpack(x):
    return pltpu.bitcast(x, _BF16)


def _dot(a, b):
    return jnp.dot(a, b, preferred_element_type=_F32)


@jax.jit
def pallas_interleave_layers__sliding_block_cached__moe_arch_mod__decode_kernel(
    A_x: jax.Array,
    A_k_cache: jax.Array,
    A_v_cache: jax.Array,
    A_wq: jax.Array,
    A_wo: jax.Array,
    B_x: jax.Array,
    B_w_r: jax.Array,
    B_w_gate: jax.Array,
    B_w_up: jax.Array,
    B_w_down: jax.Array,
):
    B, Sq, D = A_x.shape
    _, H, Sk, Dh = A_k_cache.shape
    F = B_w_gate.shape[1]
    W = min(4096, max(256, Sk // 4))
    assert Sq == 1 and H == 32 and Dh == 192 and B <= 8
    DP = 2 * Dh
    NC = H // 2
    NL = W // 128
    scale = float(Dh) ** -0.5

    def kernel(x_hbm, k_hbm, v_hbm, wq_hbm, wo_hbm, wr_hbm, wg_hbm, wu_hbm, wd_hbm,
               o_ref,
               kraw, vraw, kp, vf,
               wq_r, wo_r, wg_r, wu_r, wd_r,
               wq_p, wo_p, wg_p, wu_p, wd_p,
               x_v, wr_v, xs_v, q1_v,
               ksem, vsem, wsem):

        def k_copy(b, c):
            return pltpu.make_async_copy(
                k_hbm.at[b, c, :, pl.ds(Sk - W, W)], kraw.at[c], ksem.at[c])

        def v_copy(b, c):
            return pltpu.make_async_copy(
                v_hbm.at[b, c, :, pl.ds(Sk - W, W)], vraw.at[c], vsem.at[c])

        w_copies = [
            pltpu.make_async_copy(src, dst, wsem.at[i])
            for i, (src, dst) in enumerate([
                (wq_hbm, wq_r), (x_hbm, x_v), (wr_hbm, wr_v), (wo_hbm, wo_r),
                (wg_hbm, wg_r), (wu_hbm, wu_r), (wd_hbm, wd_r)])
        ]
        for cp in w_copies:
            cp.start()

        def start0(c, _):
            k_copy(0, c).start()
            v_copy(0, c).start()
            return 0
        lax.fori_loop(0, NC, start0, 0)

        def repack(raw, packed, rows):
            def go(i, _):
                r = pl.multiple_of(i * rows, rows)
                r2 = pl.multiple_of(i * (rows // 2), rows // 2)
                packed[pl.ds(r2, rows // 2), :] = _pack(raw[pl.ds(r, rows), :])
                return 0
            lax.fori_loop(0, raw.shape[0] // rows, go, 0)

        row16 = lax.broadcasted_iota(jnp.int32, (16, DP), 0)
        col16 = lax.broadcasted_iota(jnp.int32, (16, DP), 1)
        qmask = (row16 < 8) == (col16 < Dh)
        first_head = lax.broadcasted_iota(jnp.int32, (8, DP), 1) < Dh

        def q_block(q8):
            q16 = jnp.concatenate([q8, q8], axis=0)
            return jnp.where(qmask, q16, 0.0).astype(_BF16)

        def softmax_parts(s):
            m = jnp.max(s, axis=-1, keepdims=True)
            p = jnp.exp(s - m)
            return p, jnp.sum(p, axis=-1, keepdims=True)

        def pv(p, l, load_v):
            parts = []
            for t in range(DP // 16):
                pp = p[0:8] if t < Dh // 16 else p[8:16]
                pr = load_v(t) * jnp.concatenate([pp, pp], axis=0)
                a = pr[:, 0:128]
                for j in range(1, NL):
                    a = a + pr[:, j * 128:(j + 1) * 128]
                parts.append(a)
            acc = jnp.concatenate(parts, axis=0)
            o = jnp.sum(acc.T, axis=0, keepdims=True)
            linv = 1.0 / l
            linv = jnp.where(first_head, jnp.broadcast_to(linv[0:8], (8, DP)),
                             jnp.broadcast_to(linv[8:16], (8, DP)))
            o = jnp.broadcast_to(o, (8, DP)) * linv
            return jnp.concatenate([o, o], axis=0).astype(_BF16)

        def ffn(x, wr):
            xn = _layernorm(x)
            r = jnp.sum(xn * wr, axis=-1, keepdims=True)
            xb = jnp.concatenate([xn, xn], axis=0).astype(_BF16)
            g = _dot(xb, _unpack(wg_p[...]))[0:8]
            u = _dot(xb, _unpack(wu_p[...]))[0:8]
            hm = g * jax.nn.sigmoid(g) * u
            hb = jnp.concatenate([hm, hm], axis=0).astype(_BF16)
            y = _dot(hb, _unpack(wd_p[...]))[0:8]
            return x + xn + y * jax.nn.sigmoid(r)

        w_copies[0].wait()
        w_copies[1].wait()
        w_copies[2].wait()
        repack(wq_r, wq_p, 16)
        xs_v[...] = jnp.zeros(xs_v.shape, _F32)
        xs_v[0:B, :] = x_v[...].astype(_F32)
        wr = wr_v[...].astype(_F32).reshape(1, D)
        xn0 = _layernorm(xs_v[...])
        xn0 = jnp.concatenate([xn0, xn0], axis=0).astype(_BF16)

        def q1_go(c, _):
            col = pl.multiple_of(c * DP, 128)
            q1_v[:, pl.ds(col, DP)] = _dot(xn0, _unpack(wq_p[:, pl.ds(col, DP)]))[0:8] * scale
            return 0
        lax.fori_loop(0, NC, q1_go, 0)

        w_copies[3].wait()
        repack(wo_r, wo_p, 128)
        w_copies[4].wait()
        repack(wg_r, wg_p, 64)
        w_copies[5].wait()
        repack(wu_r, wu_p, 64)
        w_copies[6].wait()
        repack(wd_r, wd_p, 128)

        def batch(b, _):
            x = jnp.broadcast_to(xs_v[pl.ds(b, 1), :], (8, D))

            def pair(c, acc):
                col = pl.multiple_of(c * DP, 128)
                q = q_block(jnp.broadcast_to(q1_v[pl.ds(b, 1), pl.ds(col, DP)], (8, DP)))
                k_copy(b, c).wait()
                kk = kraw[c]
                kp[c] = _pack(kk)
                p, l = softmax_parts(_dot(q, kk))

                @pl.when(b + 1 < B)
                def _():
                    k_copy(b + 1, c).start()

                v_copy(b, c).wait()

                def load_v(t):
                    vv = vraw[c, t * 16:(t + 1) * 16, :].astype(_F32)
                    vf[c, t * 16:(t + 1) * 16, :] = vv
                    return vv
                o = pv(p, l, load_v)

                @pl.when(b + 1 < B)
                def _():
                    v_copy(b + 1, c).start()

                row = pl.multiple_of(c * (DP // 2), 64)
                return acc + _dot(o, _unpack(wo_p[pl.ds(row, DP // 2), :]))[0:8]

            x = x + lax.fori_loop(0, NC, pair, jnp.zeros((8, D), _F32))
            x = ffn(x, wr)

            xn = _layernorm(x)
            xb = jnp.concatenate([xn, xn], axis=0).astype(_BF16)
            SA, SB, SD = 3, 2, 1
            qs, pls, os_ = {}, {}, {}
            acc = jnp.zeros((8, D), _F32)
            for g in range(-SA, NC + SD):
                ga, gb, gd = g + SA, g + SB, g - SD
                if 0 <= ga < NC:
                    q = _dot(xb, _unpack(wq_p[:, ga * DP:(ga + 1) * DP])) * scale
                    qs[ga] = jnp.where(qmask, q, 0.0).astype(_BF16)
                if 0 <= gb < NC:
                    pls[gb] = softmax_parts(_dot(qs[gb], _unpack(kp[gb])))
                if 0 <= gd < NC:
                    acc = acc + _dot(os_[gd], _unpack(wo_p[gd * (DP // 2):(gd + 1) * (DP // 2), :]))[0:8]
                if 0 <= g < NC:
                    os_[g] = pv(*pls[g], lambda t, g=g: vf[g, t * 16:(t + 1) * 16, :])
            x = x + acc
            x = ffn(x, wr)
            xs_v[pl.ds(b, 1), :] = x[0:1, :]
            return 0

        lax.fori_loop(0, B, batch, 0)
        o_ref[...] = xs_v[0:B, :].astype(o_ref.dtype)

    any_spec = pl.BlockSpec(memory_space=pl.ANY)
    out = pl.pallas_call(
        kernel,
        in_specs=[any_spec] * 9,
        out_specs=pl.BlockSpec(memory_space=pltpu.VMEM),
        out_shape=jax.ShapeDtypeStruct((B, D), A_x.dtype),
        scratch_shapes=[
            pltpu.VMEM((NC, DP, W), _BF16),
            pltpu.VMEM((NC, DP, W), _BF16),
            pltpu.VMEM((NC, DP // 2, W), _U32),
            pltpu.VMEM((NC, DP, W), _F32),
            pltpu.VMEM((D, H * Dh), _BF16),
            pltpu.VMEM((H * Dh, D), _BF16),
            pltpu.VMEM((D, F), _BF16),
            pltpu.VMEM((D, F), _BF16),
            pltpu.VMEM((F, D), _BF16),
            pltpu.VMEM((D // 2, H * Dh), _U32),
            pltpu.VMEM((H * Dh // 2, D), _U32),
            pltpu.VMEM((D // 2, F), _U32),
            pltpu.VMEM((D // 2, F), _U32),
            pltpu.VMEM((F // 2, D), _U32),
            pltpu.VMEM((B, D), _BF16),
            pltpu.VMEM((D,), _BF16),
            pltpu.VMEM((8, D), _F32),
            pltpu.VMEM((8, H * Dh), _F32),
            pltpu.SemaphoreType.DMA((NC,)),
            pltpu.SemaphoreType.DMA((NC,)),
            pltpu.SemaphoreType.DMA((7,)),
        ],
        compiler_params=pltpu.CompilerParams(vmem_limit_bytes=120 * 1024 * 1024),
    )(
        A_x.reshape(B, D),
        jnp.swapaxes(A_k_cache, 2, 3).reshape(B, NC, DP, Sk),
        jnp.swapaxes(A_v_cache, 2, 3).reshape(B, NC, DP, Sk),
        A_wq, A_wo, B_w_r, B_w_gate, B_w_up, B_w_down,
    )
    return out.reshape(B, Sq, D)
```

```python
import jax
import jax.numpy as jnp
from jax import lax
import jax.experimental.pallas as pl
import jax.experimental.pallas.tpu as pltpu

_F32 = jnp.float32
_BF16 = jnp.bfloat16
_U32 = jnp.uint32


def _layernorm(x):
    m = jnp.mean(x, axis=-1, keepdims=True)
    xc = x - m
    v = jnp.mean(xc * xc, axis=-1, keepdims=True)
    return xc * lax.rsqrt(v + 1e-5)


def _pack(x):
    return pltpu.bitcast(x, _U32)


def _unpack(x):
    return pltpu.bitcast(x, _BF16)


def _dot(a, b):
    return jnp.dot(a, b, preferred_element_type=_F32)


@jax.jit
def pallas_interleave_layers__sliding_block_cached__moe_arch_mod__decode_kernel(
    A_x: jax.Array,
    A_k_cache: jax.Array,
    A_v_cache: jax.Array,
    A_wq: jax.Array,
    A_wo: jax.Array,
    B_x: jax.Array,
    B_w_r: jax.Array,
    B_w_gate: jax.Array,
    B_w_up: jax.Array,
    B_w_down: jax.Array,
):
    B, Sq, D = A_x.shape
    _, H, Sk, Dh = A_k_cache.shape
    F = B_w_gate.shape[1]
    W = min(4096, max(256, Sk // 4))
    assert Sq == 1 and H == 32 and Dh == 192 and B <= 8
    DP = 2 * Dh
    NC = H // 2
    NL = W // 128
    NJ = 3
    GP = 2
    NG = NC // GP
    GI = GP * DP // (16 * NJ)
    PI = GI // GP
    scale = float(Dh) ** -0.5

    def kernel(x_hbm, k_hbm, v_hbm, wq_hbm, wo_hbm, wr_hbm, wg_hbm, wu_hbm, wd_hbm,
               o_ref,
               kraw, vraw, kp, vf,
               wq_r, wo_r, wg_r, wu_r, wd_r,
               wq_p, wo_p, wg_p, wu_p, wd_p,
               x_v, wr_v, xs_v, q1_v,
               ksem, vsem, wsem):

        def k_copies(b, g):
            return [pltpu.make_async_copy(
                k_hbm.at[b, g, :, j, :, pl.ds(Sk - W, W)], kraw.at[g, :, j],
                ksem.at[g * NJ + j]) for j in range(NJ)]

        def v_copies(b, g):
            return [pltpu.make_async_copy(
                v_hbm.at[b, g, :, j, :, pl.ds(Sk - W, W)], vraw.at[g, :, j],
                vsem.at[g * NJ + j]) for j in range(NJ)]

        w_copies = [
            pltpu.make_async_copy(src, dst, wsem.at[i])
            for i, (src, dst) in enumerate([
                (wq_hbm, wq_r), (x_hbm, x_v), (wr_hbm, wr_v), (wo_hbm, wo_r),
                (wg_hbm, wg_r), (wu_hbm, wu_r), (wd_hbm, wd_r)])
        ]
        for cp in w_copies:
            cp.start()

        def start0(g, _):
            for cp in k_copies(0, g) + v_copies(0, g):
                cp.start()
            return 0
        lax.fori_loop(0, NG, start0, 0)

        def repack(raw, packed, rows):
            def go(i, _):
                r = pl.multiple_of(i * rows, rows)
                r2 = pl.multiple_of(i * (rows // 2), rows // 2)
                packed[pl.ds(r2, rows // 2), :] = _pack(raw[pl.ds(r, rows), :])
                return 0
            lax.fori_loop(0, raw.shape[0] // rows, go, 0)

        row16 = lax.broadcasted_iota(jnp.int32, (16, DP), 0)
        col16 = lax.broadcasted_iota(jnp.int32, (16, DP), 1)
        qmask = (row16 < 8) == (col16 < Dh)
        first_head = lax.broadcasted_iota(jnp.int32, (8, DP), 1) < Dh

        def q_block(q8):
            q16 = jnp.concatenate([q8, q8], axis=0)
            return jnp.where(qmask, q16, 0.0).astype(_BF16)

        def softmax_parts(s):
            m = jnp.max(s, axis=-1, keepdims=True)
            p = jnp.exp(s - m)
            return p, jnp.sum(p, axis=-1, keepdims=True)

        def pv(p, l, load_v):
            parts = []
            for t in range(DP // 16):
                pp = p[0:8] if t < Dh // 16 else p[8:16]
                pr = load_v(t) * jnp.concatenate([pp, pp], axis=0)
                a = pr[:, 0:128]
                for j in range(1, NL):
                    a = a + pr[:, j * 128:(j + 1) * 128]
                parts.append(a)
            acc = jnp.concatenate(parts, axis=0)
            o = jnp.sum(acc.T, axis=0, keepdims=True)
            linv = 1.0 / l
            linv = jnp.where(first_head, jnp.broadcast_to(linv[0:8], (8, DP)),
                             jnp.broadcast_to(linv[8:16], (8, DP)))
            o = jnp.broadcast_to(o, (8, DP)) * linv
            return jnp.concatenate([o, o], axis=0).astype(_BF16)

        def ffn(x, wr):
            xn = _layernorm(x)
            r = jnp.sum(xn * wr, axis=-1, keepdims=True)
            xb = jnp.concatenate([xn, xn], axis=0).astype(_BF16)
            g = _dot(xb, _unpack(wg_p[...]))[0:8]
            u = _dot(xb, _unpack(wu_p[...]))[0:8]
            hm = g * jax.nn.sigmoid(g) * u
            hb = jnp.concatenate([hm, hm], axis=0).astype(_BF16)
            y = _dot(hb, _unpack(wd_p[...]))[0:8]
            return x + xn + y * jax.nn.sigmoid(r)

        w_copies[0].wait()
        w_copies[1].wait()
        w_copies[2].wait()
        repack(wq_r, wq_p, 16)
        xs_v[...] = jnp.zeros(xs_v.shape, _F32)
        xs_v[0:B, :] = x_v[...].astype(_F32)
        wr = wr_v[...].astype(_F32).reshape(1, D)
        xn0 = _layernorm(xs_v[...])
        xn0 = jnp.concatenate([xn0, xn0], axis=0).astype(_BF16)

        def q1_go(c, _):
            col = pl.multiple_of(c * DP, 128)
            q1_v[:, pl.ds(col, DP)] = _dot(xn0, _unpack(wq_p[:, pl.ds(col, DP)]))[0:8] * scale
            return 0
        lax.fori_loop(0, NC, q1_go, 0)

        w_copies[3].wait()
        repack(wo_r, wo_p, 128)
        w_copies[4].wait()
        repack(wg_r, wg_p, 64)
        w_copies[5].wait()
        repack(wu_r, wu_p, 64)
        w_copies[6].wait()
        repack(wd_r, wd_p, 128)

        def batch(b, _):
            x = jnp.broadcast_to(xs_v[pl.ds(b, 1), :], (8, D))

            def group(g, acc):
                for cp in k_copies(b, g):
                    cp.wait()
                pls = []
                for i in range(GP):
                    c = g * GP + i
                    col = pl.multiple_of(c * DP, 128)
                    q = q_block(jnp.broadcast_to(q1_v[pl.ds(b, 1), pl.ds(col, DP)], (8, DP)))
                    kk = kraw[g, i * PI:(i + 1) * PI].reshape(DP, W)
                    kp[c] = _pack(kk)
                    pls.append(softmax_parts(_dot(q, kk)))

                @pl.when(b + 1 < B)
                def _():
                    for cp in k_copies(b + 1, g):
                        cp.start()

                for cp in v_copies(b, g):
                    cp.wait()
                os_ = []
                for i in range(GP):
                    c = g * GP + i

                    def load_v(t):
                        vv = vraw[g, i * PI + t // NJ, t % NJ].astype(_F32)
                        vf[c, t * 16:(t + 1) * 16, :] = vv
                        return vv
                    os_.append(pv(*pls[i], load_v))

                @pl.when(b + 1 < B)
                def _():
                    for cp in v_copies(b + 1, g):
                        cp.start()

                row = pl.multiple_of(g * (GP * DP // 2), 64)
                o = jnp.concatenate(os_, axis=1)
                return acc + _dot(o, _unpack(wo_p[pl.ds(row, GP * DP // 2), :]))[0:8]

            x = x + lax.fori_loop(0, NG, group, jnp.zeros((8, D), _F32))
            x = ffn(x, wr)

            xn = _layernorm(x)
            xb = jnp.concatenate([xn, xn], axis=0).astype(_BF16)
            SA, SB, SD = 3, 2, 1
            qs, pls, os_ = {}, {}, {}
            acc = jnp.zeros((8, D), _F32)
            for g in range(-SA, NC + SD):
                ga, gb, gd = g + SA, g + SB, g - SD
                if 0 <= ga < NC:
                    q = _dot(xb, _unpack(wq_p[:, ga * DP:(ga + 1) * DP])) * scale
                    qs[ga] = jnp.where(qmask, q, 0.0).astype(_BF16)
                if 0 <= gb < NC:
                    pls[gb] = softmax_parts(_dot(qs[gb], _unpack(kp[gb])))
                if 0 <= gd < NC:
                    acc = acc + _dot(os_[gd], _unpack(wo_p[gd * (DP // 2):(gd + 1) * (DP // 2), :]))[0:8]
                if 0 <= g < NC:
                    os_[g] = pv(*pls[g], lambda t, g=g: vf[g, t * 16:(t + 1) * 16, :])
            x = x + acc
            x = ffn(x, wr)
            xs_v[pl.ds(b, 1), :] = x[0:1, :]
            return 0

        lax.fori_loop(0, B, batch, 0)
        o_ref[...] = xs_v[0:B, :].astype(o_ref.dtype)

    any_spec = pl.BlockSpec(memory_space=pl.ANY)
    out = pl.pallas_call(
        kernel,
        in_specs=[any_spec] * 9,
        out_specs=pl.BlockSpec(memory_space=pltpu.VMEM),
        out_shape=jax.ShapeDtypeStruct((B, D), A_x.dtype),
        scratch_shapes=[
            pltpu.VMEM((NG, GI, NJ, 16, W), _BF16),
            pltpu.VMEM((NG, GI, NJ, 16, W), _BF16),
            pltpu.VMEM((NC, DP // 2, W), _U32),
            pltpu.VMEM((NC, DP, W), _F32),
            pltpu.VMEM((D, H * Dh), _BF16),
            pltpu.VMEM((H * Dh, D), _BF16),
            pltpu.VMEM((D, F), _BF16),
            pltpu.VMEM((D, F), _BF16),
            pltpu.VMEM((F, D), _BF16),
            pltpu.VMEM((D // 2, H * Dh), _U32),
            pltpu.VMEM((H * Dh // 2, D), _U32),
            pltpu.VMEM((D // 2, F), _U32),
            pltpu.VMEM((D // 2, F), _U32),
            pltpu.VMEM((F // 2, D), _U32),
            pltpu.VMEM((B, D), _BF16),
            pltpu.VMEM((D,), _BF16),
            pltpu.VMEM((8, D), _F32),
            pltpu.VMEM((8, H * Dh), _F32),
            pltpu.SemaphoreType.DMA((NG * NJ,)),
            pltpu.SemaphoreType.DMA((NG * NJ,)),
            pltpu.SemaphoreType.DMA((7,)),
        ],
        compiler_params=pltpu.CompilerParams(vmem_limit_bytes=120 * 1024 * 1024),
    )(
        A_x.reshape(B, D),
        jnp.swapaxes(A_k_cache, 2, 3).reshape(B, NG, GI, NJ, 16, Sk),
        jnp.swapaxes(A_v_cache, 2, 3).reshape(B, NG, GI, NJ, 16, Sk),
        A_wq, A_wo, B_w_r, B_w_gate, B_w_up, B_w_down,
    )
    return out.reshape(B, Sq, D)
```

```python
import jax
import jax.numpy as jnp
from jax import lax
import jax.experimental.pallas as pl
import jax.experimental.pallas.tpu as pltpu

_F32 = jnp.float32
_BF16 = jnp.bfloat16
_U32 = jnp.uint32
_LOG2E = 1.4426950408889634


def _center(x):
    xc = x - jnp.mean(x, axis=-1, keepdims=True)
    v = jnp.mean(xc * xc, axis=-1, keepdims=True)
    return xc, lax.rsqrt(v + 1e-5)


def _pack(x):
    return pltpu.bitcast(x, _U32)


def _unpack(x):
    return pltpu.bitcast(x, _BF16)


def _dot(a, b):
    return jnp.dot(a, b, preferred_element_type=_F32)


def _lhs(x8):
    return jnp.concatenate([x8, x8], axis=0).astype(_BF16)


@jax.jit
def pallas_interleave_layers__sliding_block_cached__moe_arch_mod__decode_kernel(
    A_x: jax.Array,
    A_k_cache: jax.Array,
    A_v_cache: jax.Array,
    A_wq: jax.Array,
    A_wo: jax.Array,
    B_x: jax.Array,
    B_w_r: jax.Array,
    B_w_gate: jax.Array,
    B_w_up: jax.Array,
    B_w_down: jax.Array,
):
    B, Sq, D = A_x.shape
    _, H, Sk, Dh = A_k_cache.shape
    F = B_w_gate.shape[1]
    W = min(4096, max(256, Sk // 4))
    assert Sq == 1 and H == 32 and Dh == 192 and B <= 8
    DP = 2 * Dh
    NC = H // 2
    NL = W // 128
    NJ = 3
    GP = 2
    NG = NC // GP
    GI = GP * DP // (16 * NJ)
    PI = GI // GP
    HI = PI // 2
    NS = 4
    qscale = float(Dh) ** -0.5 * _LOG2E

    def kernel(x_hbm, k_hbm, v_hbm, wq_hbm, wo_hbm, wr_hbm, wg_hbm, wu_hbm, wd_hbm,
               o_ref,
               kraw, vraw, kp, vf,
               wq_r, wo_r, wg_r, wu_r, wd_r,
               wq_p, wo_p, wg_p, wu_p, wd_p,
               x_v, wr_v, xs_v, q1_v, p_v,
               ksem, vsem, lsem):

        def k_copies(b, g):
            s = g % NS
            return [pltpu.make_async_copy(
                k_hbm.at[b, g, :, j, :, pl.ds(Sk - W, W)], kraw.at[s, :, j],
                ksem.at[s]) for j in range(NJ)]

        def v_copies(b, g, last):
            s = g % NS
            return [pltpu.make_async_copy(
                v_hbm.at[b, g, :, j, :, pl.ds(Sk - W, W)], vraw.at[s, :, j],
                lsem.at[j] if last else vsem.at[s]) for j in range(NJ)]

        def start_next(copies, b, g, **kw):
            n = b * NG + g + NS

            @pl.when(n < B * NG)
            def _():
                for cp in copies(n // NG, n % NG, **kw):
                    cp.start()

        w_sets = [
            [(x_hbm, x_v), (wr_hbm, wr_v), (wq_hbm, wq_r)],
            [(wo_hbm, wo_r)],
            [(wg_hbm, wg_r), (wu_hbm, wu_r), (wd_hbm, wd_r)],
        ]
        w_copies = [[pltpu.make_async_copy(src, dst, lsem.at[i]) for src, dst in ws]
                    for i, ws in enumerate(w_sets)]
        for ws in w_copies:
            for cp in ws:
                cp.start()

        def start0(g, _):
            for cp in k_copies(0, g) + v_copies(0, g, False):
                cp.start()
            return 0
        lax.fori_loop(0, NS, start0, 0)

        def repack(raw, packed, rows):
            def go(i, _):
                r = pl.multiple_of(i * rows, rows)
                r2 = pl.multiple_of(i * (rows // 2), rows // 2)
                packed[pl.ds(r2, rows // 2), :] = _pack(raw[pl.ds(r, rows), :])
                return 0
            lax.fori_loop(0, raw.shape[0] // rows, go, 0)

        row16 = lax.broadcasted_iota(jnp.int32, (16, DP), 0)
        col16 = lax.broadcasted_iota(jnp.int32, (16, DP), 1)
        qmask = (row16 < 8) == (col16 < Dh)
        low_half = lax.broadcasted_iota(jnp.int32, (8, 128), 1) < 64

        def scores(q16, kk):
            q = jnp.where(qmask, q16, 0.0).astype(_BF16)
            s0 = _dot(q[:, 0:128], kk[0:128])
            s1 = _dot(q[:, 128:256], kk[128:256])
            s2 = _dot(q[:, 256:384], kk[256:384])
            return s1 + jnp.concatenate([s0[0:8], s2[8:16]], axis=0)

        def softmax_parts(s):
            m = jnp.max(s, axis=-1, keepdims=True)
            p = jnp.exp2(s - m)
            linv = 1.0 / jnp.sum(p, axis=-1, keepdims=True)
            return p, jnp.where(low_half, linv[0:8], linv[8:16])

        def pv_chunk(pp, vv):
            pr = vv * jnp.concatenate([pp, pp], axis=0)
            a = pr[:, 0:128]
            for j in range(1, NL):
                a = a + pr[:, j * 128:(j + 1) * 128]
            return a

        def lane_sums(parts, linv):
            acc = jnp.concatenate(parts, axis=0)
            o = jnp.sum(acc.T, axis=0, keepdims=True)
            return _lhs(jnp.broadcast_to(o, linv.shape) * linv)

        def ffn(x, wr):
            xc, rstd = _center(x)
            r = jnp.sum(xc * wr, axis=-1, keepdims=True) * rstd
            xb = _lhs(xc)
            g = _dot(xb, _unpack(wg_p[...]))[0:8] * rstd
            u = _dot(xb, _unpack(wu_p[...]))[0:8] * rstd
            hm = g * jax.nn.sigmoid(g) * u
            y = _dot(_lhs(hm), _unpack(wd_p[...]))[0:8]
            return x + xc * rstd + y * jax.nn.sigmoid(r)

        for cp in w_copies[0]:
            cp.wait()
        repack(wq_r, wq_p, 16)
        xs_v[...] = jnp.zeros(xs_v.shape, _F32)
        xs_v[0:B, :] = x_v[...].astype(_F32)
        wr = wr_v[...].astype(_F32).reshape(1, D)
        xc0, rstd0 = _center(xs_v[...])
        xb0 = _lhs(xc0)

        def q1_go(c, _):
            col = pl.multiple_of(c * DP, 128)
            q1_v[:, pl.ds(col, DP)] = (
                _dot(xb0, _unpack(wq_p[:, pl.ds(col, DP)]))[0:8] * (rstd0 * qscale))
            return 0
        lax.fori_loop(0, NC, q1_go, 0)

        for cp in w_copies[1]:
            cp.wait()

        def wo_go(n, _):
            g = n // GI
            i = n % GI
            for j in range(NJ):
                wo_p[g, j, pl.ds(pl.multiple_of(i * 8, 8), 8), :] = _pack(wo_r[g, i, j])
            return 0
        lax.fori_loop(0, NG * GI, wo_go, 0)

        for cp in w_copies[2]:
            cp.wait()
        repack(wg_r, wg_p, 64)
        repack(wu_r, wu_p, 64)
        repack(wd_r, wd_p, 128)

        def batch(b, _):
            x = jnp.broadcast_to(xs_v[pl.ds(b, 1), :], (8, D))

            def group(g, acc, last):
                s = g % NS
                for cp in k_copies(b, g):
                    cp.wait()
                linvs = []
                for i in range(GP):
                    c = g * GP + i
                    col = c * DP if last else pl.multiple_of(c * DP, 128)
                    q16 = jnp.broadcast_to(q1_v[pl.ds(b, 1), pl.ds(col, DP)], (16, DP))
                    kk = kraw[s, i * PI:(i + 1) * PI].reshape(DP, W)
                    kp[c] = _pack(kk)
                    p, linv = softmax_parts(scores(q16, kk))
                    p_v[i] = p
                    linvs.append(linv)
                linv = jnp.concatenate(linvs, axis=1)
                start_next(k_copies, b, g)

                vcs = v_copies(b, g, last)
                if not last:
                    for cp in vcs:
                        cp.wait()
                for j in range(NJ):
                    if last:
                        vcs[j].wait()
                    parts = []
                    for i in range(GI):
                        h = i // HI
                        vv = vraw[s, i, j].astype(_F32)
                        if not (last and j == NJ - 1):
                            vf[g, j, i] = vv
                        pp = p_v[h // 2, (h % 2) * 8:(h % 2) * 8 + 8, :]
                        parts.append(pv_chunk(pp, vv))
                    acc = acc + _dot(lane_sums(parts, linv), _unpack(wo_p[g, j]))[0:8]
                if not last:
                    @pl.when(g == NG - 1 - NS)
                    def _():
                        for cp in v_copies(b, NG - 1, True):
                            cp.start()

                    @pl.when(g != NG - 1 - NS)
                    def _():
                        start_next(v_copies, b, g, last=False)
                return acc

            acc = lax.fori_loop(0, NG - 1, lambda g, a: group(g, a, False),
                                jnp.zeros((8, D), _F32))
            x = x + group(NG - 1, acc, True)
            x = ffn(x, wr)
            for i in range(GI):
                vf[NG - 1, NJ - 1, i] = vraw[(NG - 1) % NS, i, NJ - 1].astype(_F32)
            start_next(v_copies, b, NG - 1, last=False)

            xc, rstd = _center(x)
            xb = _lhs(xc)
            qs16 = jnp.concatenate([rstd, rstd], axis=0) * qscale
            SA, SB, SD = 3, 2, 1
            qs, pls, os_ = {}, {}, {}
            acc = jnp.zeros((8, D), _F32)
            for c in range(-SA, NC + SD):
                ca, cb, cd = c + SA, c + SB, c - SD
                if 0 <= ca < NC:
                    qs[ca] = _dot(xb, _unpack(wq_p[:, ca * DP:(ca + 1) * DP])) * qs16
                if 0 <= cb < NC:
                    pls[cb] = softmax_parts(scores(qs[cb], _unpack(kp[cb])))
                if 0 <= cd < NC:
                    r0 = (cd % GP) * PI * 8
                    w = jnp.concatenate(
                        [wo_p[cd // GP, j, r0:r0 + PI * 8, :] for j in range(NJ)], axis=0)
                    acc = acc + _dot(os_[cd], _unpack(w))[0:8]
                if 0 <= c < NC:
                    p, linv = pls[c]
                    parts = {}
                    for i in range(PI):
                        pp = p[0:8] if i < HI else p[8:16]
                        for j in range(NJ):
                            parts[j, i] = pv_chunk(pp, vf[c // GP, j, (c % GP) * PI + i])
                    os_[c] = lane_sums([parts[j, i] for j in range(NJ) for i in range(PI)],
                                       jnp.concatenate([linv] * NJ, axis=1))
            x = x + acc
            x = ffn(x, wr)
            xs_v[pl.ds(b, 1), :] = x[0:1, :]
            return 0

        lax.fori_loop(0, B, batch, 0)
        o_ref[...] = xs_v[0:B, :].astype(o_ref.dtype)

    any_spec = pl.BlockSpec(memory_space=pl.ANY)
    out = pl.pallas_call(
        kernel,
        in_specs=[any_spec] * 9,
        out_specs=pl.BlockSpec(memory_space=pltpu.VMEM),
        out_shape=jax.ShapeDtypeStruct((B, D), A_x.dtype),
        scratch_shapes=[
            pltpu.VMEM((NS, GI, NJ, 16, W), _BF16),
            pltpu.VMEM((NS, GI, NJ, 16, W), _BF16),
            pltpu.VMEM((NC, DP // 2, W), _U32),
            pltpu.VMEM((NG, NJ, GI, 16, W), _F32),
            pltpu.VMEM((D, H * Dh), _BF16),
            pltpu.VMEM((NG, GI, NJ, 16, D), _BF16),
            pltpu.VMEM((D, F), _BF16),
            pltpu.VMEM((D, F), _BF16),
            pltpu.VMEM((F, D), _BF16),
            pltpu.VMEM((D // 2, H * Dh), _U32),
            pltpu.VMEM((NG, NJ, GI * 8, D), _U32),
            pltpu.VMEM((D // 2, F), _U32),
            pltpu.VMEM((D // 2, F), _U32),
            pltpu.VMEM((F // 2, D), _U32),
            pltpu.VMEM((B, D), _BF16),
            pltpu.VMEM((D,), _BF16),
            pltpu.VMEM((8, D), _F32),
            pltpu.VMEM((8, H * Dh), _F32),
            pltpu.VMEM((GP, 16, W), _F32),
            pltpu.SemaphoreType.DMA((NS,)),
            pltpu.SemaphoreType.DMA((NS,)),
            pltpu.SemaphoreType.DMA((NJ,)),
        ],
        compiler_params=pltpu.CompilerParams(vmem_limit_bytes=120 * 1024 * 1024),
    )(
        A_x.reshape(B, D),
        jnp.swapaxes(A_k_cache, 2, 3).reshape(B, NG, GI, NJ, 16, Sk),
        jnp.swapaxes(A_v_cache, 2, 3).reshape(B, NG, GI, NJ, 16, Sk),
        A_wq, A_wo.reshape(NG, GI, NJ, 16, D), B_w_r, B_w_gate, B_w_up, B_w_down,
    )
    return out.reshape(B, Sq, D)
```

```python
import jax
import jax.numpy as jnp
from jax import lax
import jax.experimental.pallas as pl
import jax.experimental.pallas.tpu as pltpu

_F32 = jnp.float32
_BF16 = jnp.bfloat16
_U32 = jnp.uint32
_LOG2E = 1.4426950408889634

_CFG = dict(
    SA=3, SB=2, SM=1, SS=1, order="ABDMSC",
    ka="0022211111111111",
    bd="1111111111111113",
    sd="1111111111111111",
)


def _center(x):
    xc = x - jnp.mean(x, axis=-1, keepdims=True)
    v = jnp.mean(xc * xc, axis=-1, keepdims=True)
    return xc, lax.rsqrt(v + 1e-5)


def _pack(x):
    return pltpu.bitcast(x, _U32)


def _unpack(x):
    return pltpu.bitcast(x, _BF16)


def _dot(a, b):
    return jnp.dot(a, b, preferred_element_type=_F32)


def _lhs(x8):
    return jnp.concatenate([x8, x8], axis=0).astype(_BF16)


def _forward(cfg, A_x, A_k_cache, A_v_cache, A_wq, A_wo, B_w_r, B_w_gate, B_w_up, B_w_down):
    B, Sq, D = A_x.shape
    _, H, Sk, Dh = A_k_cache.shape
    F = B_w_gate.shape[1]
    W = min(4096, max(256, Sk // 4))
    assert Sq == 1 and H == 32 and Dh == 192 and B <= 8 and D % 128 == 0
    DP = 2 * Dh
    NC = H // 2
    NL = W // 128
    DT = D // 128
    NJ = 3
    GP = 2
    NG = NC // GP
    GI = GP * DP // (16 * NJ)
    PI = GI // GP
    HI = PI // 2
    PT = DP // 16
    NS = 4
    qscale = float(Dh) ** -0.5 * _LOG2E

    ka = [int(c) for c in cfg["ka"]]
    bd = [int(c) for c in cfg["bd"]]
    dpos = [n + int(c, 16) for n, c in enumerate(cfg["sd"])]
    wqf_slot = {(c, i): None for c in range(NC) for i in range(DT - ka[c], DT)}
    wqf_slot = {key: n for n, key in enumerate(wqf_slot)}
    wof_slot = {(c, i): None for c in range(NC) for i in range(3 - bd[c], 3)}
    wof_slot = {key: n for n, key in enumerate(wof_slot)}

    def chunk_pos(c, t):
        return c // GP, t % NJ, (c % GP) * PI + t // NJ

    def kernel(x_hbm, k_hbm, v_hbm, wq_hbm, wo_hbm, wr_hbm, wg_hbm, wu_hbm, wd_hbm,
               o_ref,
               kraw, vraw, kp, vf,
               wq_r, wo_r, wg_r, wu_r, wd_r,
               wq_p, wo_p, wg_p, wu_p, wd_p, wq_f, wo_f,
               x_v, wr_v, xs_v, q1_v, p_v,
               ksem, vsem, lsem):

        def k_copies(b, g):
            s = g % NS
            return [pltpu.make_async_copy(
                k_hbm.at[b, g, :, j, :, pl.ds(Sk - W, W)], kraw.at[s, :, j],
                ksem.at[s]) for j in range(NJ)]

        def v_copies(b, g, last):
            s = g % NS
            return [pltpu.make_async_copy(
                v_hbm.at[b, g, :, j, :, pl.ds(Sk - W, W)], vraw.at[s, :, j],
                lsem.at[j] if last else vsem.at[s]) for j in range(NJ)]

        def start_next(copies, b, g, **kw):
            n = b * NG + g + NS

            @pl.when(n < B * NG)
            def _():
                for cp in copies(n // NG, n % NG, **kw):
                    cp.start()

        w_sets = [
            [(wq_hbm, wq_r), (x_hbm, x_v), (wr_hbm, wr_v)],
            [(wo_hbm, wo_r)],
            [(wg_hbm, wg_r), (wu_hbm, wu_r), (wd_hbm, wd_r)],
        ]
        w_copies = [[pltpu.make_async_copy(src, dst, lsem.at[i]) for src, dst in ws]
                    for i, ws in enumerate(w_sets)]
        for ws in w_copies:
            for cp in ws:
                cp.start()

        def start0(g, _):
            for cp in k_copies(0, g) + v_copies(0, g, False):
                cp.start()
            return 0
        lax.fori_loop(0, NS, start0, 0)

        def repack(raw, packed, rows):
            def go(i, _):
                r = pl.multiple_of(i * rows, rows)
                r2 = pl.multiple_of(i * (rows // 2), rows // 2)
                packed[pl.ds(r2, rows // 2), :] = _pack(raw[pl.ds(r, rows), :])
                return 0
            lax.fori_loop(0, raw.shape[0] // rows, go, 0)

        row16 = lax.broadcasted_iota(jnp.int32, (16, DP), 0)
        col16 = lax.broadcasted_iota(jnp.int32, (16, DP), 1)
        qmask = (row16 < 8) == (col16 < Dh)
        low_half = lax.broadcasted_iota(jnp.int32, (8, 128), 1) < 64

        def scores(q16, kk):
            q = jnp.where(qmask, q16, 0.0).astype(_BF16)
            s0 = _dot(q[:, 0:128], kk[0:128])
            s1 = _dot(q[:, 128:256], kk[128:256])
            s2 = _dot(q[:, 256:384], kk[256:384])
            return s1 + jnp.concatenate([s0[0:8], s2[8:16]], axis=0)

        def probs(s):
            return jnp.exp2(s - jnp.max(s, axis=-1, keepdims=True))

        def inv_sum(p):
            return 1.0 / jnp.sum(p, axis=-1, keepdims=True)

        def pv_chunk(pp, vv):
            pr = vv * jnp.concatenate([pp, pp], axis=0)
            a = pr[:, 0:128]
            for j in range(1, NL):
                a = a + pr[:, j * 128:(j + 1) * 128]
            return a

        def lane_sums(parts, linv):
            acc = jnp.concatenate(parts, axis=0)
            o = jnp.sum(acc.T, axis=0, keepdims=True)
            return _lhs(jnp.broadcast_to(o, linv.shape) * linv)

        def ffn(x, wr):
            xc, rstd = _center(x)
            r = jnp.sum(xc * wr, axis=-1, keepdims=True) * rstd
            xb = _lhs(xc)
            g = _dot(xb, _unpack(wg_p[...]))[0:8] * rstd
            u = _dot(xb, _unpack(wu_p[...]))[0:8] * rstd
            hm = g * jax.nn.sigmoid(g) * u
            y = _dot(_lhs(hm), _unpack(wd_p[...]))[0:8]
            return x + xc * rstd + y * jax.nn.sigmoid(r)

        for cp in w_copies[0]:
            cp.wait()
        repack(wq_r, wq_p, 16)

        def wqf_go(t, _):
            for (c, i), n in wqf_slot.items():
                r = pl.multiple_of(i * 128 + t * 16, 16)
                wq_f[n, pl.ds(pl.multiple_of(t * 16, 16), 16), :] = (
                    wq_r[pl.ds(r, 16), c * DP:(c + 1) * DP].astype(_F32))
            return 0
        lax.fori_loop(0, 8, wqf_go, 0)

        xs_v[...] = jnp.zeros(xs_v.shape, _F32)
        xs_v[0:B, :] = x_v[...].astype(_F32)
        wr = wr_v[...].astype(_F32).reshape(1, D)
        xc0, rstd0 = _center(xs_v[...])
        xb0 = _lhs(xc0)

        def q1_go(c, _):
            col = pl.multiple_of(c * DP, 128)
            q1_v[:, pl.ds(col, DP)] = (
                _dot(xb0, _unpack(wq_p[:, pl.ds(col, DP)]))[0:8] * (rstd0 * qscale))
            return 0
        lax.fori_loop(0, NC, q1_go, 0)

        for cp in w_copies[1]:
            cp.wait()

        def wo_go(n, _):
            g = n // GI
            i = n % GI
            for j in range(NJ):
                r = pl.multiple_of((n * NJ + j) * 16, 16)
                wo_p[g, j, pl.ds(pl.multiple_of(i * 8, 8), 8), :] = _pack(wo_r[pl.ds(r, 16), :])
            return 0
        lax.fori_loop(0, NG * GI, wo_go, 0)

        def wof_go(t, _):
            for (c, i), n in wof_slot.items():
                r = pl.multiple_of(c * DP + i * 128 + t * 16, 16)
                wo_f[n, pl.ds(pl.multiple_of(t * 16, 16), 16), :] = (
                    wo_r[pl.ds(r, 16), :].astype(_F32))
            return 0
        lax.fori_loop(0, 8, wof_go, 0)

        for cp in w_copies[2]:
            cp.wait()
        repack(wg_r, wg_p, 64)
        repack(wu_r, wu_p, 64)
        repack(wd_r, wd_p, 128)

        def attention3(x):
            xc, rstd = _center(x)
            qs8 = rstd * qscale
            xb = _lhs(xc)
            xcol = {i: jnp.broadcast_to(xc[0:1, i * 128:(i + 1) * 128], (128, 128)).T
                    for i in range(DT - max(ka), DT)}

            def stage_a(c):
                km = (DT - ka[c]) * 128
                q = None
                if km:
                    q = _dot(xb[:, 0:km], _unpack(wq_p[0:km // 2, c * DP:(c + 1) * DP]))[0:8]
                if ka[c]:
                    a = None
                    for i in range(DT - ka[c], DT):
                        for t in range(16):
                            xx = xcol[i][t * 8:(t + 1) * 8, :]
                            cc = (jnp.concatenate([xx] * (DP // 128), axis=1)
                                  * wq_f[wqf_slot[c, i], t * 8:(t + 1) * 8, :])
                            a = cc if a is None else a + cc
                    a = jnp.sum(a, axis=0, keepdims=True)
                    q = jnp.broadcast_to(a, (8, DP)) if q is None else q + a
                return q * qs8

            def stage_c(p, linv, c):
                nt = (3 - bd[c]) * 8
                head = lambda t: t // (PT // 2)
                chunk = lambda t: pv_chunk(p[head(t) * 8:head(t) * 8 + 8], vf[chunk_pos(c, t)])
                o = None
                if nt:
                    l0 = jnp.broadcast_to(linv[0:8], (8, 128))
                    l1 = jnp.broadcast_to(linv[8:16], (8, 128))
                    li = [l0, jnp.where(low_half, l0, l1), l1][0:nt // 8]
                    o = lane_sums([chunk(t) for t in range(nt)], jnp.concatenate(li, axis=1))
                tot = None
                for hh in range(2):
                    a = None
                    for t in range(nt, PT):
                        if head(t) != hh:
                            continue
                        oc = jnp.sum(chunk(t), axis=1, keepdims=True)
                        cc = oc * wo_f[wof_slot[c, t // 8], (t % 8) * 16:(t % 8) * 16 + 16, :]
                        cc = cc[0:8] + cc[8:16]
                        a = cc if a is None else a + cc
                    if a is not None:
                        a = a * linv[hh * 8:hh * 8 + 8]
                        tot = a if tot is None else tot + a
                return o, tot

            def stage_d(o, c):
                ws = []
                for t in range(o.shape[1] // 16):
                    g, j, i = chunk_pos(c, t)
                    ws.append(wo_p[g, j, i * 8:(i + 1) * 8, :])
                return _dot(o, _unpack(jnp.concatenate(ws, axis=0)))[0:8]

            acc = jnp.zeros((8, D), _F32)
            accv = None
            qs, ss, ps, ls, os_ = {}, {}, {}, {}, {}
            off = dict(A=cfg["SA"], B=cfg["SB"], M=cfg["SM"], S=cfg["SS"], C=0)
            for step in range(-cfg["SA"], max(dpos) + 1):
                for st in cfg["order"]:
                    if st == "D":
                        for n in range(NC):
                            if dpos[n] == step and os_[n] is not None:
                                acc = acc + stage_d(os_[n], n)
                        continue
                    n = step + off[st]
                    if not 0 <= n < NC:
                        continue
                    if st == "A":
                        qs[n] = stage_a(n)
                    elif st == "B":
                        ss[n] = scores(jnp.concatenate([qs[n], qs[n]], axis=0), _unpack(kp[n]))
                    elif st == "M":
                        ps[n] = probs(ss[n])
                    elif st == "S":
                        ls[n] = inv_sum(ps[n])
                    elif st == "C":
                        os_[n], part = stage_c(ps[n], ls[n], n)
                        if part is not None:
                            accv = part if accv is None else accv + part
            if accv is not None:
                acc = acc + jnp.sum(accv, axis=0, keepdims=True)
            return acc

        def batch(b, _):
            x = jnp.broadcast_to(xs_v[pl.ds(b, 1), :], (8, D))

            def group(g, acc, last):
                s = g % NS
                for cp in k_copies(b, g):
                    cp.wait()
                linvs = []
                for i in range(GP):
                    c = g * GP + i
                    col = c * DP if last else pl.multiple_of(c * DP, 128)
                    q16 = jnp.broadcast_to(q1_v[pl.ds(b, 1), pl.ds(col, DP)], (16, DP))
                    kk = kraw[s, i * PI:(i + 1) * PI].reshape(DP, W)
                    kp[c] = _pack(kk)
                    p = probs(scores(q16, kk))
                    p_v[i] = p
                    linv = inv_sum(p)
                    linvs.append(jnp.where(low_half, linv[0:8], linv[8:16]))
                linv = jnp.concatenate(linvs, axis=1)
                start_next(k_copies, b, g)

                vcs = v_copies(b, g, last)
                if not last:
                    for cp in vcs:
                        cp.wait()
                for j in range(NJ):
                    if last:
                        vcs[j].wait()
                    parts = []
                    for i in range(GI):
                        h = i // HI
                        vv = vraw[s, i, j].astype(_F32)
                        if not (last and j == NJ - 1):
                            vf[g, j, i] = vv
                        pp = p_v[h // 2, (h % 2) * 8:(h % 2) * 8 + 8, :]
                        parts.append(pv_chunk(pp, vv))
                    acc = acc + _dot(lane_sums(parts, linv), _unpack(wo_p[g, j]))[0:8]
                if not last:
                    @pl.when(g == NG - 1 - NS)
                    def _():
                        for cp in v_copies(b, NG - 1, True):
                            cp.start()

                    @pl.when(g != NG - 1 - NS)
                    def _():
                        start_next(v_copies, b, g, last=False)
                return acc

            acc = lax.fori_loop(0, NG - 1, lambda g, a: group(g, a, False),
                                jnp.zeros((8, D), _F32))
            x = x + group(NG - 1, acc, True)
            x = ffn(x, wr)
            for i in range(GI):
                vf[NG - 1, NJ - 1, i] = vraw[(NG - 1) % NS, i, NJ - 1].astype(_F32)
            start_next(v_copies, b, NG - 1, last=False)
            x = x + attention3(x)
            x = ffn(x, wr)
            xs_v[pl.ds(b, 1), :] = x[0:1, :]
            return 0

        lax.fori_loop(0, B, batch, 0)
        o_ref[...] = xs_v[0:B, :].astype(o_ref.dtype)

    any_spec = pl.BlockSpec(memory_space=pl.ANY)
    out = pl.pallas_call(
        kernel,
        in_specs=[any_spec] * 9,
        out_specs=pl.BlockSpec(memory_space=pltpu.VMEM),
        out_shape=jax.ShapeDtypeStruct((B, D), A_x.dtype),
        scratch_shapes=[
            pltpu.VMEM((NS, GI, NJ, 16, W), _BF16),
            pltpu.VMEM((NS, GI, NJ, 16, W), _BF16),
            pltpu.VMEM((NC, DP // 2, W), _U32),
            pltpu.VMEM((NG, NJ, GI, 16, W), _F32),
            pltpu.VMEM((D, H * Dh), _BF16),
            pltpu.VMEM((H * Dh, D), _BF16),
            pltpu.VMEM((D, F), _BF16),
            pltpu.VMEM((D, F), _BF16),
            pltpu.VMEM((F, D), _BF16),
            pltpu.VMEM((D // 2, H * Dh), _U32),
            pltpu.VMEM((NG, NJ, GI * 8, D), _U32),
            pltpu.VMEM((D // 2, F), _U32),
            pltpu.VMEM((D // 2, F), _U32),
            pltpu.VMEM((F // 2, D), _U32),
            pltpu.VMEM((max(len(wqf_slot), 1), 128, DP), _F32),
            pltpu.VMEM((max(len(wof_slot), 1), 128, D), _F32),
            pltpu.VMEM((B, D), _BF16),
            pltpu.VMEM((D,), _BF16),
            pltpu.VMEM((8, D), _F32),
            pltpu.VMEM((8, H * Dh), _F32),
            pltpu.VMEM((GP, 16, W), _F32),
            pltpu.SemaphoreType.DMA((NS,)),
            pltpu.SemaphoreType.DMA((NS,)),
            pltpu.SemaphoreType.DMA((NJ,)),
        ],
        compiler_params=pltpu.CompilerParams(vmem_limit_bytes=120 * 1024 * 1024),
    )(
        A_x.reshape(B, D),
        jnp.swapaxes(A_k_cache, 2, 3).reshape(B, NG, GI, NJ, 16, Sk),
        jnp.swapaxes(A_v_cache, 2, 3).reshape(B, NG, GI, NJ, 16, Sk),
        A_wq, A_wo, B_w_r, B_w_gate, B_w_up, B_w_down,
    )
    return out.reshape(B, Sq, D)


@jax.jit
def pallas_interleave_layers__sliding_block_cached__moe_arch_mod__decode_kernel(
    A_x: jax.Array,
    A_k_cache: jax.Array,
    A_v_cache: jax.Array,
    A_wq: jax.Array,
    A_wo: jax.Array,
    B_x: jax.Array,
    B_w_r: jax.Array,
    B_w_gate: jax.Array,
    B_w_up: jax.Array,
    B_w_down: jax.Array,
):
    return _forward(_CFG, A_x, A_k_cache, A_v_cache, A_wq, A_wo,
                    B_w_r, B_w_gate, B_w_up, B_w_down)
```

```python
import jax
import jax.numpy as jnp
from jax import lax
import jax.experimental.pallas as pl
import jax.experimental.pallas.tpu as pltpu

_F32 = jnp.float32
_BF16 = jnp.bfloat16
_U32 = jnp.uint32
_LOG2E = 1.4426950408889634

_CFG = dict(
    SA=3, SB=2, SM=1, SS=1, order="ABDMSC",
    rot=15,
    ka="0022211111111111",
    ra="0000000000000000",
    bd="1111111111111113",
    sd="1111111111111111",
    nv=6, fgrp=3,
)


def _pack(x):
    return pltpu.bitcast(x, _U32)


def _unpack(x):
    return pltpu.bitcast(x, _BF16)


def _dot(a, b):
    return jnp.dot(a, b, preferred_element_type=_F32)


def _dot_t(a, b):
    return lax.dot_general(a, b, (((1,), (1,)), ((), ())), preferred_element_type=_F32)


def _lhs(x8):
    return jnp.concatenate([x8, x8], axis=0).astype(_BF16)


def _lane_fold(x):
    a = x[:, 0:128]
    for j in range(1, x.shape[1] // 128):
        a = a + x[:, j * 128:(j + 1) * 128]
    return a


def _row_sums(parts):
    return jnp.sum(jnp.concatenate(parts, axis=0).T, axis=0, keepdims=True)


def _rstd(xc):
    return lax.rsqrt(jnp.mean(xc * xc, axis=-1, keepdims=True) + 1e-5)


def _compiler_params():
    limit = 120 * 1024 * 1024
    try:
        return pltpu.CompilerParams(vmem_limit_bytes=limit, disable_semaphore_checks=True)
    except TypeError:
        return pltpu.CompilerParams(vmem_limit_bytes=limit)


def _forward(cfg, A_x, A_k_cache, A_v_cache, A_wq, A_wo, B_w_r, B_w_gate, B_w_up, B_w_down):
    B, Sq, D = A_x.shape
    _, H, Sk, Dh = A_k_cache.shape
    F = B_w_gate.shape[1]
    W = min(4096, max(256, Sk // 4))
    assert Sq == 1 and H == 32 and Dh == 192 and B <= 8 and D % 128 == 0 and F % 128 == 0
    DP = 2 * Dh
    NC = H // 2
    DT = D // 128
    FT = F // 128
    NJ = 3
    GP = 2
    NG = NC // GP
    GI = GP * DP // (16 * NJ)
    PI = GI // GP
    HI = PI // 2
    PT = DP // 16
    NS = 4
    IA = GI // 2
    qscale = float(Dh) ** -0.5 * _LOG2E

    perm = [(cfg["rot"] + n) % NC for n in range(NC)]
    ka = {perm[n]: int(c) for n, c in enumerate(cfg["ka"])}
    ra = {perm[n]: int(c) for n, c in enumerate(cfg["ra"])}
    bd = {perm[n]: int(c) for n, c in enumerate(cfg["bd"])}
    dpos = [n + int(c, 16) for n, c in enumerate(cfg["sd"])]
    nv = cfg["nv"]

    def slots(keys):
        return {key: n for n, key in enumerate(keys)}
    wqf_slot = slots((c, i) for c in range(NC) for i in range(DT - ka[c], DT))
    wof_slot = slots((c, i) for c in range(NC) for i in range(3 - bd[c], 3))
    wt_slot = slots([("q", c * 3 + i) for c in range(NC) for i in range(3 - ra[c], 3)]
                    + [(w, n) for n in range(FT - nv, FT) for w in "gu"])

    def chunk_pos(c, t):
        return c // GP, t % NJ, (c % GP) * PI + t // NJ

    def kernel(x_hbm, k_hbm, v_hbm, wq_hbm, wo_hbm, wr_hbm, wg_hbm, wu_hbm, wd_hbm,
               o_ref,
               kraw, vraw, kp, vf,
               wq_r, wo_r, wg_r, wu_r, wd_r,
               wq_p, wo_p, wg_p, wu_p, wd_p, wq_f, wo_f, wl_f, w_t,
               x_v, wr_v, xs_v, q1_v, p_v, rmo_v, rmd_v,
               ksem, vsem, lsem):

        def k_copies(b, g):
            s = g % NS
            return [pltpu.make_async_copy(
                k_hbm.at[b, g, :, j, :, pl.ds(Sk - W, W)], kraw.at[s, :, j],
                ksem.at[s]) for j in range(NJ)]

        def v_copies(b, g):
            s = g % NS
            return [pltpu.make_async_copy(
                v_hbm.at[b, g, :, j, :, pl.ds(Sk - W, W)], vraw.at[s, :, j],
                vsem.at[s]) for j in range(NJ)]

        def v_last_copies(b):
            g = NG - 1
            rng = [(j, 0, GI) for j in range(NJ - 1)] + [(NJ - 1, 0, IA), (NJ - 1, IA, GI - IA)]
            return [pltpu.make_async_copy(
                v_hbm.at[b, g, pl.ds(i0, n), j, :, pl.ds(Sk - W, W)],
                vraw.at[g % NS, pl.ds(i0, n), j], lsem.at[e])
                for e, (j, i0, n) in enumerate(rng)]

        def start_next(copies, b, g):
            n = b * NG + g + NS

            @pl.when(n < B * NG)
            def _():
                for cp in copies(n // NG, n % NG):
                    cp.start()

        w_sets = [
            [(wq_hbm, wq_r), (x_hbm, x_v), (wr_hbm, wr_v)],
            [(wo_hbm, wo_r)],
            [(wg_hbm, wg_r), (wu_hbm, wu_r), (wd_hbm, wd_r)],
        ]
        w_copies = [[pltpu.make_async_copy(src, dst, lsem.at[i]) for src, dst in ws]
                    for i, ws in enumerate(w_sets)]
        for ws in w_copies:
            for cp in ws:
                cp.start()

        def start0(g, _):
            for cp in k_copies(0, g) + v_copies(0, g):
                cp.start()
            return 0
        lax.fori_loop(0, NS, start0, 0)

        def repack(raw, packed, rows):
            def go(i, _):
                r = pl.multiple_of(i * rows, rows)
                r2 = pl.multiple_of(i * (rows // 2), rows // 2)
                packed[pl.ds(r2, rows // 2), :] = _pack(raw[pl.ds(r, rows), :])
                return 0
            lax.fori_loop(0, raw.shape[0] // rows, go, 0)

        def transpose_blocks(raw, name):
            keys = [key for key in wt_slot if key[0] == name]
            if keys:
                def go(i, _):
                    r = pl.multiple_of(i * 128, 128)
                    for key in keys:
                        blk = raw[pl.ds(r, 128), key[1] * 128:(key[1] + 1) * 128]
                        w_t[wt_slot[key], :, pl.ds(r, 128)] = blk.astype(_F32).T
                    return 0
                lax.fori_loop(0, DT, go, 0)

        def row_means(raw, dst):
            ones = jnp.ones((16, D), _BF16)

            def go(i, _):
                r = pl.multiple_of(i * 128, 128)
                dst[:, pl.ds(r, 128)] = _dot_t(ones, raw[pl.ds(r, 128), :])[0:8] * (1.0 / D)
                return 0
            lax.fori_loop(0, raw.shape[0] // 128, go, 0)

        def with_mean(rows):
            w = rows.astype(_F32)
            m = jnp.mean(w, axis=-1, keepdims=True)
            return jnp.concatenate([w, jnp.broadcast_to(m, (w.shape[0], 128))], axis=1)

        row16 = lax.broadcasted_iota(jnp.int32, (16, DP), 0)
        col16 = lax.broadcasted_iota(jnp.int32, (16, DP), 1)
        qmask = (row16 < 8) == (col16 < Dh)
        low_half = lax.broadcasted_iota(jnp.int32, (8, 128), 1) < 64

        def tile_d(m):
            return jnp.concatenate([m] * DT, axis=1)

        def lane_mean_part(x):
            return jnp.broadcast_to(jnp.sum(_lane_fold(x), axis=-1, keepdims=True), (8, 128))

        def scores(q16, kk):
            q = jnp.where(qmask, q16, 0.0).astype(_BF16)
            s0 = _dot(q[:, 0:128], kk[0:128])
            s1 = _dot(q[:, 128:256], kk[128:256])
            s2 = _dot(q[:, 256:384], kk[256:384])
            return s1 + jnp.concatenate([s0[0:8], s2[8:16]], axis=0)

        def probs(s):
            return jnp.exp2(s - jnp.max(s, axis=-1, keepdims=True))

        def inv_sum(p):
            return 1.0 / jnp.sum(p, axis=-1, keepdims=True)

        def pv_chunk(pp, vv):
            return _lane_fold(vv * jnp.concatenate([pp, pp], axis=0))

        def vpu_out(part, w):
            cc = jnp.sum(part, axis=1, keepdims=True) * w
            return cc[0:8] + cc[8:16]

        def vpu_cols(xc, key):
            parts = [_lane_fold(w_t[wt_slot[key], t * 8:(t + 1) * 8, :] * xc) for t in range(16)]
            return jnp.broadcast_to(_row_sums(parts), (8, 128))

        def ffn(x, m, wr):
            xc = x - tile_d(m)
            rstd = _rstd(xc)
            gate = jax.nn.sigmoid(jnp.sum(xc * wr, axis=-1, keepdims=True) * rstd)
            xb = _lhs(xc)
            hs = []
            for n0 in range(0, FT - nv, cfg["fgrp"]):
                n1 = min(FT - nv, n0 + cfg["fgrp"])
                g = _dot(xb, _unpack(wg_p[:, n0 * 128:n1 * 128]))[0:8] * rstd
                u = _dot(xb, _unpack(wu_p[:, n0 * 128:n1 * 128]))[0:8] * rstd
                hs.append((n0, n1, _lhs(g * jax.nn.sigmoid(g) * u)))
            for n in range(FT - nv, FT):
                g = vpu_cols(xc, ("g", n)) * rstd
                u = vpu_cols(xc, ("u", n)) * rstd
                hs.append((n, n + 1, _lhs(g * jax.nn.sigmoid(g) * u)))
            y = None
            for n0, n1, h in hs:
                d = _dot(h, _unpack(wd_p[n0 * 64:n1 * 64, :]))[0:8]
                y = d if y is None else y + d
            hall = jnp.concatenate([h[0:8].astype(_F32) for _, _, h in hs], axis=1)
            my = lane_mean_part(hall * rmd_v[...])
            return x + xc * rstd + y * gate, m + my * gate

        for cp in w_copies[0]:
            cp.wait()
        repack(wq_r, wq_p, 16)
        transpose_blocks(wq_r, "q")

        def wqf_go(t, _):
            for (c, i), n in wqf_slot.items():
                r = pl.multiple_of(i * 128 + t * 16, 16)
                wq_f[n, pl.ds(pl.multiple_of(t * 16, 16), 16), :] = (
                    wq_r[pl.ds(r, 16), c * DP:(c + 1) * DP].astype(_F32))
            return 0
        lax.fori_loop(0, 8, wqf_go, 0)

        xs_v[...] = jnp.zeros(xs_v.shape, _F32)
        xs_v[0:B, :] = x_v[...].astype(_F32)
        wr = wr_v[...].astype(_F32).reshape(1, D)
        xc0 = xs_v[...] - jnp.mean(xs_v[...], axis=-1, keepdims=True)
        qs0 = _rstd(xc0) * qscale
        xb0 = _lhs(xc0)

        def q1_go(c, _):
            col = pl.multiple_of(c * DP, 128)
            q1_v[:, pl.ds(col, DP)] = _dot(xb0, _unpack(wq_p[:, pl.ds(col, DP)]))[0:8] * qs0
            return 0
        lax.fori_loop(0, NC, q1_go, 0)

        for cp in w_copies[1]:
            cp.wait()

        def wo_go(n, _):
            g = n // GI
            i = n % GI
            for j in range(NJ):
                r = pl.multiple_of((n * NJ + j) * 16, 16)
                wo_p[g, j, pl.ds(pl.multiple_of(i * 8, 8), 8), :] = _pack(wo_r[pl.ds(r, 16), :])
            return 0
        lax.fori_loop(0, NG * GI, wo_go, 0)

        def wof_go(t, _):
            for (c, i), n in wof_slot.items():
                r = pl.multiple_of(c * DP + i * 128 + t * 16, 16)
                wo_f[n, pl.ds(pl.multiple_of(t * 16, 16), 16), :] = with_mean(wo_r[pl.ds(r, 16), :])
            return 0
        lax.fori_loop(0, 8, wof_go, 0)
        for i in range(IA, GI):
            r = (((NG - 1) * GI + i) * NJ + NJ - 1) * 16
            wl_f[i - IA] = with_mean(wo_r[r:r + 16, :])
        row_means(wo_r, rmo_v)

        for cp in w_copies[2]:
            cp.wait()
        repack(wg_r, wg_p, 64)
        repack(wu_r, wu_p, 64)
        repack(wd_r, wd_p, 128)
        transpose_blocks(wg_r, "g")
        transpose_blocks(wu_r, "u")
        row_means(wd_r, rmd_v)

        def attention3(x, m):
            xc = x - tile_d(m)
            qs8 = _rstd(xc) * qscale
            xb = _lhs(xc)
            xcol = {i: jnp.broadcast_to(xc[0:1, i * 128:(i + 1) * 128], (128, 128)).T
                    for i in range(DT - max(ka.values()), DT)}

            def stage_a(c):
                km = (DT - ka[c]) * 128
                nm = (3 - ra[c]) * 128
                q = None
                if km and nm:
                    q = _dot(xb[:, 0:km], _unpack(wq_p[0:km // 2, c * DP:c * DP + nm]))[0:8]
                if ka[c] and nm:
                    a = None
                    for i in range(DT - ka[c], DT):
                        for t in range(16):
                            xx = xcol[i][t * 8:(t + 1) * 8, :]
                            cc = (jnp.concatenate([xx] * (nm // 128), axis=1)
                                  * wq_f[wqf_slot[c, i], t * 8:(t + 1) * 8, 0:nm])
                            a = cc if a is None else a + cc
                    a = jnp.sum(a, axis=0, keepdims=True)
                    q = jnp.broadcast_to(a, (8, nm)) if q is None else q + a
                cols = [] if q is None else [q]
                cols += [vpu_cols(xc, ("q", c * 3 + i)) for i in range(3 - ra[c], 3)]
                return jnp.concatenate(cols, axis=1) * qs8

            def v_rows(c, t):
                g, j, i = chunk_pos(c, t)
                if g == NG - 1 and j == NJ - 1 and i >= IA:
                    return vraw[g % NS, i, j].astype(_F32)
                return vf[g, j, i]

            def stage_c(p, linv, c):
                nt = (3 - bd[c]) * 8
                head = lambda t: t // (PT // 2)
                chunk = lambda t: pv_chunk(p[head(t) * 8:head(t) * 8 + 8], v_rows(c, t))
                o = None
                if nt:
                    l0 = jnp.broadcast_to(linv[0:8], (8, 128))
                    l1 = jnp.broadcast_to(linv[8:16], (8, 128))
                    li = [l0, jnp.where(low_half, l0, l1), l1][0:nt // 8]
                    o = _lhs(_row_sums([chunk(t) for t in range(nt)])
                             * jnp.concatenate(li, axis=1))
                tot = None
                for hh in range(2):
                    a = None
                    for t in range(nt, PT):
                        if head(t) != hh:
                            continue
                        r = (t % 8) * 16
                        cc = vpu_out(chunk(t), wo_f[wof_slot[c, t // 8], r:r + 16, :])
                        a = cc if a is None else a + cc
                    if a is not None:
                        a = a * linv[hh * 8:hh * 8 + 8]
                        tot = a if tot is None else tot + a
                return o, tot

            def stage_d(o, c):
                ws = []
                for t in range(o.shape[1] // 16):
                    g, j, i = chunk_pos(c, t)
                    ws.append(wo_p[g, j, i * 8:(i + 1) * 8, :])
                mo = _lane_fold(o[0:8].astype(_F32) * rmo_v[:, c * DP:c * DP + o.shape[1]])
                return _dot(o, _unpack(jnp.concatenate(ws, axis=0)))[0:8], mo

            acc, accm, accv = x, None, None
            qs, ss, ps, ls, os_ = {}, {}, {}, {}, {}
            off = dict(A=cfg["SA"], B=cfg["SB"], M=cfg["SM"], S=cfg["SS"], C=0)
            for step in range(-cfg["SA"], max(dpos) + 1):
                for st in cfg["order"]:
                    if st == "D":
                        for n in range(NC):
                            if dpos[n] == step and os_[n] is not None:
                                d, mo = stage_d(os_[n], perm[n])
                                acc = acc + d
                                accm = mo if accm is None else accm + mo
                        continue
                    n = step + off[st]
                    if not 0 <= n < NC:
                        continue
                    c = perm[n]
                    if st == "A":
                        qs[n] = stage_a(c)
                    elif st == "B":
                        ss[n] = scores(jnp.concatenate([qs[n], qs[n]], axis=0), _unpack(kp[c]))
                    elif st == "M":
                        ps[n] = probs(ss[n])
                    elif st == "S":
                        ls[n] = inv_sum(ps[n])
                    elif st == "C":
                        os_[n], part = stage_c(ps[n], ls[n], c)
                        if part is not None:
                            accv = part if accv is None else accv + part
            if accm is not None:
                m = m + lane_mean_part(accm)
            if accv is not None:
                accv = jnp.sum(accv, axis=0, keepdims=True)
                acc = acc + accv[:, 0:D]
                m = m + accv[:, D:]
            return acc, m

        def batch(b, _):
            def group_probs(g, s, static):
                for cp in k_copies(b, g):
                    cp.wait()
                linvs = []
                for i in range(GP):
                    c = g * GP + i
                    col = c * DP if static else pl.multiple_of(c * DP, 128)
                    q16 = jnp.broadcast_to(q1_v[pl.ds(b, 1), pl.ds(col, DP)], (16, DP))
                    kk = kraw[s, i * PI:(i + 1) * PI].reshape(DP, W)
                    kp[c] = _pack(kk)
                    p = probs(scores(q16, kk))
                    p_v[i] = p
                    linvs.append(inv_sum(p))
                start_next(k_copies, b, g)
                return linvs

            def head_probs(i):
                h = i // HI
                return p_v[h // 2, (h % 2) * 8:(h % 2) * 8 + 8, :]

            def piece(g, s, j, n, linvs):
                parts = []
                for i in range(n):
                    vv = vraw[s, i, j].astype(_F32)
                    vf[g, j, i] = vv
                    parts.append(pv_chunk(head_probs(i), vv))
                li = [jnp.where(low_half, l[0:8], l[8:16]) for l in linvs][0:n // PI]
                o = _lhs(_row_sums(parts) * jnp.concatenate(li, axis=1))
                return _dot(o, _unpack(wo_p[g, j, 0:n * 8, :]))[0:8]

            def group(g, acc):
                s = g % NS
                linvs = group_probs(g, s, False)
                for cp in v_copies(b, g):
                    cp.wait()
                for j in range(NJ):
                    acc = acc + piece(g, s, j, GI, linvs)

                @pl.when(g == NG - 1 - NS)
                def _():
                    for cp in v_last_copies(b):
                        cp.start()

                @pl.when(g != NG - 1 - NS)
                def _():
                    start_next(v_copies, b, g)
                return acc

            x = lax.fori_loop(0, NG - 1, group, jnp.broadcast_to(xs_v[pl.ds(b, 1), :], (8, D)))
            g = NG - 1
            s = g % NS
            linvs = group_probs(g, s, True)
            vcs = v_last_copies(b)
            for j in range(NJ):
                vcs[j].wait()
                x = x + piece(g, s, j, GI if j < NJ - 1 else IA, linvs)
            m = lane_mean_part(x) * (1.0 / D)
            vcs[NJ].wait()
            tot = None
            for h in range(IA // HI, GI // HI):
                a = None
                for i in range(h * HI, (h + 1) * HI):
                    part = pv_chunk(head_probs(i), vraw[s, i, NJ - 1].astype(_F32))
                    cc = vpu_out(part, wl_f[i - IA])
                    a = cc if a is None else a + cc
                a = a * linvs[h // 2][(h % 2) * 8:(h % 2) * 8 + 8]
                tot = a if tot is None else tot + a
            tot = jnp.sum(tot, axis=0, keepdims=True)
            x = x + tot[:, 0:D]
            m = m + tot[:, D:]

            x, m = ffn(x, m, wr)
            x, m = attention3(x, m)
            x, _ = ffn(x, m, wr)
            xs_v[pl.ds(b, 1), :] = x[0:1, :]
            start_next(v_copies, b, NG - 1)
            return 0

        lax.fori_loop(0, B, batch, 0)
        o_ref[...] = xs_v[0:B, :].astype(o_ref.dtype)

    any_spec = pl.BlockSpec(memory_space=pl.ANY)
    out = pl.pallas_call(
        kernel,
        in_specs=[any_spec] * 9,
        out_specs=pl.BlockSpec(memory_space=pltpu.VMEM),
        out_shape=jax.ShapeDtypeStruct((B, D), A_x.dtype),
        scratch_shapes=[
            pltpu.VMEM((NS, GI, NJ, 16, W), _BF16),
            pltpu.VMEM((NS, GI, NJ, 16, W), _BF16),
            pltpu.VMEM((NC, DP // 2, W), _U32),
            pltpu.VMEM((NG, NJ, GI, 16, W), _F32),
            pltpu.VMEM((D, H * Dh), _BF16),
            pltpu.VMEM((H * Dh, D), _BF16),
            pltpu.VMEM((D, F), _BF16),
            pltpu.VMEM((D, F), _BF16),
            pltpu.VMEM((F, D), _BF16),
            pltpu.VMEM((D // 2, H * Dh), _U32),
            pltpu.VMEM((NG, NJ, GI * 8, D), _U32),
            pltpu.VMEM((D // 2, F), _U32),
            pltpu.VMEM((D // 2, F), _U32),
            pltpu.VMEM((F // 2, D), _U32),
            pltpu.VMEM((max(len(wqf_slot), 1), 128, DP), _F32),
            pltpu.VMEM((max(len(wof_slot), 1), 128, D + 128), _F32),
            pltpu.VMEM((GI - IA, 16, D + 128), _F32),
            pltpu.VMEM((max(len(wt_slot), 1), 128, D), _F32),
            pltpu.VMEM((B, D), _BF16),
            pltpu.VMEM((D,), _BF16),
            pltpu.VMEM((8, D), _F32),
            pltpu.VMEM((8, H * Dh), _F32),
            pltpu.VMEM((GP, 16, W), _F32),
            pltpu.VMEM((8, H * Dh), _F32),
            pltpu.VMEM((8, F), _F32),
            pltpu.SemaphoreType.DMA((NS,)),
            pltpu.SemaphoreType.DMA((NS,)),
            pltpu.SemaphoreType.DMA((NJ + 1,)),
        ],
        compiler_params=_compiler_params(),
    )(
        A_x.reshape(B, D),
        jnp.swapaxes(A_k_cache, 2, 3).reshape(B, NG, GI, NJ, 16, Sk),
        jnp.swapaxes(A_v_cache, 2, 3).reshape(B, NG, GI, NJ, 16, Sk),
        A_wq, A_wo, B_w_r, B_w_gate, B_w_up, B_w_down,
    )
    return out.reshape(B, Sq, D)


@jax.jit
def pallas_interleave_layers__sliding_block_cached__moe_arch_mod__decode_kernel(
    A_x: jax.Array,
    A_k_cache: jax.Array,
    A_v_cache: jax.Array,
    A_wq: jax.Array,
    A_wo: jax.Array,
    B_x: jax.Array,
    B_w_r: jax.Array,
    B_w_gate: jax.Array,
    B_w_up: jax.Array,
    B_w_down: jax.Array,
):
    return _forward(_CFG, A_x, A_k_cache, A_v_cache, A_wq, A_wo,
                    B_w_r, B_w_gate, B_w_up, B_w_down)
```

```python
import jax
import jax.numpy as jnp
from jax import lax
import jax.experimental.pallas as pl
import jax.experimental.pallas.tpu as pltpu

_F32 = jnp.float32
_BF16 = jnp.bfloat16
_U32 = jnp.uint32
_LOG2E = 1.4426950408889634

_CFG = dict(
    SA=5, SB=2, SM=1, SS=0, order="MSCABD",
    rot=13,
    ka="0122211111111111",
    ra="0000000000000000",
    bd="2111121111111113",
    sd="3211141111121123",
    cuts=(0, 8, 11, 16),
    nv=6, fgrp=2,
)


def _pack(x):
    return pltpu.bitcast(x, _U32)


def _unpack(x):
    return pltpu.bitcast(x, _BF16)


def _dot(a, b):
    return jnp.dot(a, b, preferred_element_type=_F32)


def _dot_t(a, b):
    return lax.dot_general(a, b, (((1,), (1,)), ((), ())), preferred_element_type=_F32)


def _lhs(x8):
    return jnp.concatenate([x8, x8], axis=0).astype(_BF16)


def _lane_fold(x):
    a = x[:, 0:128]
    for j in range(1, x.shape[1] // 128):
        a = a + x[:, j * 128:(j + 1) * 128]
    return a


def _row_sums(parts):
    return jnp.sum(jnp.concatenate(parts, axis=0).T, axis=0, keepdims=True)


def _sigmoid(x):
    return 0.5 * jnp.tanh(0.5 * x) + 0.5


def _rstd(xc):
    return lax.rsqrt(jnp.mean(xc * xc, axis=-1, keepdims=True) + 1e-5)


def _compiler_params():
    limit = 120 * 1024 * 1024
    try:
        return pltpu.CompilerParams(vmem_limit_bytes=limit, disable_semaphore_checks=True)
    except TypeError:
        return pltpu.CompilerParams(vmem_limit_bytes=limit)


def _forward(cfg, A_x, A_k_cache, A_v_cache, A_wq, A_wo, B_w_r, B_w_gate, B_w_up, B_w_down):
    B, Sq, D = A_x.shape
    _, H, Sk, Dh = A_k_cache.shape
    F = B_w_gate.shape[1]
    W = min(4096, max(256, Sk // 4))
    assert Sq == 1 and H == 32 and Dh == 192 and B <= 8 and D % 128 == 0 and F % 128 == 0
    DP = 2 * Dh
    NC = H // 2
    DT = D // 128
    FT = F // 128
    NJ = 3
    GP = 2
    NG = NC // GP
    GI = GP * DP // (16 * NJ)
    PI = GI // GP
    HI = PI // 2
    PT = DP // 16
    NS = 4
    cuts = cfg["cuts"]
    IA = cuts[-2]
    last_parts = [(j, 0, GI) for j in range(NJ - 1)]
    last_parts += [(NJ - 1, i0, i1) for i0, i1 in zip(cuts[:-1], cuts[1:])]
    qscale = float(Dh) ** -0.5 * _LOG2E

    perm = [(cfg["rot"] + n) % NC for n in range(NC)]
    ka = {perm[n]: int(c) for n, c in enumerate(cfg["ka"])}
    ra = {perm[n]: int(c) for n, c in enumerate(cfg["ra"])}
    bd = {perm[n]: int(c) for n, c in enumerate(cfg["bd"])}
    dpos = [n + int(c, 16) for n, c in enumerate(cfg["sd"])]
    nv = cfg["nv"]

    def slots(keys):
        return {key: n for n, key in enumerate(keys)}
    wqf_slot = slots((c, i) for c in range(NC) for i in range(DT - ka[c], DT))
    wof_slot = slots((c, i) for c in range(NC) for i in range(3 - bd[c], 3))
    wt_slot = slots([("q", c * 3 + i) for c in range(NC) for i in range(3 - ra[c], 3)]
                    + [(w, n) for n in range(FT - nv, FT) for w in "gu"])

    def chunk_pos(c, t):
        return c // GP, t % NJ, (c % GP) * PI + t // NJ

    def kernel(x_hbm, k_hbm, v_hbm, wq_hbm, wo_hbm, wr_hbm, wg_hbm, wu_hbm, wd_hbm,
               o_ref,
               kraw, vraw, kp, vf,
               wq_r, wo_r, wg_r, wu_r, wd_r,
               wq_p, wo_p, wg_p, wu_p, wd_p, wq_f, wo_f, wl_f, w_t,
               x_v, wr_v, xs_v, q1_v, p_v, rmo_v, rmd_v,
               ksem, vsem, lsem):

        def k_copies(b, g):
            s = g % NS
            return [pltpu.make_async_copy(
                k_hbm.at[b, g, :, j, :, pl.ds(Sk - W, W)], kraw.at[s, :, j],
                ksem.at[s]) for j in range(NJ)]

        def v_copies(b, g):
            s = g % NS
            return [pltpu.make_async_copy(
                v_hbm.at[b, g, :, j, :, pl.ds(Sk - W, W)], vraw.at[s, :, j],
                vsem.at[s]) for j in range(NJ)]

        def v_last_copies(b):
            g = NG - 1
            return [pltpu.make_async_copy(
                v_hbm.at[b, g, pl.ds(i0, i1 - i0), j, :, pl.ds(Sk - W, W)],
                vraw.at[g % NS, pl.ds(i0, i1 - i0), j], lsem.at[e])
                for e, (j, i0, i1) in enumerate(last_parts)]

        def start_next(copies, b, g):
            n = b * NG + g + NS

            @pl.when(n < B * NG)
            def _():
                for cp in copies(n // NG, n % NG):
                    cp.start()

        w_sets = [
            [(wq_hbm, wq_r), (x_hbm, x_v), (wr_hbm, wr_v)],
            [(wo_hbm, wo_r)],
            [(wg_hbm, wg_r), (wu_hbm, wu_r), (wd_hbm, wd_r)],
        ]
        w_copies = [[pltpu.make_async_copy(src, dst, lsem.at[i]) for src, dst in ws]
                    for i, ws in enumerate(w_sets)]
        for ws in w_copies:
            for cp in ws:
                cp.start()

        def start0(g, _):
            for cp in k_copies(0, g) + v_copies(0, g):
                cp.start()
            return 0
        lax.fori_loop(0, NS, start0, 0)

        def repack(raw, packed, rows):
            def go(i, _):
                r = pl.multiple_of(i * rows, rows)
                r2 = pl.multiple_of(i * (rows // 2), rows // 2)
                packed[pl.ds(r2, rows // 2), :] = _pack(raw[pl.ds(r, rows), :])
                return 0
            lax.fori_loop(0, raw.shape[0] // rows, go, 0)

        def transpose_blocks(raw, name):
            keys = [key for key in wt_slot if key[0] == name]
            if keys:
                def go(i, _):
                    r = pl.multiple_of(i * 128, 128)
                    for key in keys:
                        blk = raw[pl.ds(r, 128), key[1] * 128:(key[1] + 1) * 128]
                        w_t[wt_slot[key], :, pl.ds(r, 128)] = blk.astype(_F32).T
                    return 0
                lax.fori_loop(0, DT, go, 0)

        def row_means(raw, dst):
            ones = jnp.ones((16, D), _BF16)

            def go(i, _):
                r = pl.multiple_of(i * 128, 128)
                dst[:, pl.ds(r, 128)] = _dot_t(ones, raw[pl.ds(r, 128), :])[0:8] * (1.0 / D)
                return 0
            lax.fori_loop(0, raw.shape[0] // 128, go, 0)

        def with_mean(rows):
            w = rows.astype(_F32)
            m = jnp.mean(w, axis=-1, keepdims=True)
            return jnp.concatenate([w, jnp.broadcast_to(m, (w.shape[0], 128))], axis=1)

        row16 = lax.broadcasted_iota(jnp.int32, (16, DP), 0)
        col16 = lax.broadcasted_iota(jnp.int32, (16, DP), 1)
        qmask = (row16 < 8) == (col16 < Dh)
        low_half = lax.broadcasted_iota(jnp.int32, (8, 128), 1) < 64

        def tile_d(m):
            return jnp.concatenate([m] * DT, axis=1)

        def lane_mean_part(x):
            return jnp.broadcast_to(jnp.sum(_lane_fold(x), axis=-1, keepdims=True), (8, 128))

        def scores(q16, kk):
            q = jnp.where(qmask, q16, 0.0).astype(_BF16)
            s0 = _dot(q[:, 0:128], kk[0:128])
            s1 = _dot(q[:, 128:256], kk[128:256])
            s2 = _dot(q[:, 256:384], kk[256:384])
            return s1 + jnp.concatenate([s0[0:8], s2[8:16]], axis=0)

        def probs(s):
            return jnp.exp2(s - jnp.max(s, axis=-1, keepdims=True))

        def inv_sum(p):
            return 1.0 / jnp.sum(p, axis=-1, keepdims=True)

        def pv_chunk(pp, vv):
            return _lane_fold(vv * jnp.concatenate([pp, pp], axis=0))

        def vpu_out(part, w):
            cc = jnp.sum(part, axis=1, keepdims=True) * w
            return cc[0:8] + cc[8:16]

        def vpu_cols(xc, key):
            parts = [_lane_fold(w_t[wt_slot[key], t * 8:(t + 1) * 8, :] * xc) for t in range(16)]
            return jnp.broadcast_to(_row_sums(parts), (8, 128))

        def ffn(x, m, wr):
            xc = x - tile_d(m)
            rstd = _rstd(xc)
            gate = _sigmoid(jnp.sum(xc * wr, axis=-1, keepdims=True) * rstd)
            xb = _lhs(xc)
            hs = []
            for n0 in range(0, FT - nv, cfg["fgrp"]):
                n1 = min(FT - nv, n0 + cfg["fgrp"])
                g = _dot(xb, _unpack(wg_p[:, n0 * 128:n1 * 128]))[0:8] * rstd
                u = _dot(xb, _unpack(wu_p[:, n0 * 128:n1 * 128]))[0:8] * rstd
                hs.append((n0, n1, _lhs(g * _sigmoid(g) * u)))
            for n in range(FT - nv, FT):
                g = vpu_cols(xc, ("g", n)) * rstd
                u = vpu_cols(xc, ("u", n)) * rstd
                hs.append((n, n + 1, _lhs(g * _sigmoid(g) * u)))
            y = None
            for n0, n1, h in hs:
                d = _dot(h, _unpack(wd_p[n0 * 64:n1 * 64, :]))[0:8]
                y = d if y is None else y + d
            hall = jnp.concatenate([h[0:8].astype(_F32) for _, _, h in hs], axis=1)
            my = lane_mean_part(hall * rmd_v[...])
            return x + xc * rstd + y * gate, m + my * gate

        for cp in w_copies[0]:
            cp.wait()
        repack(wq_r, wq_p, 16)
        transpose_blocks(wq_r, "q")

        def wqf_go(t, _):
            for (c, i), n in wqf_slot.items():
                r = pl.multiple_of(i * 128 + t * 16, 16)
                wq_f[n, pl.ds(pl.multiple_of(t * 16, 16), 16), :] = (
                    wq_r[pl.ds(r, 16), c * DP:(c + 1) * DP].astype(_F32))
            return 0
        lax.fori_loop(0, 8, wqf_go, 0)

        xs_v[...] = jnp.zeros(xs_v.shape, _F32)
        xs_v[0:B, :] = x_v[...].astype(_F32)
        wr = wr_v[...].astype(_F32).reshape(1, D)
        xc0 = xs_v[...] - jnp.mean(xs_v[...], axis=-1, keepdims=True)
        qs0 = _rstd(xc0) * qscale
        xb0 = _lhs(xc0)

        def q1_go(c, _):
            col = pl.multiple_of(c * DP, 128)
            q1_v[:, pl.ds(col, DP)] = _dot(xb0, _unpack(wq_p[:, pl.ds(col, DP)]))[0:8] * qs0
            return 0
        lax.fori_loop(0, NC, q1_go, 0)

        for cp in w_copies[1]:
            cp.wait()

        def wo_go(n, _):
            g = n // GI
            i = n % GI
            for j in range(NJ):
                r = pl.multiple_of((n * NJ + j) * 16, 16)
                wo_p[g, j, pl.ds(pl.multiple_of(i * 8, 8), 8), :] = _pack(wo_r[pl.ds(r, 16), :])
            return 0
        lax.fori_loop(0, NG * GI, wo_go, 0)

        def wof_go(t, _):
            for (c, i), n in wof_slot.items():
                r = pl.multiple_of(c * DP + i * 128 + t * 16, 16)
                wo_f[n, pl.ds(pl.multiple_of(t * 16, 16), 16), :] = with_mean(wo_r[pl.ds(r, 16), :])
            return 0
        lax.fori_loop(0, 8, wof_go, 0)

        def wlf_go(i, _):
            for j in range(NJ):
                r = pl.multiple_of((((NG - 1) * GI + i) * NJ + j) * 16, 16)
                wl_f[j, i] = with_mean(wo_r[pl.ds(r, 16), :])
            return 0
        lax.fori_loop(0, GI, wlf_go, 0)
        row_means(wo_r, rmo_v)

        for cp in w_copies[2]:
            cp.wait()
        repack(wg_r, wg_p, 64)
        repack(wu_r, wu_p, 64)
        repack(wd_r, wd_p, 128)
        transpose_blocks(wg_r, "g")
        transpose_blocks(wu_r, "u")
        row_means(wd_r, rmd_v)

        def attention3(x, m):
            xc = x - tile_d(m)
            qs8 = _rstd(xc) * qscale
            xb = _lhs(xc)
            xcol = {i: jnp.broadcast_to(xc[0:1, i * 128:(i + 1) * 128], (128, 128)).T
                    for i in range(DT - max(ka.values()), DT)}

            def stage_a(c):
                km = (DT - ka[c]) * 128
                nm = (3 - ra[c]) * 128
                q = None
                if km and nm:
                    q = _dot(xb[:, 0:km], _unpack(wq_p[0:km // 2, c * DP:c * DP + nm]))[0:8]
                if ka[c] and nm:
                    a = None
                    for i in range(DT - ka[c], DT):
                        for t in range(16):
                            xx = xcol[i][t * 8:(t + 1) * 8, :]
                            cc = (jnp.concatenate([xx] * (nm // 128), axis=1)
                                  * wq_f[wqf_slot[c, i], t * 8:(t + 1) * 8, 0:nm])
                            a = cc if a is None else a + cc
                    a = jnp.sum(a, axis=0, keepdims=True)
                    q = jnp.broadcast_to(a, (8, nm)) if q is None else q + a
                cols = [] if q is None else [q]
                cols += [vpu_cols(xc, ("q", c * 3 + i)) for i in range(3 - ra[c], 3)]
                return jnp.concatenate(cols, axis=1) * qs8

            def v_rows(c, t):
                g, j, i = chunk_pos(c, t)
                if g == NG - 1 and j == NJ - 1 and i >= IA:
                    return vraw[g % NS, i, j].astype(_F32)
                return vf[g, j, i]

            def stage_c(p, linv, c):
                nt = (3 - bd[c]) * 8
                head = lambda t: t // (PT // 2)
                chunk = lambda t: pv_chunk(p[head(t) * 8:head(t) * 8 + 8], v_rows(c, t))
                o = None
                if nt:
                    l0 = jnp.broadcast_to(linv[0:8], (8, 128))
                    l1 = jnp.broadcast_to(linv[8:16], (8, 128))
                    li = [l0, jnp.where(low_half, l0, l1), l1][0:nt // 8]
                    o = _lhs(_row_sums([chunk(t) for t in range(nt)])
                             * jnp.concatenate(li, axis=1))
                tot = None
                for hh in range(2):
                    a = None
                    for t in range(nt, PT):
                        if head(t) != hh:
                            continue
                        r = (t % 8) * 16
                        cc = vpu_out(chunk(t), wo_f[wof_slot[c, t // 8], r:r + 16, :])
                        a = cc if a is None else a + cc
                    if a is not None:
                        a = a * linv[hh * 8:hh * 8 + 8]
                        tot = a if tot is None else tot + a
                return o, tot

            def stage_d(o, c):
                ws = []
                for t in range(o.shape[1] // 16):
                    g, j, i = chunk_pos(c, t)
                    ws.append(wo_p[g, j, i * 8:(i + 1) * 8, :])
                mo = _lane_fold(o[0:8].astype(_F32) * rmo_v[:, c * DP:c * DP + o.shape[1]])
                return _dot(o, _unpack(jnp.concatenate(ws, axis=0)))[0:8], mo

            acc, accm, accv = x, None, None
            qs, ss, ps, ls, os_ = {}, {}, {}, {}, {}
            off = dict(A=cfg["SA"], B=cfg["SB"], M=cfg["SM"], S=cfg["SS"], C=0)
            for step in range(-cfg["SA"], max(dpos) + 1):
                for st in cfg["order"]:
                    if st == "D":
                        for n in range(NC):
                            if dpos[n] == step and os_[n] is not None:
                                d, mo = stage_d(os_[n], perm[n])
                                acc = acc + d
                                accm = mo if accm is None else accm + mo
                        continue
                    n = step + off[st]
                    if not 0 <= n < NC:
                        continue
                    c = perm[n]
                    if st == "A":
                        qs[n] = stage_a(c)
                    elif st == "B":
                        ss[n] = scores(jnp.concatenate([qs[n], qs[n]], axis=0), _unpack(kp[c]))
                    elif st == "M":
                        ps[n] = probs(ss[n])
                    elif st == "S":
                        ls[n] = inv_sum(ps[n])
                    elif st == "C":
                        os_[n], part = stage_c(ps[n], ls[n], c)
                        if part is not None:
                            accv = part if accv is None else accv + part
            if accm is not None:
                m = m + lane_mean_part(accm)
            if accv is not None:
                accv = jnp.sum(accv, axis=0, keepdims=True)
                acc = acc + accv[:, 0:D]
                m = m + accv[:, D:]
            return acc, m

        def batch(b, _):
            @pl.when(b > 0)
            def _():
                for cp in v_copies(b, (NG - 1 + NS) % NG):
                    cp.start()

            def group_probs(g, s, static):
                for cp in k_copies(b, g):
                    cp.wait()
                linvs = []
                for i in range(GP):
                    c = g * GP + i
                    col = c * DP if static else pl.multiple_of(c * DP, 128)
                    q16 = jnp.broadcast_to(q1_v[pl.ds(b, 1), pl.ds(col, DP)], (16, DP))
                    kk = kraw[s, i * PI:(i + 1) * PI].reshape(DP, W)
                    kp[c] = _pack(kk)
                    p = probs(scores(q16, kk))
                    p_v[i] = p
                    linvs.append(inv_sum(p))
                start_next(k_copies, b, g)
                return linvs

            def head_probs(i):
                h = i // HI
                return p_v[h // 2, (h % 2) * 8:(h % 2) * 8 + 8, :]

            def piece(g, s, j, linvs):
                parts = []
                for i in range(GI):
                    vv = vraw[s, i, j].astype(_F32)
                    vf[g, j, i] = vv
                    parts.append(pv_chunk(head_probs(i), vv))
                li = [jnp.where(low_half, l[0:8], l[8:16]) for l in linvs]
                o = _lhs(_row_sums(parts) * jnp.concatenate(li, axis=1))
                return _dot(o, _unpack(wo_p[g, j]))[0:8]

            def group(g, acc):
                s = g % NS
                linvs = group_probs(g, s, False)
                for cp in v_copies(b, g):
                    cp.wait()
                for j in range(NJ):
                    acc = acc + piece(g, s, j, linvs)

                @pl.when(g == NG - 1 - NS)
                def _():
                    for cp in v_last_copies(b):
                        cp.start()

                @pl.when(g != NG - 1 - NS)
                def _():
                    start_next(v_copies, b, g)
                return acc

            x = lax.fori_loop(0, NG - 1, group, jnp.broadcast_to(xs_v[pl.ds(b, 1), :], (8, D)))
            g = NG - 1
            s = g % NS
            m = lane_mean_part(x) * (1.0 / D)
            linvs = group_probs(g, s, True)
            tot = None
            for cp, (j, i0, i1) in zip(v_last_copies(b), last_parts):
                cp.wait()
                for h in range(GI // HI):
                    a = None
                    for i in range(max(i0, h * HI), min(i1, (h + 1) * HI)):
                        vv = vraw[s, i, j].astype(_F32)
                        if j < NJ - 1 or i < IA:
                            vf[g, j, i] = vv
                        cc = vpu_out(pv_chunk(head_probs(i), vv), wl_f[j, i])
                        a = cc if a is None else a + cc
                    if a is not None:
                        a = a * linvs[h // 2][(h % 2) * 8:(h % 2) * 8 + 8]
                        tot = a if tot is None else tot + a
            tot = jnp.sum(tot, axis=0, keepdims=True)
            x = x + tot[:, 0:D]
            m = m + tot[:, D:]

            x, m = ffn(x, m, wr)
            x, m = attention3(x, m)
            x, _ = ffn(x, m, wr)
            xs_v[pl.ds(b, 1), :] = x[0:1, :]
            return 0

        lax.fori_loop(0, B, batch, 0)
        o_ref[...] = xs_v[0:B, :].astype(o_ref.dtype)

    any_spec = pl.BlockSpec(memory_space=pl.ANY)
    out = pl.pallas_call(
        kernel,
        in_specs=[any_spec] * 9,
        out_specs=pl.BlockSpec(memory_space=pltpu.VMEM),
        out_shape=jax.ShapeDtypeStruct((B, D), A_x.dtype),
        scratch_shapes=[
            pltpu.VMEM((NS, GI, NJ, 16, W), _BF16),
            pltpu.VMEM((NS, GI, NJ, 16, W), _BF16),
            pltpu.VMEM((NC, DP // 2, W), _U32),
            pltpu.VMEM((NG, NJ, GI, 16, W), _F32),
            pltpu.VMEM((D, H * Dh), _BF16),
            pltpu.VMEM((H * Dh, D), _BF16),
            pltpu.VMEM((D, F), _BF16),
            pltpu.VMEM((D, F), _BF16),
            pltpu.VMEM((F, D), _BF16),
            pltpu.VMEM((D // 2, H * Dh), _U32),
            pltpu.VMEM((NG, NJ, GI * 8, D), _U32),
            pltpu.VMEM((D // 2, F), _U32),
            pltpu.VMEM((D // 2, F), _U32),
            pltpu.VMEM((F // 2, D), _U32),
            pltpu.VMEM((max(len(wqf_slot), 1), 128, DP), _F32),
            pltpu.VMEM((max(len(wof_slot), 1), 128, D + 128), _F32),
            pltpu.VMEM((NJ, GI, 16, D + 128), _F32),
            pltpu.VMEM((max(len(wt_slot), 1), 128, D), _F32),
            pltpu.VMEM((B, D), _BF16),
            pltpu.VMEM((D,), _BF16),
            pltpu.VMEM((8, D), _F32),
            pltpu.VMEM((8, H * Dh), _F32),
            pltpu.VMEM((GP, 16, W), _F32),
            pltpu.VMEM((8, H * Dh), _F32),
            pltpu.VMEM((8, F), _F32),
            pltpu.SemaphoreType.DMA((NS,)),
            pltpu.SemaphoreType.DMA((NS,)),
            pltpu.SemaphoreType.DMA((len(last_parts),)),
        ],
        compiler_params=_compiler_params(),
    )(
        A_x.reshape(B, D),
        jnp.swapaxes(A_k_cache, 2, 3).reshape(B, NG, GI, NJ, 16, Sk),
        jnp.swapaxes(A_v_cache, 2, 3).reshape(B, NG, GI, NJ, 16, Sk),
        A_wq, A_wo, B_w_r, B_w_gate, B_w_up, B_w_down,
    )
    return out.reshape(B, Sq, D)


@jax.jit
def pallas_interleave_layers__sliding_block_cached__moe_arch_mod__decode_kernel(
    A_x: jax.Array,
    A_k_cache: jax.Array,
    A_v_cache: jax.Array,
    A_wq: jax.Array,
    A_wo: jax.Array,
    B_x: jax.Array,
    B_w_r: jax.Array,
    B_w_gate: jax.Array,
    B_w_up: jax.Array,
    B_w_down: jax.Array,
):
    return _forward(_CFG, A_x, A_k_cache, A_v_cache, A_wq, A_wo,
                    B_w_r, B_w_gate, B_w_up, B_w_down)
```

```python
import jax
import jax.numpy as jnp
from jax import lax
import jax.experimental.pallas as pl
import jax.experimental.pallas.tpu as pltpu

_F32 = jnp.float32
_BF16 = jnp.bfloat16
_U32 = jnp.uint32
_LOG2E = 1.4426950408889634

_CFG = dict(
    SA=5, SB=2, SM=1, SS=0, order="MSCABD",
    rot=13,
    ka="0122211111111111",
    ra="0000000000000000",
    bd="2111121111111113",
    sd="3211141111121123",
    LM=1,
    LT=0, LV=0, LA="",
    NJ=6,
    cuts=(0, 3, 8),
    nv=6, fgrp=2,
)


def _pack(x):
    return pltpu.bitcast(x, _U32)


def _unpack(x):
    return pltpu.bitcast(x, _BF16)


def _dot(a, b):
    return jnp.dot(a, b, preferred_element_type=_F32)


def _dot_t(a, b):
    return lax.dot_general(a, b, (((1,), (1,)), ((), ())), preferred_element_type=_F32)


def _lhs(x8):
    return jnp.concatenate([x8, x8], axis=0).astype(_BF16)


def _lane_fold(x):
    a = x[:, 0:128]
    for j in range(1, x.shape[1] // 128):
        a = a + x[:, j * 128:(j + 1) * 128]
    return a


def _row_sums(parts):
    return jnp.sum(jnp.concatenate(parts, axis=0).T, axis=0, keepdims=True)


def _row_sums8(parts):
    t = jnp.concatenate(parts, axis=0).T
    a = t[0:8]
    for i in range(1, 16):
        a = a + t[i * 8:(i + 1) * 8]
    return a


def _sigmoid(x):
    return 0.5 * jnp.tanh(0.5 * x) + 0.5


def _rstd(xc):
    return lax.rsqrt(jnp.mean(xc * xc, axis=-1, keepdims=True) + 1e-5)


def _compiler_params():
    limit = 120 * 1024 * 1024
    try:
        return pltpu.CompilerParams(vmem_limit_bytes=limit, disable_semaphore_checks=True)
    except TypeError:
        return pltpu.CompilerParams(vmem_limit_bytes=limit)


def _forward(cfg, A_x, A_k_cache, A_v_cache, A_wq, A_wo, B_w_r, B_w_gate, B_w_up, B_w_down):
    B, Sq, D = A_x.shape
    _, H, Sk, Dh = A_k_cache.shape
    F = B_w_gate.shape[1]
    W = min(4096, max(256, Sk // 4))
    assert Sq == 1 and H == 32 and Dh == 192 and B <= 8 and D % 128 == 0 and F % 128 == 0
    DP = 2 * Dh
    NC = H // 2
    DT = D // 128
    FT = F // 128
    NJ = cfg["NJ"]
    GP = 2
    NG = NC // GP
    GI = GP * DP // (16 * NJ)
    PI = GI // GP
    HI = PI // 2
    PT = DP // 16
    NS = 4
    cuts = cfg["cuts"]
    IA = cuts[-2]
    last_parts = [(j, 0, GI) for j in range(NJ - 1)]
    last_parts += [(NJ - 1, i0, i1) for i0, i1 in zip(cuts[:-1], cuts[1:])]
    qscale = float(Dh) ** -0.5 * _LOG2E

    perm = [(cfg["rot"] + n) % NC for n in range(NC)]
    ka = {perm[n]: int(c) for n, c in enumerate(cfg["ka"])}
    ra = {perm[n]: int(c) for n, c in enumerate(cfg["ra"])}
    bd = {perm[n]: int(c) for n, c in enumerate(cfg["bd"])}
    dpos = [n + int(c, 16) for n, c in enumerate(cfg["sd"])]
    nv = cfg["nv"]

    def slots(keys):
        return {key: n for n, key in enumerate(keys)}
    wqf_slot = slots((c, i) for c in range(NC) for i in range(DT - ka[c], DT))
    wof_slot = slots((c, i) for c in range(NC) for i in range(3 - bd[c], 3))
    wt_slot = slots([("q", c * 3 + i) for c in range(NC) for i in range(3 - ra[c], 3)]
                    + [(w, n) for n in range(FT - nv, FT) for w in "gu"])

    def chunk_pos(c, t):
        return c // GP, t % NJ, (c % GP) * PI + t // NJ

    def kernel(x_hbm, k_hbm, v_hbm, wq_hbm, wo_hbm, wr_hbm, wg_hbm, wu_hbm, wd_hbm,
               o_ref,
               kraw, vraw, kp, vf,
               wq_r, wo_r, wg_r, wu_r, wd_r,
               wq_p, wo_p, wg_p, wu_p, wd_p, wq_f, wo_f, wl_f, w_t,
               x_v, wr_v, xs_v, q1_v, p_v, rmo_v, rmd_v,
               ksem, vsem, lsem):

        def k_copies(b, g):
            s = g % NS
            return [pltpu.make_async_copy(
                k_hbm.at[b, g, :, j, :, pl.ds(Sk - W, W)], kraw.at[s, :, j],
                ksem.at[s]) for j in range(NJ)]

        def v_copies(b, g):
            s = g % NS
            return [pltpu.make_async_copy(
                v_hbm.at[b, g, :, j, :, pl.ds(Sk - W, W)], vraw.at[s, :, j],
                vsem.at[s]) for j in range(NJ)]

        def v_last_copies(b):
            g = NG - 1
            return [pltpu.make_async_copy(
                v_hbm.at[b, g, pl.ds(i0, i1 - i0), j, :, pl.ds(Sk - W, W)],
                vraw.at[g % NS, pl.ds(i0, i1 - i0), j], lsem.at[e])
                for e, (j, i0, i1) in enumerate(last_parts)]

        def start_next(copies, b, g):
            n = b * NG + g + NS

            @pl.when(n < B * NG)
            def _():
                for cp in copies(n // NG, n % NG):
                    cp.start()

        w_sets = [
            [(wq_hbm, wq_r), (x_hbm, x_v), (wr_hbm, wr_v)],
            [(wo_hbm, wo_r)],
            [(wg_hbm, wg_r), (wu_hbm, wu_r), (wd_hbm, wd_r)],
        ]
        w_copies = [[pltpu.make_async_copy(src, dst, lsem.at[i]) for src, dst in ws]
                    for i, ws in enumerate(w_sets)]
        for ws in w_copies:
            for cp in ws:
                cp.start()

        def start0(g, _):
            for cp in k_copies(0, g) + v_copies(0, g):
                cp.start()
            return 0
        lax.fori_loop(0, NS, start0, 0)

        def repack(raw, packed, rows):
            def go(i, _):
                r = pl.multiple_of(i * rows, rows)
                r2 = pl.multiple_of(i * (rows // 2), rows // 2)
                packed[pl.ds(r2, rows // 2), :] = _pack(raw[pl.ds(r, rows), :])
                return 0
            lax.fori_loop(0, raw.shape[0] // rows, go, 0)

        def transpose_blocks(raw, name):
            keys = [key for key in wt_slot if key[0] == name]
            if keys:
                def go(i, _):
                    r = pl.multiple_of(i * 128, 128)
                    for key in keys:
                        blk = raw[pl.ds(r, 128), key[1] * 128:(key[1] + 1) * 128]
                        w_t[wt_slot[key], :, pl.ds(r, 128)] = blk.astype(_F32).T
                    return 0
                lax.fori_loop(0, DT, go, 0)

        def row_means(raw, dst):
            ones = jnp.ones((16, D), _BF16)

            def go(i, _):
                r = pl.multiple_of(i * 128, 128)
                dst[:, pl.ds(r, 128)] = _dot_t(ones, raw[pl.ds(r, 128), :])[0:8] * (1.0 / D)
                return 0
            lax.fori_loop(0, raw.shape[0] // 128, go, 0)

        def with_mean(rows):
            w = rows.astype(_F32)
            m = jnp.mean(w, axis=-1, keepdims=True)
            return jnp.concatenate([w, jnp.broadcast_to(m, (w.shape[0], 128))], axis=1)

        row16 = lax.broadcasted_iota(jnp.int32, (16, DP), 0)
        col16 = lax.broadcasted_iota(jnp.int32, (16, DP), 1)
        qmask = (row16 < 8) == (col16 < Dh)
        low_half = lax.broadcasted_iota(jnp.int32, (8, 128), 1) < 64

        def tile_d(m):
            return jnp.concatenate([m] * DT, axis=1)

        def lane_mean_part(x):
            return jnp.broadcast_to(jnp.sum(_lane_fold(x), axis=-1, keepdims=True), (8, 128))

        def scores(q16, kk):
            q = jnp.where(qmask, q16, 0.0).astype(_BF16)
            s0 = _dot(q[:, 0:128], kk[0:128])
            s1 = _dot(q[:, 128:256], kk[128:256])
            s2 = _dot(q[:, 256:384], kk[256:384])
            return s1 + jnp.concatenate([s0[0:8], s2[8:16]], axis=0)

        def after(x, deps):
            for d in deps:
                d = _lane_fold(d)
                x = jnp.where(d != d, d, x)
            return x

        def probs(s, deps=()):
            pm = s[:, 0:128]
            for j in range(1, s.shape[1] // 128):
                pm = jnp.maximum(pm, s[:, j * 128:(j + 1) * 128])
            pm = jnp.concatenate([after(pm[0:8], deps), pm[8:16]], axis=0)
            return jnp.exp2(s - jnp.max(pm, axis=-1, keepdims=True))

        def inv_sum(p):
            l = jnp.sum(p, axis=-1, keepdims=True)
            r = pl.reciprocal(l, approx=True)
            return r * (2.0 - l * r)

        def pv_chunk(pp, vv):
            return _lane_fold(vv * jnp.concatenate([pp, pp], axis=0))

        def vpu_out(part, w):
            cc = jnp.sum(part, axis=1, keepdims=True) * w
            return cc[0:8] + cc[8:16]

        def vpu_cols(xc, key):
            parts = [_lane_fold(w_t[wt_slot[key], t * 8:(t + 1) * 8, :] * xc) for t in range(16)]
            return jnp.broadcast_to(_row_sums(parts), (8, 128))

        def ffn(x, m, wr):
            xc = x - tile_d(m)
            rstd = _rstd(xc)
            gate = _sigmoid(jnp.sum(xc * wr, axis=-1, keepdims=True) * rstd)
            xb = _lhs(xc)
            hs = []
            for n0 in range(0, FT - nv, cfg["fgrp"]):
                n1 = min(FT - nv, n0 + cfg["fgrp"])
                g = _dot(xb, _unpack(wg_p[:, n0 * 128:n1 * 128]))[0:8] * rstd
                u = _dot(xb, _unpack(wu_p[:, n0 * 128:n1 * 128]))[0:8] * rstd
                hs.append((n0, n1, _lhs(g * _sigmoid(g) * u)))
            for n in range(FT - nv, FT):
                g = vpu_cols(xc, ("g", n)) * rstd
                u = vpu_cols(xc, ("u", n)) * rstd
                hs.append((n, n + 1, _lhs(g * _sigmoid(g) * u)))
            y = None
            for n0, n1, h in hs:
                d = _dot(h, _unpack(wd_p[n0 * 64:n1 * 64, :]))[0:8]
                y = d if y is None else y + d
            hall = jnp.concatenate([h[0:8].astype(_F32) for _, _, h in hs], axis=1)
            my = lane_mean_part(hall * rmd_v[...])
            return x + xc * rstd + y * gate, m + my * gate

        for cp in w_copies[0]:
            cp.wait()
        repack(wq_r, wq_p, 16)
        transpose_blocks(wq_r, "q")

        def wqf_go(t, _):
            for (c, i), n in wqf_slot.items():
                r = pl.multiple_of(i * 128 + t * 16, 16)
                wq_f[n, pl.ds(pl.multiple_of(t * 16, 16), 16), :] = (
                    wq_r[pl.ds(r, 16), c * DP:(c + 1) * DP].astype(_F32))
            return 0
        lax.fori_loop(0, 8, wqf_go, 0)

        xs_v[...] = jnp.zeros(xs_v.shape, _F32)
        xs_v[0:B, :] = x_v[...].astype(_F32)
        wr = wr_v[...].astype(_F32).reshape(1, D)
        xc0 = xs_v[...] - jnp.mean(xs_v[...], axis=-1, keepdims=True)
        qs0 = _rstd(xc0) * qscale
        xb0 = _lhs(xc0)

        def q1_go(c, _):
            col = pl.multiple_of(c * DP, 128)
            q1_v[:, pl.ds(col, DP)] = _dot(xb0, _unpack(wq_p[:, pl.ds(col, DP)]))[0:8] * qs0
            return 0
        lax.fori_loop(0, NC, q1_go, 0)

        for cp in w_copies[1]:
            cp.wait()

        def wo_go(n, _):
            g = n // GI
            i = n % GI
            for j in range(NJ):
                r = pl.multiple_of((n * NJ + j) * 16, 16)
                wo_p[g, j, pl.ds(pl.multiple_of(i * 8, 8), 8), :] = _pack(wo_r[pl.ds(r, 16), :])
            return 0
        lax.fori_loop(0, NG * GI, wo_go, 0)

        def wof_go(t, _):
            for (c, i), n in wof_slot.items():
                r = pl.multiple_of(c * DP + i * 128 + t * 16, 16)
                wo_f[n, pl.ds(pl.multiple_of(t * 16, 16), 16), :] = with_mean(wo_r[pl.ds(r, 16), :])
            return 0
        lax.fori_loop(0, 8, wof_go, 0)

        def wlf_go(i, _):
            for j in range(NJ):
                r = pl.multiple_of((((NG - 1) * GI + i) * NJ + j) * 16, 16)
                wl_f[j, i] = with_mean(wo_r[pl.ds(r, 16), :])
            return 0
        lax.fori_loop(0, GI, wlf_go, 0)
        row_means(wo_r, rmo_v)

        for cp in w_copies[2]:
            cp.wait()
        repack(wg_r, wg_p, 64)
        repack(wu_r, wu_p, 64)
        repack(wd_r, wd_p, 128)
        transpose_blocks(wg_r, "g")
        transpose_blocks(wu_r, "u")
        row_means(wd_r, rmd_v)

        def attention3(x, m):
            xc = x - tile_d(m)
            qs8 = _rstd(xc) * qscale
            xb = _lhs(xc)
            xcol = {i: jnp.broadcast_to(xc[0:1, i * 128:(i + 1) * 128], (128, 128)).T
                    for i in range(DT - max(ka.values()), DT)}

            def stage_a(c):
                km = (DT - ka[c]) * 128
                nm = (3 - ra[c]) * 128
                q = None
                if km and nm:
                    q = _dot(xb[:, 0:km], _unpack(wq_p[0:km // 2, c * DP:c * DP + nm]))[0:8]
                if ka[c] and nm:
                    a = None
                    for i in range(DT - ka[c], DT):
                        for t in range(16):
                            xx = xcol[i][t * 8:(t + 1) * 8, :]
                            cc = (jnp.concatenate([xx] * (nm // 128), axis=1)
                                  * wq_f[wqf_slot[c, i], t * 8:(t + 1) * 8, 0:nm])
                            a = cc if a is None else a + cc
                    a = jnp.sum(a, axis=0, keepdims=True)
                    q = jnp.broadcast_to(a, (8, nm)) if q is None else q + a
                cols = [] if q is None else [q]
                cols += [vpu_cols(xc, ("q", c * 3 + i)) for i in range(3 - ra[c], 3)]
                return jnp.concatenate(cols, axis=1) * qs8

            def v_rows(c, t):
                g, j, i = chunk_pos(c, t)
                if g == NG - 1 and j == NJ - 1 and i >= IA:
                    return vraw[g % NS, i, j].astype(_F32)
                return vf[g, j, i]

            def stage_c(p, linv, c, wide):
                nt = (3 - bd[c]) * 8
                head = lambda t: t // (PT // 2)
                chunk = lambda t: pv_chunk(p[head(t) * 8:head(t) * 8 + 8], v_rows(c, t))
                o = mo = None
                if nt:
                    l0 = jnp.broadcast_to(linv[0:8], (8, 128))
                    l1 = jnp.broadcast_to(linv[8:16], (8, 128))
                    li = [l0, jnp.where(low_half, l0, l1), l1][0:nt // 8]
                    o = _lhs(_row_sums8([chunk(t) for t in range(nt)])
                             * jnp.concatenate(li, axis=1))
                    mo = _lane_fold(o[0:8].astype(_F32) * rmo_v[:, c * DP:c * DP + nt * 16])
                tot = None
                for hh in range(2):
                    a = None
                    for t in range(nt, PT):
                        if head(t) != hh:
                            continue
                        r = (t % 8) * 16
                        cc = vpu_out(chunk(t), wo_f[wof_slot[c, t // 8], r:r + 16, 0:wide])
                        a = cc if a is None else a + cc
                    if a is not None:
                        a = a * linv[hh * 8:hh * 8 + 8]
                        tot = a if tot is None else tot + a
                return o, mo, tot

            def stage_d(o, c):
                ws = []
                for t in range(o.shape[1] // 16):
                    g, j, i = chunk_pos(c, t)
                    ws.append(wo_p[g, j, i * 8:(i + 1) * 8, :])
                return _dot(o, _unpack(jnp.concatenate(ws, axis=0)))[0:8]

            acc, accm, accv, accw = None, None, None, None
            qs, ss, ps, ls, os_, mos, pvs = {}, {}, {}, {}, {}, {}, {}
            early = {int(a, 16): int(t, 16) for a, t in zip(cfg["LA"][0::2], cfg["LA"][1::2])}
            for n in early:
                qs[n] = stage_a(perm[n])
            off = dict(A=cfg["SA"], B=cfg["SB"], M=cfg["SM"], S=cfg["SS"], C=0)
            for step in range(-cfg["SA"], max(dpos) + 1):
                for st in cfg["order"]:
                    if st == "D":
                        for n in range(NC):
                            if dpos[n] == step and os_[n] is not None:
                                d = stage_d(os_[n], perm[n])
                                acc = d if acc is None else acc + d
                        continue
                    n = step + off[st]
                    if not 0 <= n < NC:
                        continue
                    c = perm[n]
                    if st == "A":
                        if n not in early:
                            qs[n] = stage_a(c)
                    elif st == "B":
                        ss[n] = scores(jnp.concatenate([qs[n], qs[n]], axis=0), _unpack(kp[c]))
                    elif st == "M":
                        deps = [qs[a] for a, t in early.items() if t == n]
                        if cfg["LT"] and mos.get(n - cfg["LT"]) is not None:
                            deps.append(mos[n - cfg["LT"]])
                        if cfg["LV"] and pvs.get(n - cfg["LV"]) is not None:
                            deps.append(pvs[n - cfg["LV"]])
                        ps[n] = probs(ss[n], deps)
                    elif st == "S":
                        ls[n] = inv_sum(ps[n])
                    elif st == "C":
                        late = n >= NC - cfg["LM"]
                        os_[n], mos[n], part = stage_c(ps[n], ls[n], c, D + 128 if late else D)
                        if mos[n] is not None:
                            accm = mos[n] if accm is None else accm + mos[n]
                        if part is not None and late:
                            accw = part if accw is None else accw + part
                        elif part is not None:
                            accv = part if accv is None else accv + part
                            pvs[n] = accv
            if accv is not None:
                mv = _lane_fold(accv) * (1.0 / D)
                accm = mv if accm is None else accm + mv
                acc = accv if acc is None else acc + accv
            tot = jnp.concatenate([acc, lane_mean_part(accm)], axis=1)
            if accw is not None:
                tot = tot + accw
            tot = jnp.sum(tot, axis=0, keepdims=True)
            return x + tot[:, 0:D], m + tot[:, D:]

        def batch(b, _):
            @pl.when(b > 0)
            def _():
                for cp in v_copies(b, (NG - 1 + NS) % NG):
                    cp.start()

            def group_probs(g, s, static):
                for cp in k_copies(b, g):
                    cp.wait()
                linvs = []
                for i in range(GP):
                    c = g * GP + i
                    col = c * DP if static else pl.multiple_of(c * DP, 128)
                    q16 = jnp.broadcast_to(q1_v[pl.ds(b, 1), pl.ds(col, DP)], (16, DP))
                    kk = kraw[s, i * PI:(i + 1) * PI].reshape(DP, W)
                    kp[c] = _pack(kk)
                    p = probs(scores(q16, kk))
                    p_v[i] = p
                    linvs.append(inv_sum(p))
                start_next(k_copies, b, g)
                return linvs

            def head_probs(i):
                h = i // HI
                return p_v[h // 2, (h % 2) * 8:(h % 2) * 8 + 8, :]

            def piece(g, s, j, li):
                parts = []
                for i in range(GI):
                    vv = vraw[s, i, j].astype(_F32)
                    vf[g, j, i] = vv
                    parts.append(pv_chunk(head_probs(i), vv))
                o = _lhs(_row_sums(parts) * li)
                return _dot(o, _unpack(wo_p[g, j]))[0:8]

            def group(g, acc):
                s = g % NS
                linvs = group_probs(g, s, False)
                lane = lax.broadcasted_iota(jnp.int32, (8, GI * 16), 1)
                li = jnp.broadcast_to(linvs[0][0:8], (8, GI * 16))
                for h in range(1, 2 * GP):
                    li = jnp.where(lane >= h * HI * 16,
                                   linvs[h // 2][(h % 2) * 8:(h % 2) * 8 + 8], li)
                for cp in v_copies(b, g):
                    cp.wait()
                for j in range(NJ):
                    acc = acc + piece(g, s, j, li)

                @pl.when(g == NG - 1 - NS)
                def _():
                    for cp in v_last_copies(b):
                        cp.start()

                @pl.when(g != NG - 1 - NS)
                def _():
                    start_next(v_copies, b, g)
                return acc

            x = lax.fori_loop(0, NG - 1, group, jnp.broadcast_to(xs_v[pl.ds(b, 1), :], (8, D)))
            g = NG - 1
            s = g % NS
            m = lane_mean_part(x) * (1.0 / D)
            linvs = group_probs(g, s, True)
            tot = None
            for cp, (j, i0, i1) in zip(v_last_copies(b), last_parts):
                cp.wait()
                for h in range(GI // HI):
                    a = None
                    for i in range(max(i0, h * HI), min(i1, (h + 1) * HI)):
                        vv = vraw[s, i, j].astype(_F32)
                        if j < NJ - 1 or i < IA:
                            vf[g, j, i] = vv
                        cc = vpu_out(pv_chunk(head_probs(i), vv), wl_f[j, i])
                        a = cc if a is None else a + cc
                    if a is not None:
                        a = a * linvs[h // 2][(h % 2) * 8:(h % 2) * 8 + 8]
                        tot = a if tot is None else tot + a
            tot = jnp.sum(tot, axis=0, keepdims=True)
            x = x + tot[:, 0:D]
            m = m + tot[:, D:]

            x, m = ffn(x, m, wr)
            x, m = attention3(x, m)
            x, _ = ffn(x, m, wr)
            xs_v[pl.ds(b, 1), :] = x[0:1, :]
            return 0

        lax.fori_loop(0, B, batch, 0)
        o_ref[...] = xs_v[0:B, :].astype(o_ref.dtype)

    any_spec = pl.BlockSpec(memory_space=pl.ANY)
    out = pl.pallas_call(
        kernel,
        in_specs=[any_spec] * 9,
        out_specs=pl.BlockSpec(memory_space=pltpu.VMEM),
        out_shape=jax.ShapeDtypeStruct((B, D), A_x.dtype),
        scratch_shapes=[
            pltpu.VMEM((NS, GI, NJ, 16, W), _BF16),
            pltpu.VMEM((NS, GI, NJ, 16, W), _BF16),
            pltpu.VMEM((NC, DP // 2, W), _U32),
            pltpu.VMEM((NG, NJ, GI, 16, W), _F32),
            pltpu.VMEM((D, H * Dh), _BF16),
            pltpu.VMEM((H * Dh, D), _BF16),
            pltpu.VMEM((D, F), _BF16),
            pltpu.VMEM((D, F), _BF16),
            pltpu.VMEM((F, D), _BF16),
            pltpu.VMEM((D // 2, H * Dh), _U32),
            pltpu.VMEM((NG, NJ, GI * 8, D), _U32),
            pltpu.VMEM((D // 2, F), _U32),
            pltpu.VMEM((D // 2, F), _U32),
            pltpu.VMEM((F // 2, D), _U32),
            pltpu.VMEM((max(len(wqf_slot), 1), 128, DP), _F32),
            pltpu.VMEM((max(len(wof_slot), 1), 128, D + 128), _F32),
            pltpu.VMEM((NJ, GI, 16, D + 128), _F32),
            pltpu.VMEM((max(len(wt_slot), 1), 128, D), _F32),
            pltpu.VMEM((B, D), _BF16),
            pltpu.VMEM((D,), _BF16),
            pltpu.VMEM((8, D), _F32),
            pltpu.VMEM((8, H * Dh), _F32),
            pltpu.VMEM((GP, 16, W), _F32),
            pltpu.VMEM((8, H * Dh), _F32),
            pltpu.VMEM((8, F), _F32),
            pltpu.SemaphoreType.DMA((NS,)),
            pltpu.SemaphoreType.DMA((NS,)),
            pltpu.SemaphoreType.DMA((len(last_parts),)),
        ],
        compiler_params=_compiler_params(),
    )(
        A_x.reshape(B, D),
        jnp.swapaxes(A_k_cache, 2, 3).reshape(B, NG, GI, NJ, 16, Sk),
        jnp.swapaxes(A_v_cache, 2, 3).reshape(B, NG, GI, NJ, 16, Sk),
        A_wq, A_wo, B_w_r, B_w_gate, B_w_up, B_w_down,
    )
    return out.reshape(B, Sq, D)


@jax.jit
def pallas_interleave_layers__sliding_block_cached__moe_arch_mod__decode_kernel(
    A_x: jax.Array,
    A_k_cache: jax.Array,
    A_v_cache: jax.Array,
    A_wq: jax.Array,
    A_wo: jax.Array,
    B_x: jax.Array,
    B_w_r: jax.Array,
    B_w_gate: jax.Array,
    B_w_up: jax.Array,
    B_w_down: jax.Array,
):
    return _forward(_CFG, A_x, A_k_cache, A_v_cache, A_wq, A_wo,
                    B_w_r, B_w_gate, B_w_up, B_w_down)
```

```python
import jax
import jax.numpy as jnp
from jax import lax
import jax.experimental.pallas as pl
import jax.experimental.pallas.tpu as pltpu

_F32 = jnp.float32
_BF16 = jnp.bfloat16
_U32 = jnp.uint32
_LOG2E = 1.4426950408889634

_CFG = dict(
    SA=5, SB=2, SM=1, SS=0, order="MSCABD",
    rot=13,
    ka="0122211111111111",
    ra="0000000000000000",
    bd="2111121111111113",
    sd="3211141111121123",
    LM=1,
    LS=0, LT=0, LV=0, L2=0, LA="",
    NJ=6,
    cuts=(0, 3, 8),
    ne=6, nv1=6,
    nv=6, fgrp=2,
)


def _pack(x):
    return pltpu.bitcast(x, _U32)


def _unpack(x):
    return pltpu.bitcast(x, _BF16)


def _dot(a, b):
    return jnp.dot(a, b, preferred_element_type=_F32)


def _dot_t(a, b):
    return lax.dot_general(a, b, (((1,), (1,)), ((), ())), preferred_element_type=_F32)


def _lhs(x8):
    return jnp.concatenate([x8, x8], axis=0).astype(_BF16)


def _lane_fold(x):
    a = x[:, 0:128]
    for j in range(1, x.shape[1] // 128):
        a = a + x[:, j * 128:(j + 1) * 128]
    return a


def _row_sums(parts):
    return jnp.sum(jnp.concatenate(parts, axis=0).T, axis=0, keepdims=True)


def _row_sums8(parts):
    t = jnp.concatenate(parts, axis=0).T
    a = t[0:8]
    for i in range(1, 16):
        a = a + t[i * 8:(i + 1) * 8]
    return a


def _sigmoid(x):
    return 0.5 * jnp.tanh(0.5 * x) + 0.5


def _rstd(xc):
    return lax.rsqrt(jnp.mean(xc * xc, axis=-1, keepdims=True) + 1e-5)


def _compiler_params():
    limit = 120 * 1024 * 1024
    try:
        return pltpu.CompilerParams(vmem_limit_bytes=limit, disable_semaphore_checks=True)
    except TypeError:
        return pltpu.CompilerParams(vmem_limit_bytes=limit)


def _forward(cfg, A_x, A_k_cache, A_v_cache, A_wq, A_wo, B_w_r, B_w_gate, B_w_up, B_w_down):
    B, Sq, D = A_x.shape
    _, H, Sk, Dh = A_k_cache.shape
    F = B_w_gate.shape[1]
    W = min(4096, max(256, Sk // 4))
    assert Sq == 1 and H == 32 and Dh == 192 and B <= 8 and D % 128 == 0 and F % 128 == 0
    DP = 2 * Dh
    NC = H // 2
    DT = D // 128
    FT = F // 128
    NJ = cfg["NJ"]
    GP = 2
    NG = NC // GP
    GI = GP * DP // (16 * NJ)
    PI = GI // GP
    HI = PI // 2
    PT = DP // 16
    NS = 4
    cuts = cfg["cuts"]
    IA = cuts[-2]
    last_parts = [(j, 0, GI) for j in range(NJ - 1)]
    last_parts += [(NJ - 1, i0, i1) for i0, i1 in zip(cuts[:-1], cuts[1:])]
    qscale = float(Dh) ** -0.5 * _LOG2E

    perm = [(cfg["rot"] + n) % NC for n in range(NC)]
    ka = {perm[n]: int(c) for n, c in enumerate(cfg["ka"])}
    ra = {perm[n]: int(c) for n, c in enumerate(cfg["ra"])}
    bd = {perm[n]: int(c) for n, c in enumerate(cfg["bd"])}
    dpos = [n + int(c, 16) for n, c in enumerate(cfg["sd"])]
    nv = cfg["nv"]
    nv1 = cfg["nv1"]
    FM1 = cfg["ne"] * 128

    def slots(keys):
        return {key: n for n, key in enumerate(keys)}
    wqf_slot = slots((c, i) for c in range(NC) for i in range(DT - ka[c], DT))
    wof_slot = slots((c, i) for c in range(NC) for i in range(3 - bd[c], 3))
    wt_slot = slots([("q", c * 3 + i) for c in range(NC) for i in range(3 - ra[c], 3)]
                    + [(w, n) for n in range(FT - max(nv, nv1), FT) for w in "gu"])

    def chunk_pos(c, t):
        return c // GP, t % NJ, (c % GP) * PI + t // NJ

    def kernel(x_hbm, k_hbm, v_hbm, wq_hbm, wo_hbm, wr_hbm, wg_hbm, wu_hbm, wd_hbm,
               o_ref,
               kraw, vraw, kp, vf,
               wq_r, wo_r, wg_r, wu_r, wd_r,
               wq_p, wo_p, wg_p, wu_p, wd_p, wq_f, wo_f, wl_f, wl2_f, w_t,
               x_v, wr_v, xs_v, q1_v, p_v, rmo_v, rmd_v,
               ksem, vsem, lsem):

        def k_copies(b, g):
            s = g % NS
            return [pltpu.make_async_copy(
                k_hbm.at[b, g, :, j, :, pl.ds(Sk - W, W)], kraw.at[s, :, j],
                ksem.at[s]) for j in range(NJ)]

        def v_copies(b, g):
            s = g % NS
            return [pltpu.make_async_copy(
                v_hbm.at[b, g, :, j, :, pl.ds(Sk - W, W)], vraw.at[s, :, j],
                vsem.at[s]) for j in range(NJ)]

        def v_last_copies(b):
            g = NG - 1
            return [pltpu.make_async_copy(
                v_hbm.at[b, g, pl.ds(i0, i1 - i0), j, :, pl.ds(Sk - W, W)],
                vraw.at[g % NS, pl.ds(i0, i1 - i0), j], lsem.at[e])
                for e, (j, i0, i1) in enumerate(last_parts)]

        def start_next(copies, b, g):
            n = b * NG + g + NS

            @pl.when(n < B * NG)
            def _():
                for cp in copies(n // NG, n % NG):
                    cp.start()

        w_sets = [
            [(wq_hbm, wq_r), (x_hbm, x_v), (wr_hbm, wr_v)],
            [(wo_hbm, wo_r)],
            [(wg_hbm, wg_r), (wu_hbm, wu_r), (wd_hbm, wd_r)],
        ]
        w_copies = [[pltpu.make_async_copy(src, dst, lsem.at[i]) for src, dst in ws]
                    for i, ws in enumerate(w_sets)]
        for ws in w_copies:
            for cp in ws:
                cp.start()

        def start0(g, _):
            for cp in k_copies(0, g) + v_copies(0, g):
                cp.start()
            return 0
        lax.fori_loop(0, NS, start0, 0)

        def repack(raw, packed, rows):
            def go(i, _):
                r = pl.multiple_of(i * rows, rows)
                r2 = pl.multiple_of(i * (rows // 2), rows // 2)
                packed[pl.ds(r2, rows // 2), :] = _pack(raw[pl.ds(r, rows), :])
                return 0
            lax.fori_loop(0, raw.shape[0] // rows, go, 0)

        def transpose_blocks(raw, name):
            keys = [key for key in wt_slot if key[0] == name]
            if keys:
                def go(i, _):
                    r = pl.multiple_of(i * 128, 128)
                    for key in keys:
                        blk = raw[pl.ds(r, 128), key[1] * 128:(key[1] + 1) * 128]
                        w_t[wt_slot[key], :, pl.ds(r, 128)] = blk.astype(_F32).T
                    return 0
                lax.fori_loop(0, DT, go, 0)

        def row_means(raw, dst):
            ones = jnp.ones((16, D), _BF16)

            def go(i, _):
                r = pl.multiple_of(i * 128, 128)
                dst[:, pl.ds(r, 128)] = _dot_t(ones, raw[pl.ds(r, 128), :])[0:8] * (1.0 / D)
                return 0
            lax.fori_loop(0, raw.shape[0] // 128, go, 0)

        def with_mean(rows):
            w = rows.astype(_F32)
            m = jnp.mean(w, axis=-1, keepdims=True)
            return jnp.concatenate([w, jnp.broadcast_to(m, (w.shape[0], 128))], axis=1)

        row16 = lax.broadcasted_iota(jnp.int32, (16, DP), 0)
        col16 = lax.broadcasted_iota(jnp.int32, (16, DP), 1)
        qmask = (row16 < 8) == (col16 < Dh)
        low_half = lax.broadcasted_iota(jnp.int32, (8, 128), 1) < 64

        def tile_d(m):
            return jnp.concatenate([m] * DT, axis=1)

        def lane_mean_part(x):
            return jnp.broadcast_to(jnp.sum(_lane_fold(x), axis=-1, keepdims=True), (8, 128))

        def scores(q16, kk):
            q = jnp.where(qmask, q16, 0.0).astype(_BF16)
            s0 = _dot(q[:, 0:128], kk[0:128])
            s1 = _dot(q[:, 128:256], kk[128:256])
            s2 = _dot(q[:, 256:384], kk[256:384])
            return s1 + jnp.concatenate([s0[0:8], s2[8:16]], axis=0)

        def after(x, deps):
            if not deps:
                return x
            d = _lane_fold(jnp.concatenate(list(deps), axis=1))
            d = jnp.concatenate([d] * (x.shape[0] // 8), axis=0)
            return jnp.where(d != d, d, x)

        def probs(s, deps=(), scale=None):
            pm = s[:, 0:128]
            for j in range(1, s.shape[1] // 128):
                pm = jnp.maximum(pm, s[:, j * 128:(j + 1) * 128])
            if cfg["L2"]:
                pm = after(pm, deps)
            else:
                pm = jnp.concatenate([after(pm[0:8], deps), pm[8:16]], axis=0)
            e = s - jnp.max(pm, axis=-1, keepdims=True)
            return jnp.exp2(e if scale is None else e * scale)

        def inv_sum(p):
            l = jnp.sum(p, axis=-1, keepdims=True)
            r = pl.reciprocal(l, approx=True)
            return r * (2.0 - l * r)

        def pv_chunk(pp, vv):
            return _lane_fold(vv * jnp.concatenate([pp, pp], axis=0))

        def vpu_out(part, w):
            cc = jnp.sum(part, axis=1, keepdims=True) * w
            return cc[0:8] + cc[8:16]

        def vpu_cols(xc, key):
            parts = [_lane_fold(w_t[wt_slot[key], t * 8:(t + 1) * 8, :] * xc) for t in range(16)]
            return jnp.broadcast_to(_row_sums(parts), (8, 128))

        def ffn(x, m, wr, nv, early=None):
            xc = x - tile_d(m)
            rstd = _rstd(xc)
            gate = _sigmoid(jnp.sum(xc * wr, axis=-1, keepdims=True) * rstd)
            xb = _lhs(xc if early is None else early[0])
            hs = []
            for n0 in range(0, FT - nv, cfg["fgrp"]):
                n1 = min(FT - nv, n0 + cfg["fgrp"])
                g = _dot(xb, _unpack(wg_p[:, n0 * 128:n1 * 128]))[0:8]
                u = _dot(xb, _unpack(wu_p[:, n0 * 128:n1 * 128]))[0:8]
                if early is not None:
                    g = g + early[1][:, n0 * 128:n1 * 128]
                    u = u + early[1][:, FM1 + n0 * 128:FM1 + n1 * 128]
                g = g * rstd
                hs.append((n0, n1, _lhs(g * _sigmoid(g) * (u * rstd))))
            for n in range(FT - nv, FT):
                if early is not None and n * 128 < FM1:
                    g = vpu_cols(early[0], ("g", n)) + early[1][:, n * 128:(n + 1) * 128]
                    u = (vpu_cols(early[0], ("u", n))
                         + early[1][:, FM1 + n * 128:FM1 + (n + 1) * 128])
                else:
                    g = vpu_cols(xc, ("g", n))
                    u = vpu_cols(xc, ("u", n))
                g = g * rstd
                u = u * rstd
                hs.append((n, n + 1, _lhs(g * _sigmoid(g) * u)))
            y = None
            for n0, n1, h in hs:
                d = _dot(h, _unpack(wd_p[n0 * 64:n1 * 64, :]))[0:8]
                y = d if y is None else y + d
            hall = jnp.concatenate([h[0:8].astype(_F32) for _, _, h in hs], axis=1)
            my = lane_mean_part(hall * rmd_v[...])
            return x + xc * rstd + y * gate, m + my * gate

        for cp in w_copies[0]:
            cp.wait()
        repack(wq_r, wq_p, 16)
        transpose_blocks(wq_r, "q")

        def wqf_go(t, _):
            for (c, i), n in wqf_slot.items():
                r = pl.multiple_of(i * 128 + t * 16, 16)
                wq_f[n, pl.ds(pl.multiple_of(t * 16, 16), 16), :] = (
                    wq_r[pl.ds(r, 16), c * DP:(c + 1) * DP].astype(_F32))
            return 0
        lax.fori_loop(0, 8, wqf_go, 0)

        xs_v[...] = jnp.zeros(xs_v.shape, _F32)
        xs_v[0:B, :] = x_v[...].astype(_F32)
        wr = wr_v[...].astype(_F32).reshape(1, D)
        xc0 = xs_v[...] - jnp.mean(xs_v[...], axis=-1, keepdims=True)
        qs0 = _rstd(xc0) * qscale
        xb0 = _lhs(xc0)

        def q1_go(c, _):
            col = pl.multiple_of(c * DP, 128)
            q1_v[:, pl.ds(col, DP)] = _dot(xb0, _unpack(wq_p[:, pl.ds(col, DP)]))[0:8] * qs0
            return 0
        lax.fori_loop(0, NC, q1_go, 0)

        for cp in w_copies[1]:
            cp.wait()

        def wo_go(n, _):
            g = n // GI
            i = n % GI
            for j in range(NJ):
                r = pl.multiple_of((n * NJ + j) * 16, 16)
                wo_p[g, j, pl.ds(pl.multiple_of(i * 8, 8), 8), :] = _pack(wo_r[pl.ds(r, 16), :])
            return 0
        lax.fori_loop(0, NG * GI, wo_go, 0)

        def wof_go(t, _):
            for (c, i), n in wof_slot.items():
                r = pl.multiple_of(c * DP + i * 128 + t * 16, 16)
                wo_f[n, pl.ds(pl.multiple_of(t * 16, 16), 16), :] = with_mean(wo_r[pl.ds(r, 16), :])
            return 0
        lax.fori_loop(0, 8, wof_go, 0)

        def wlf_go(i, _):
            for j in range(NJ):
                r = pl.multiple_of((((NG - 1) * GI + i) * NJ + j) * 16, 16)
                wl_f[j, i] = with_mean(wo_r[pl.ds(r, 16), :])
            return 0
        lax.fori_loop(0, GI, wlf_go, 0)
        row_means(wo_r, rmo_v)

        for cp in w_copies[2]:
            cp.wait()
        repack(wg_r, wg_p, 64)
        repack(wu_r, wu_p, 64)
        repack(wd_r, wd_p, 128)
        transpose_blocks(wg_r, "g")
        transpose_blocks(wu_r, "u")
        row_means(wd_r, rmd_v)

        def wl2_go(i, _):
            r = pl.multiple_of((((NG - 1) * GI + IA + i) * NJ + NJ - 1) * 16, 16)
            rows = wo_r[pl.ds(r, 16), :]
            mean = wl_f[NJ - 1, IA + i, :, D:]
            for e, w_p in enumerate((wg_p, wu_p)):
                w = _unpack(w_p[:, 0:FM1])
                csum = _dot(jnp.ones((16, D), _BF16), w)
                wl2_f[i, :, e * FM1:(e + 1) * FM1] = (
                    _dot(rows, w) - jnp.concatenate([mean] * (FM1 // 128), axis=1) * csum)
            return 0
        lax.fori_loop(0, GI - IA, wl2_go, 0)

        def attention3(x, m):
            xc = x - tile_d(m)
            qs8 = _rstd(xc) * qscale
            xb = _lhs(xc)
            xcol = {i: jnp.broadcast_to(xc[0:1, i * 128:(i + 1) * 128], (128, 128)).T
                    for i in range(DT - max(ka.values()), DT)}

            def stage_a(c):
                km = (DT - ka[c]) * 128
                nm = (3 - ra[c]) * 128
                q = None
                if km and nm:
                    q = _dot(xb[:, 0:km], _unpack(wq_p[0:km // 2, c * DP:c * DP + nm]))[0:8]
                if ka[c] and nm:
                    a = None
                    for i in range(DT - ka[c], DT):
                        for t in range(16):
                            xx = xcol[i][t * 8:(t + 1) * 8, :]
                            cc = (jnp.concatenate([xx] * (nm // 128), axis=1)
                                  * wq_f[wqf_slot[c, i], t * 8:(t + 1) * 8, 0:nm])
                            a = cc if a is None else a + cc
                    a = jnp.sum(a, axis=0, keepdims=True)
                    q = jnp.broadcast_to(a, (8, nm)) if q is None else q + a
                cols = [] if q is None else [q]
                cols += [vpu_cols(xc, ("q", c * 3 + i)) for i in range(3 - ra[c], 3)]
                q = jnp.concatenate(cols, axis=1)
                return q if perm.index(c) < cfg["LS"] else q * qs8

            def v_rows(c, t):
                g, j, i = chunk_pos(c, t)
                if g == NG - 1 and j == NJ - 1 and i >= IA:
                    return vraw[g % NS, i, j].astype(_F32)
                return vf[g, j, i]

            def stage_c(p, linv, c, wide):
                nt = (3 - bd[c]) * 8
                head = lambda t: t // (PT // 2)
                chunk = lambda t: pv_chunk(p[head(t) * 8:head(t) * 8 + 8], v_rows(c, t))
                o = mo = None
                if nt:
                    l0 = jnp.broadcast_to(linv[0:8], (8, 128))
                    l1 = jnp.broadcast_to(linv[8:16], (8, 128))
                    li = [l0, jnp.where(low_half, l0, l1), l1][0:nt // 8]
                    o = _lhs(_row_sums8([chunk(t) for t in range(nt)])
                             * jnp.concatenate(li, axis=1))
                    mo = _lane_fold(o[0:8].astype(_F32) * rmo_v[:, c * DP:c * DP + nt * 16])
                tot = None
                for hh in range(2):
                    a = None
                    for t in range(nt, PT):
                        if head(t) != hh:
                            continue
                        r = (t % 8) * 16
                        cc = vpu_out(chunk(t), wo_f[wof_slot[c, t // 8], r:r + 16, 0:wide])
                        a = cc if a is None else a + cc
                    if a is not None:
                        a = a * linv[hh * 8:hh * 8 + 8]
                        tot = a if tot is None else tot + a
                return o, mo, tot

            def stage_d(o, c):
                ws = []
                for t in range(o.shape[1] // 16):
                    g, j, i = chunk_pos(c, t)
                    ws.append(wo_p[g, j, i * 8:(i + 1) * 8, :])
                return _dot(o, _unpack(jnp.concatenate(ws, axis=0)))[0:8]

            acc, accm, accv, accw = None, None, None, None
            qs, ss, ps, ls, os_, mos, pvs = {}, {}, {}, {}, {}, {}, {}
            early = {int(a, 16): int(t, 16) for a, t in zip(cfg["LA"][0::2], cfg["LA"][1::2])}
            for n in early:
                qs[n] = stage_a(perm[n])
            off = dict(A=cfg["SA"], B=cfg["SB"], M=cfg["SM"], S=cfg["SS"], C=0)
            for step in range(-cfg["SA"], max(dpos) + 1):
                for st in cfg["order"]:
                    if st == "D":
                        for n in range(NC):
                            if dpos[n] == step and os_[n] is not None:
                                d = stage_d(os_[n], perm[n])
                                acc = d if acc is None else acc + d
                        continue
                    n = step + off[st]
                    if not 0 <= n < NC:
                        continue
                    c = perm[n]
                    if st == "A":
                        if n not in early:
                            qs[n] = stage_a(c)
                    elif st == "B":
                        ss[n] = scores(jnp.concatenate([qs[n], qs[n]], axis=0), _unpack(kp[c]))
                    elif st == "M":
                        deps = [qs[a] for a, t in early.items() if t == n]
                        if cfg["LT"] and mos.get(n - cfg["LT"]) is not None:
                            deps.append(mos[n - cfg["LT"]])
                        if cfg["LV"] and pvs.get(n - cfg["LV"]) is not None:
                            deps.append(pvs[n - cfg["LV"]])
                        late_scale = None
                        if n < cfg["LS"]:
                            late_scale = jnp.concatenate([qs8, qs8], axis=0)
                        ps[n] = probs(ss[n], deps, late_scale)
                    elif st == "S":
                        ls[n] = inv_sum(ps[n])
                    elif st == "C":
                        late = n >= NC - cfg["LM"]
                        os_[n], mos[n], part = stage_c(ps[n], ls[n], c, D + 128 if late else D)
                        if mos[n] is not None:
                            accm = mos[n] if accm is None else accm + mos[n]
                        if part is not None and late:
                            accw = part if accw is None else accw + part
                        elif part is not None:
                            accv = part if accv is None else accv + part
                            pvs[n] = accv
            if accv is not None:
                mv = _lane_fold(accv) * (1.0 / D)
                accm = mv if accm is None else accm + mv
                acc = accv if acc is None else acc + accv
            tot = jnp.concatenate([acc, lane_mean_part(accm)], axis=1)
            if accw is not None:
                tot = tot + accw
            tot = jnp.sum(tot, axis=0, keepdims=True)
            return x + tot[:, 0:D], m + tot[:, D:]

        def batch(b, _):
            @pl.when(b > 0)
            def _():
                for cp in v_copies(b, (NG - 1 + NS) % NG):
                    cp.start()

            def group_probs(g, s, static):
                for cp in k_copies(b, g):
                    cp.wait()
                linvs = []
                for i in range(GP):
                    c = g * GP + i
                    col = c * DP if static else pl.multiple_of(c * DP, 128)
                    q16 = jnp.broadcast_to(q1_v[pl.ds(b, 1), pl.ds(col, DP)], (16, DP))
                    kk = kraw[s, i * PI:(i + 1) * PI].reshape(DP, W)
                    kp[c] = _pack(kk)
                    p = probs(scores(q16, kk))
                    p_v[i] = p
                    linvs.append(inv_sum(p))
                start_next(k_copies, b, g)
                return linvs

            def head_probs(i):
                h = i // HI
                return p_v[h // 2, (h % 2) * 8:(h % 2) * 8 + 8, :]

            def piece(g, s, j, li):
                parts = []
                for i in range(GI):
                    vv = vraw[s, i, j].astype(_F32)
                    vf[g, j, i] = vv
                    parts.append(pv_chunk(head_probs(i), vv))
                o = _lhs(_row_sums(parts) * li)
                return _dot(o, _unpack(wo_p[g, j]))[0:8]

            def group(g, acc):
                s = g % NS
                linvs = group_probs(g, s, False)
                lane = lax.broadcasted_iota(jnp.int32, (8, GI * 16), 1)
                li = jnp.broadcast_to(linvs[0][0:8], (8, GI * 16))
                for h in range(1, 2 * GP):
                    li = jnp.where(lane >= h * HI * 16,
                                   linvs[h // 2][(h % 2) * 8:(h % 2) * 8 + 8], li)
                for cp in v_copies(b, g):
                    cp.wait()
                for j in range(NJ):
                    acc = acc + piece(g, s, j, li)

                @pl.when(g == NG - 1 - NS)
                def _():
                    for cp in v_last_copies(b):
                        cp.start()

                @pl.when(g != NG - 1 - NS)
                def _():
                    start_next(v_copies, b, g)
                return acc

            x = lax.fori_loop(0, NG - 1, group, jnp.broadcast_to(xs_v[pl.ds(b, 1), :], (8, D)))
            g = NG - 1
            s = g % NS
            m = lane_mean_part(x) * (1.0 / D)
            linvs = group_probs(g, s, True)
            tot = None
            for cp, (j, i0, i1) in zip(v_last_copies(b), last_parts):
                final = j == NJ - 1 and i0 == IA
                if final:
                    tot = jnp.sum(tot, axis=0, keepdims=True)
                    x = x + tot[:, 0:D]
                    m = m + tot[:, D:]
                    xc_early = x - tile_d(m)
                    tot = None
                cp.wait()
                for h in range(GI // HI):
                    a = None
                    for i in range(max(i0, h * HI), min(i1, (h + 1) * HI)):
                        vv = vraw[s, i, j].astype(_F32)
                        w = wl_f[j, i]
                        if final:
                            w = jnp.concatenate([w, wl2_f[i - IA]], axis=1)
                        else:
                            vf[g, j, i] = vv
                        cc = vpu_out(pv_chunk(head_probs(i), vv), w)
                        a = cc if a is None else a + cc
                    if a is not None:
                        a = a * linvs[h // 2][(h % 2) * 8:(h % 2) * 8 + 8]
                        tot = a if tot is None else tot + a
            tot = jnp.sum(tot, axis=0, keepdims=True)
            x = x + tot[:, 0:D]
            m = m + tot[:, D:D + 128]

            x, m = ffn(x, m, wr, nv1, (xc_early, tot[:, D + 128:]))
            x, m = attention3(x, m)
            x, _ = ffn(x, m, wr, nv)
            xs = jnp.where(lax.broadcasted_iota(jnp.int32, (8, D), 0) == b, x, xs_v[...])
            xs_v[...] = xs
            o_ref[...] = xs[0:B].astype(o_ref.dtype)
            return 0

        lax.fori_loop(0, B, batch, 0)

    any_spec = pl.BlockSpec(memory_space=pl.ANY)
    out = pl.pallas_call(
        kernel,
        in_specs=[any_spec] * 9,
        out_specs=pl.BlockSpec(memory_space=pltpu.VMEM),
        out_shape=jax.ShapeDtypeStruct((B, D), A_x.dtype),
        scratch_shapes=[
            pltpu.VMEM((NS, GI, NJ, 16, W), _BF16),
            pltpu.VMEM((NS, GI, NJ, 16, W), _BF16),
            pltpu.VMEM((NC, DP // 2, W), _U32),
            pltpu.VMEM((NG, NJ, GI, 16, W), _F32),
            pltpu.VMEM((D, H * Dh), _BF16),
            pltpu.VMEM((H * Dh, D), _BF16),
            pltpu.VMEM((D, F), _BF16),
            pltpu.VMEM((D, F), _BF16),
            pltpu.VMEM((F, D), _BF16),
            pltpu.VMEM((D // 2, H * Dh), _U32),
            pltpu.VMEM((NG, NJ, GI * 8, D), _U32),
            pltpu.VMEM((D // 2, F), _U32),
            pltpu.VMEM((D // 2, F), _U32),
            pltpu.VMEM((F // 2, D), _U32),
            pltpu.VMEM((max(len(wqf_slot), 1), 128, DP), _F32),
            pltpu.VMEM((max(len(wof_slot), 1), 128, D + 128), _F32),
            pltpu.VMEM((NJ, GI, 16, D + 128), _F32),
            pltpu.VMEM((GI - IA, 16, 2 * FM1), _F32),
            pltpu.VMEM((max(len(wt_slot), 1), 128, D), _F32),
            pltpu.VMEM((B, D), _BF16),
            pltpu.VMEM((D,), _BF16),
            pltpu.VMEM((8, D), _F32),
            pltpu.VMEM((8, H * Dh), _F32),
            pltpu.VMEM((GP, 16, W), _F32),
            pltpu.VMEM((8, H * Dh), _F32),
            pltpu.VMEM((8, F), _F32),
            pltpu.SemaphoreType.DMA((NS,)),
            pltpu.SemaphoreType.DMA((NS,)),
            pltpu.SemaphoreType.DMA((len(last_parts),)),
        ],
        compiler_params=_compiler_params(),
    )(
        A_x.reshape(B, D),
        jnp.swapaxes(A_k_cache, 2, 3).reshape(B, NG, GI, NJ, 16, Sk),
        jnp.swapaxes(A_v_cache, 2, 3).reshape(B, NG, GI, NJ, 16, Sk),
        A_wq, A_wo, B_w_r, B_w_gate, B_w_up, B_w_down,
    )
    return out.reshape(B, Sq, D)


@jax.jit
def pallas_interleave_layers__sliding_block_cached__moe_arch_mod__decode_kernel(
    A_x: jax.Array,
    A_k_cache: jax.Array,
    A_v_cache: jax.Array,
    A_wq: jax.Array,
    A_wo: jax.Array,
    B_x: jax.Array,
    B_w_r: jax.Array,
    B_w_gate: jax.Array,
    B_w_up: jax.Array,
    B_w_down: jax.Array,
):
    return _forward(_CFG, A_x, A_k_cache, A_v_cache, A_wq, A_wo,
                    B_w_r, B_w_gate, B_w_up, B_w_down)
```

```python
import jax
import jax.numpy as jnp
from jax import lax
import jax.experimental.pallas as pl
import jax.experimental.pallas.tpu as pltpu

_F32 = jnp.float32
_BF16 = jnp.bfloat16
_U32 = jnp.uint32
_LOG2E = 1.4426950408889634

_CFG = dict(
    SA=5, SB=2, SM=1, SS=0, order="MSCABD",
    rot=13,
    ka="0122211111111111",
    ra="0000000000000000",
    bd="2111121111111113",
    sd="3211141111121123",
    LM=1,
    LK="--" * 16,
    LS=0, LT=0, LV=0, L2=0, LA="",
    NJ=6,
    cuts=(0, 3, 8),
    nv1=6, nr1=0,
    nr=2,
    nv=5, fgrp=3,
)


def _pack(x):
    return pltpu.bitcast(x, _U32)


def _unpack(x):
    return pltpu.bitcast(x, _BF16)


def _dot(a, b):
    return jnp.dot(a, b, preferred_element_type=_F32)


def _dot_t(a, b):
    return lax.dot_general(a, b, (((1,), (1,)), ((), ())), preferred_element_type=_F32)


def _lhs(x8):
    return jnp.concatenate([x8, x8], axis=0).astype(_BF16)


def _lane_fold(x):
    a = x[:, 0:128]
    for j in range(1, x.shape[1] // 128):
        a = a + x[:, j * 128:(j + 1) * 128]
    return a


def _row_sums(parts):
    return jnp.sum(jnp.concatenate(parts, axis=0).T, axis=0, keepdims=True)


def _row_sums8(parts):
    t = jnp.concatenate(parts, axis=0).T
    a = t[0:8]
    for i in range(1, 16):
        a = a + t[i * 8:(i + 1) * 8]
    return a


def _sigmoid(x):
    return 0.5 * jnp.tanh(0.5 * x) + 0.5


def _rstd(xc):
    return lax.rsqrt(jnp.mean(xc * xc, axis=-1, keepdims=True) + 1e-5)


def _compiler_params():
    limit = 120 * 1024 * 1024
    try:
        return pltpu.CompilerParams(vmem_limit_bytes=limit, disable_semaphore_checks=True)
    except TypeError:
        return pltpu.CompilerParams(vmem_limit_bytes=limit)


def _forward(cfg, A_x, A_k_cache, A_v_cache, A_wq, A_wo, B_w_r, B_w_gate, B_w_up, B_w_down):
    B, Sq, D = A_x.shape
    _, H, Sk, Dh = A_k_cache.shape
    F = B_w_gate.shape[1]
    W = min(4096, max(256, Sk // 4))
    assert Sq == 1 and H == 32 and Dh == 192 and B <= 8 and D % 128 == 0 and F % 128 == 0
    DP = 2 * Dh
    NC = H // 2
    DT = D // 128
    FT = F // 128
    NJ = cfg["NJ"]
    GP = 2
    NG = NC // GP
    GI = GP * DP // (16 * NJ)
    PI = GI // GP
    HI = PI // 2
    PT = DP // 16
    NS = 4
    cuts = cfg["cuts"]
    IA = cuts[-2]
    last_parts = [(j, 0, GI) for j in range(NJ - 1)]
    last_parts += [(NJ - 1, i0, i1) for i0, i1 in zip(cuts[:-1], cuts[1:])]
    qscale = float(Dh) ** -0.5 * _LOG2E

    perm = [(cfg["rot"] + n) % NC for n in range(NC)]
    ka = {perm[n]: int(c) for n, c in enumerate(cfg["ka"])}
    ra = {perm[n]: int(c) for n, c in enumerate(cfg["ra"])}
    bd = {perm[n]: int(c) for n, c in enumerate(cfg["bd"])}
    dpos = [n + int(c, 16) for n, c in enumerate(cfg["sd"])]
    nv, nr, nv1, nr1 = cfg["nv"], cfg["nr"], cfg["nv1"], cfg["nr1"]
    NR = max(nr, nr1)
    FM1 = (FT - nv1 - nr1) * 128

    def slots(keys):
        return {key: n for n, key in enumerate(keys)}
    wqf_slot = slots((c, i) for c in range(NC) for i in range(DT - ka[c], DT))
    wof_slot = slots((c, i) for c in range(NC) for i in range(3 - bd[c], 3))
    wt_slot = slots([("q", c * 3 + i) for c in range(NC) for i in range(3 - ra[c], 3)]
                    + [(w, n) for n in range(FT - max(nv + nr, nv1 + nr1), FT) for w in "gu"])

    def chunk_pos(c, t):
        return c // GP, t % NJ, (c % GP) * PI + t // NJ

    def kernel(x_hbm, k_hbm, v_hbm, wq_hbm, wo_hbm, wr_hbm, wg_hbm, wu_hbm, wd_hbm,
               o_ref,
               kraw, vraw, kp, vf,
               wq_r, wo_r, wg_r, wu_r, wd_r,
               wq_p, wo_p, wg_p, wu_p, wd_p, wq_f, wo_f, wl_f, wl2_f, wd_f, w_t,
               x_v, wr_v, xs_v, q1_v, p_v, rmo_v, rmd_v,
               ksem, vsem, lsem):

        def k_copies(b, g):
            s = g % NS
            return [pltpu.make_async_copy(
                k_hbm.at[b, g, :, j, :, pl.ds(Sk - W, W)], kraw.at[s, :, j],
                ksem.at[s]) for j in range(NJ)]

        def v_copies(b, g):
            s = g % NS
            return [pltpu.make_async_copy(
                v_hbm.at[b, g, :, j, :, pl.ds(Sk - W, W)], vraw.at[s, :, j],
                vsem.at[s]) for j in range(NJ)]

        def v_last_copies(b):
            g = NG - 1
            return [pltpu.make_async_copy(
                v_hbm.at[b, g, pl.ds(i0, i1 - i0), j, :, pl.ds(Sk - W, W)],
                vraw.at[g % NS, pl.ds(i0, i1 - i0), j], lsem.at[e])
                for e, (j, i0, i1) in enumerate(last_parts)]

        def start_next(copies, b, g):
            n = b * NG + g + NS

            @pl.when(n < B * NG)
            def _():
                for cp in copies(n // NG, n % NG):
                    cp.start()

        w_sets = [
            [(wq_hbm, wq_r), (x_hbm, x_v), (wr_hbm, wr_v)],
            [(wo_hbm, wo_r)],
            [(wg_hbm, wg_r), (wu_hbm, wu_r), (wd_hbm, wd_r)],
        ]
        w_copies = [[pltpu.make_async_copy(src, dst, lsem.at[i]) for src, dst in ws]
                    for i, ws in enumerate(w_sets)]
        for ws in w_copies:
            for cp in ws:
                cp.start()

        def start0(g, _):
            for cp in k_copies(0, g) + v_copies(0, g):
                cp.start()
            return 0
        lax.fori_loop(0, NS, start0, 0)

        def repack(raw, packed, rows):
            def go(i, _):
                r = pl.multiple_of(i * rows, rows)
                r2 = pl.multiple_of(i * (rows // 2), rows // 2)
                packed[pl.ds(r2, rows // 2), :] = _pack(raw[pl.ds(r, rows), :])
                return 0
            lax.fori_loop(0, raw.shape[0] // rows, go, 0)

        def transpose_blocks(raw, name):
            keys = [key for key in wt_slot if key[0] == name]
            if keys:
                def go(i, _):
                    r = pl.multiple_of(i * 128, 128)
                    for key in keys:
                        blk = raw[pl.ds(r, 128), key[1] * 128:(key[1] + 1) * 128]
                        w_t[wt_slot[key], :, pl.ds(r, 128)] = blk.astype(_F32).T
                    return 0
                lax.fori_loop(0, DT, go, 0)

        def row_means(raw, dst):
            ones = jnp.ones((16, D), _BF16)

            def go(i, _):
                r = pl.multiple_of(i * 512, 512)
                dst[:, pl.ds(r, 512)] = _dot_t(ones, raw[pl.ds(r, 512), :])[0:8] * (1.0 / D)
                return 0
            lax.fori_loop(0, raw.shape[0] // 512, go, 0)

        def with_mean(rows):
            w = rows.astype(_F32)
            m = jnp.mean(w, axis=-1, keepdims=True)
            return jnp.concatenate([w, jnp.broadcast_to(m, (w.shape[0], 128))], axis=1)

        row16 = lax.broadcasted_iota(jnp.int32, (16, DP), 0)
        col16 = lax.broadcasted_iota(jnp.int32, (16, DP), 1)
        qmask = (row16 < 8) == (col16 < Dh)
        low_half = lax.broadcasted_iota(jnp.int32, (8, 128), 1) < 64

        def tile_d(m):
            return jnp.concatenate([m] * DT, axis=1)

        def lane_mean_part(x):
            return jnp.broadcast_to(jnp.sum(_lane_fold(x), axis=-1, keepdims=True), (8, 128))

        def scores(q16, kk):
            q = jnp.where(qmask, q16, 0.0).astype(_BF16)
            s0 = _dot(q[:, 0:128], kk[0:128])
            s1 = _dot(q[:, 128:256], kk[128:256])
            s2 = _dot(q[:, 256:384], kk[256:384])
            return s1 + jnp.concatenate([s0[0:8], s2[8:16]], axis=0)

        def after(x, deps):
            if not deps:
                return x
            d = _lane_fold(jnp.concatenate(list(deps), axis=1))
            d = jnp.concatenate([d] * (x.shape[0] // 8), axis=0)
            return jnp.where(d != d, d, x)

        def probs(s, deps=(), scale=None):
            pm = s[:, 0:128]
            for j in range(1, s.shape[1] // 128):
                pm = jnp.maximum(pm, s[:, j * 128:(j + 1) * 128])
            if cfg["L2"]:
                pm = after(pm, deps)
            else:
                pm = jnp.concatenate([after(pm[0:8], deps), pm[8:16]], axis=0)
            e = s - jnp.max(pm, axis=-1, keepdims=True)
            return jnp.exp2(e if scale is None else e * scale)

        def inv_sum(p):
            l = jnp.sum(p, axis=-1, keepdims=True)
            r = pl.reciprocal(l, approx=True)
            return r * (2.0 - l * r)

        def pv_chunk(pp, vv):
            return _lane_fold(vv * jnp.concatenate([pp, pp], axis=0))

        def vpu_out(part, w):
            cc = jnp.sum(part, axis=1, keepdims=True) * w
            return cc[0:8] + cc[8:16]

        def vpu_cols(xc, key):
            parts = [_lane_fold(w_t[wt_slot[key], t * 8:(t + 1) * 8, :] * xc) for t in range(16)]
            return jnp.broadcast_to(_row_sums(parts), (8, 128))

        def ffn(x, m, wr, nv, nr, early=None):
            xc = x - tile_d(m)
            rstd = _rstd(xc)
            half = 0.5 * rstd
            gate = _sigmoid(jnp.sum(xc * wr, axis=-1, keepdims=True) * rstd)

            def hidden(g, u):
                a = g * half
                return (a + a * jnp.tanh(a)) * u

            xb = _lhs(xc if early is None else early[0])
            nm = FT - nv - nr
            hs = []
            for n0 in range(0, nm, cfg["fgrp"]):
                n1 = min(nm, n0 + cfg["fgrp"])
                g = _dot(xb, _unpack(wg_p[:, n0 * 128:n1 * 128]))[0:8]
                u = _dot(xb, _unpack(wu_p[:, n0 * 128:n1 * 128]))[0:8]
                if early is not None:
                    g = g + early[1][:, n0 * 128:n1 * 128]
                    u = u + early[1][:, FM1 + n0 * 128:FM1 + n1 * 128]
                hs.append((n0, n1, _lhs(hidden(g, u))))
            for n in range(nm, nm + nv):
                hs.append((n, n + 1, _lhs(hidden(vpu_cols(xc, ("g", n)), vpu_cols(xc, ("u", n))))))
            yv = None
            for n in range(FT - nr, FT):
                for t in range(16):
                    g, u = [jnp.sum(w_t[wt_slot[w, n], t * 8:(t + 1) * 8, :] * xc,
                                    axis=-1, keepdims=True) for w in "gu"]
                    r = (n - FT + NR) * 128 + t * 8
                    cc = hidden(g, u) * wd_f[r:r + 8, :]
                    yv = cc if yv is None else yv + cc
            y = None
            for n0, n1, h in hs:
                d = _dot(h, _unpack(wd_p[n0 * 64:n1 * 64, :]))[0:8]
                y = d if y is None else y + d
            hall = jnp.concatenate([h[0:8].astype(_F32) for _, _, h in hs], axis=1)
            my = lane_mean_part(hall * rmd_v[:, 0:(FT - nr) * 128])
            if yv is not None:
                yv = jnp.sum(yv, axis=0, keepdims=True)
                y = y + yv[:, 0:D]
                my = my + yv[:, D:]
            gate = gate * rstd
            return x + xc * rstd + y * gate, m + my * gate

        for cp in w_copies[0]:
            cp.wait()
        repack(wq_r, wq_p, 16)
        transpose_blocks(wq_r, "q")

        def wqf_go(t, _):
            for (c, i), n in wqf_slot.items():
                r = pl.multiple_of(i * 128 + t * 16, 16)
                wq_f[n, pl.ds(pl.multiple_of(t * 16, 16), 16), :] = (
                    wq_r[pl.ds(r, 16), c * DP:(c + 1) * DP].astype(_F32))
            return 0
        lax.fori_loop(0, 8, wqf_go, 0)

        xs_v[...] = jnp.zeros(xs_v.shape, _F32)
        xs_v[0:B, :] = x_v[...].astype(_F32)
        wr = wr_v[...].astype(_F32).reshape(1, D)
        xc0 = xs_v[...] - jnp.mean(xs_v[...], axis=-1, keepdims=True)
        qs0 = _rstd(xc0) * qscale
        xb0 = _lhs(xc0)

        def q1_go(g, _):
            col = pl.ds(pl.multiple_of(g * GP * DP, 128), GP * DP)
            q1_v[:, col] = _dot(xb0, _unpack(wq_p[:, col]))[0:8] * qs0
            return 0
        lax.fori_loop(0, NG, q1_go, 0)

        for cp in w_copies[1]:
            cp.wait()

        def wo_go(n, _):
            g = n // GI
            i = n % GI
            for j in range(NJ):
                r = pl.multiple_of((n * NJ + j) * 16, 16)
                wo_p[g, j, pl.ds(pl.multiple_of(i * 8, 8), 8), :] = _pack(wo_r[pl.ds(r, 16), :])
            return 0
        lax.fori_loop(0, NG * GI, wo_go, 0)

        def wof_go(t, _):
            for (c, i), n in wof_slot.items():
                r = pl.multiple_of(c * DP + i * 128 + t * 16, 16)
                wo_f[n, pl.ds(pl.multiple_of(t * 16, 16), 16), :] = with_mean(wo_r[pl.ds(r, 16), :])
            return 0
        lax.fori_loop(0, 8, wof_go, 0)

        def wlf_go(i, _):
            for j in range(NJ):
                r = pl.multiple_of((((NG - 1) * GI + i) * NJ + j) * 16, 16)
                wl_f[j, i] = with_mean(wo_r[pl.ds(r, 16), :])
            return 0
        lax.fori_loop(0, GI, wlf_go, 0)
        row_means(wo_r, rmo_v)

        for cp in w_copies[2]:
            cp.wait()
        repack(wg_r, wg_p, 64)
        repack(wu_r, wu_p, 64)
        repack(wd_r, wd_p, 128)
        transpose_blocks(wg_r, "g")
        transpose_blocks(wu_r, "u")
        row_means(wd_r, rmd_v)

        def wdf_go(i, _):
            r = pl.multiple_of(i * 128, 128)
            wd_f[pl.ds(r, 128), :] = with_mean(wd_r[pl.ds(F - NR * 128 + r, 128), :])
            return 0
        lax.fori_loop(0, NR, wdf_go, 0)

        rows = [wo_r[pl.ds((((NG - 1) * GI + i) * NJ + NJ - 1) * 16, 16), :] for i in range(IA, GI)]
        rows = jnp.concatenate(rows + [jnp.ones((16, D), _BF16)], axis=0)

        def wl2_go(n, _):
            col = pl.multiple_of(n * 128, 128)
            for e, w_p in enumerate((wg_p, wu_p)):
                prod = _dot(rows, _unpack(w_p[:, pl.ds(col, 128)]))
                for i in range(GI - IA):
                    wl2_f[i, :, pl.ds(pl.multiple_of(e * FM1 + col, 128), 128)] = (
                        prod[i * 16:(i + 1) * 16]
                        - wl_f[NJ - 1, IA + i, :, D:] * prod[(GI - IA) * 16:])
            return 0
        lax.fori_loop(0, FM1 // 128, wl2_go, 0)

        def attention3(x, m):
            xc = x - tile_d(m)
            qs8 = _rstd(xc) * qscale
            xb = _lhs(xc)
            xcol = {i: jnp.broadcast_to(xc[0:1, i * 128:(i + 1) * 128], (128, 128)).T
                    for i in range(DT - max(ka.values()), DT)}

            def stage_a_vpu(c):
                nm = (3 - ra[c]) * 128
                a = None
                for i in range(DT - ka[c], DT):
                    for t in range(16):
                        xx = xcol[i][t * 8:(t + 1) * 8, :]
                        cc = (jnp.concatenate([xx] * (nm // 128), axis=1)
                              * wq_f[wqf_slot[c, i], t * 8:(t + 1) * 8, 0:nm])
                        a = cc if a is None else a + cc
                return jnp.broadcast_to(jnp.sum(a, axis=0, keepdims=True), (8, nm))

            lk = [cfg["LK"][2 * n:2 * n + 2] for n in range(NC)]
            qv = {perm[n]: stage_a_vpu(perm[n]) for n, t in enumerate(lk)
                  if t != "--" and ka[perm[n]] and ra[perm[n]] < 3}

            def linked(stage, n):
                return [qv[perm[a]] for a, t in enumerate(lk)
                        if t == "%s%x" % (stage, n) and perm[a] in qv]

            def first_after(v, deps):
                if not deps:
                    return v
                return jnp.concatenate([after(v[:, 0:128], deps), v[:, 128:]], axis=1)

            def stage_a(c):
                km = (DT - ka[c]) * 128
                nm = (3 - ra[c]) * 128
                q = None
                if km and nm:
                    deps = linked("A", perm.index(c))
                    lhs = _lhs(first_after(xc, deps)) if deps else xb
                    q = _dot(lhs[:, 0:km], _unpack(wq_p[0:km // 2, c * DP:c * DP + nm]))[0:8]
                if ka[c] and nm:
                    a = qv[c] if c in qv else stage_a_vpu(c)
                    q = a if q is None else q + a
                cols = [] if q is None else [q]
                cols += [vpu_cols(xc, ("q", c * 3 + i)) for i in range(3 - ra[c], 3)]
                q = jnp.concatenate(cols, axis=1)
                return q if perm.index(c) < cfg["LS"] else q * qs8

            def v_rows(c, t):
                g, j, i = chunk_pos(c, t)
                if g == NG - 1 and j == NJ - 1 and i >= IA:
                    return vraw[g % NS, i, j].astype(_F32)
                return vf[g, j, i]

            def stage_c(p, linv, c, wide):
                nt = (3 - bd[c]) * 8
                head = lambda t: t // (PT // 2)
                chunk = lambda t: pv_chunk(p[head(t) * 8:head(t) * 8 + 8], v_rows(c, t))
                o = mo = None
                if nt:
                    l0 = jnp.broadcast_to(linv[0:8], (8, 128))
                    l1 = jnp.broadcast_to(linv[8:16], (8, 128))
                    li = [l0, jnp.where(low_half, l0, l1), l1][0:nt // 8]
                    o = _lhs(_row_sums8([chunk(t) for t in range(nt)])
                             * jnp.concatenate(li, axis=1))
                    mo = _lane_fold(o[0:8].astype(_F32) * rmo_v[:, c * DP:c * DP + nt * 16])
                tot = None
                for hh in range(2):
                    a = None
                    for t in range(nt, PT):
                        if head(t) != hh:
                            continue
                        r = (t % 8) * 16
                        cc = vpu_out(chunk(t), wo_f[wof_slot[c, t // 8], r:r + 16, 0:wide])
                        a = cc if a is None else a + cc
                    if a is not None:
                        a = a * linv[hh * 8:hh * 8 + 8]
                        tot = a if tot is None else tot + a
                return o, mo, tot

            def stage_d(o, c):
                ws = []
                for t in range(o.shape[1] // 16):
                    g, j, i = chunk_pos(c, t)
                    ws.append(wo_p[g, j, i * 8:(i + 1) * 8, :])
                return _dot(o, _unpack(jnp.concatenate(ws, axis=0)))[0:8]

            acc, accm, accv, accw = None, None, None, None
            qs, ss, ps, ls, os_, mos, pvs = {}, {}, {}, {}, {}, {}, {}
            early = {int(a, 16): int(t, 16) for a, t in zip(cfg["LA"][0::2], cfg["LA"][1::2])}
            for n in early:
                qs[n] = stage_a(perm[n])
            off = dict(A=cfg["SA"], B=cfg["SB"], M=cfg["SM"], S=cfg["SS"], C=0)
            for step in range(-cfg["SA"], max(dpos) + 1):
                for st in cfg["order"]:
                    if st == "D":
                        for n in range(NC):
                            if dpos[n] == step and os_[n] is not None:
                                d = stage_d(os_[n], perm[n])
                                acc = d if acc is None else acc + d
                        continue
                    n = step + off[st]
                    if not 0 <= n < NC:
                        continue
                    c = perm[n]
                    if st == "A":
                        if n not in early:
                            qs[n] = stage_a(c)
                    elif st == "B":
                        q = first_after(qs[n], linked("B", n))
                        ss[n] = scores(jnp.concatenate([q, q], axis=0), _unpack(kp[c]))
                    elif st == "M":
                        deps = [qs[a] for a, t in early.items() if t == n]
                        deps += linked("M", n)
                        if cfg["LT"] and mos.get(n - cfg["LT"]) is not None:
                            deps.append(mos[n - cfg["LT"]])
                        if cfg["LV"] and pvs.get(n - cfg["LV"]) is not None:
                            deps.append(pvs[n - cfg["LV"]])
                        late_scale = None
                        if n < cfg["LS"]:
                            late_scale = jnp.concatenate([qs8, qs8], axis=0)
                        ps[n] = probs(ss[n], deps, late_scale)
                    elif st == "S":
                        ls[n] = inv_sum(ps[n])
                    elif st == "C":
                        late = n >= NC - cfg["LM"]
                        os_[n], mos[n], part = stage_c(ps[n], ls[n], c, D + 128 if late else D)
                        if mos[n] is not None:
                            accm = mos[n] if accm is None else accm + mos[n]
                        if part is not None and late:
                            accw = part if accw is None else accw + part
                        elif part is not None:
                            accv = part if accv is None else accv + part
                            pvs[n] = accv
            if accv is not None:
                mv = _lane_fold(accv) * (1.0 / D)
                accm = mv if accm is None else accm + mv
                acc = accv if acc is None else acc + accv
            tot = jnp.concatenate([acc, lane_mean_part(accm)], axis=1)
            if accw is not None:
                tot = tot + accw
            tot = jnp.sum(tot, axis=0, keepdims=True)
            return x + tot[:, 0:D], m + tot[:, D:]

        def batch(b, _):
            @pl.when(b > 0)
            def _():
                for cp in v_copies(b, (NG - 1 + NS) % NG):
                    cp.start()

            def group_probs(g, s, static):
                for cp in k_copies(b, g):
                    cp.wait()
                linvs = []
                for i in range(GP):
                    c = g * GP + i
                    col = c * DP if static else pl.multiple_of(c * DP, 128)
                    q16 = jnp.broadcast_to(q1_v[pl.ds(b, 1), pl.ds(col, DP)], (16, DP))
                    kk = kraw[s, i * PI:(i + 1) * PI].reshape(DP, W)
                    kp[c] = _pack(kk)
                    p = probs(scores(q16, kk))
                    p_v[i] = p
                    linvs.append(inv_sum(p))
                start_next(k_copies, b, g)
                return linvs

            def head_probs(i):
                h = i // HI
                return p_v[h // 2, (h % 2) * 8:(h % 2) * 8 + 8, :]

            def piece(g, s, j, li):
                parts = []
                for i in range(GI):
                    vv = vraw[s, i, j].astype(_F32)
                    vf[g, j, i] = vv
                    parts.append(pv_chunk(head_probs(i), vv))
                o = _lhs(_row_sums(parts) * li)
                return _dot(o, _unpack(wo_p[g, j]))[0:8]

            def group(g, acc):
                s = g % NS
                linvs = group_probs(g, s, False)
                lane = lax.broadcasted_iota(jnp.int32, (8, GI * 16), 1)
                li = jnp.broadcast_to(linvs[0][0:8], (8, GI * 16))
                for h in range(1, 2 * GP):
                    li = jnp.where(lane >= h * HI * 16,
                                   linvs[h // 2][(h % 2) * 8:(h % 2) * 8 + 8], li)
                for cp in v_copies(b, g):
                    cp.wait()
                for j in range(NJ):
                    acc = acc + piece(g, s, j, li)

                @pl.when(g == NG - 1 - NS)
                def _():
                    for cp in v_last_copies(b):
                        cp.start()

                @pl.when(g != NG - 1 - NS)
                def _():
                    start_next(v_copies, b, g)
                return acc

            x = lax.fori_loop(0, NG - 1, group, jnp.broadcast_to(xs_v[pl.ds(b, 1), :], (8, D)))
            g = NG - 1
            s = g % NS
            m = lane_mean_part(x) * (1.0 / D)
            linvs = group_probs(g, s, True)
            tot = None
            for cp, (j, i0, i1) in zip(v_last_copies(b), last_parts):
                final = j == NJ - 1 and i0 == IA
                if final:
                    tot = jnp.sum(tot, axis=0, keepdims=True)
                    x = x + tot[:, 0:D]
                    m = m + tot[:, D:]
                    xc_early = x - tile_d(m)
                    tot = None
                cp.wait()
                for h in range(GI // HI):
                    a = None
                    for i in range(max(i0, h * HI), min(i1, (h + 1) * HI)):
                        vv = vraw[s, i, j].astype(_F32)
                        w = wl_f[j, i]
                        if final:
                            w = jnp.concatenate([w, wl2_f[i - IA]], axis=1)
                        else:
                            vf[g, j, i] = vv
                        cc = vpu_out(pv_chunk(head_probs(i), vv), w)
                        a = cc if a is None else a + cc
                    if a is not None:
                        a = a * linvs[h // 2][(h % 2) * 8:(h % 2) * 8 + 8]
                        tot = a if tot is None else tot + a
            tot = jnp.sum(tot, axis=0, keepdims=True)
            x = x + tot[:, 0:D]
            m = m + tot[:, D:D + 128]

            x, m = ffn(x, m, wr, nv1, nr1, (xc_early, tot[:, D + 128:]))
            x, m = attention3(x, m)
            x, _ = ffn(x, m, wr, nv, nr)
            xs = jnp.where(lax.broadcasted_iota(jnp.int32, (8, D), 0) == b, x, xs_v[...])
            xs_v[...] = xs
            o_ref[...] = xs[0:B].astype(o_ref.dtype)
            return 0

        lax.fori_loop(0, B, batch, 0)

    any_spec = pl.BlockSpec(memory_space=pl.ANY)
    out = pl.pallas_call(
        kernel,
        in_specs=[any_spec] * 9,
        out_specs=pl.BlockSpec(memory_space=pltpu.VMEM),
        out_shape=jax.ShapeDtypeStruct((B, D), A_x.dtype),
        scratch_shapes=[
            pltpu.VMEM((NS, GI, NJ, 16, W), _BF16),
            pltpu.VMEM((NS, GI, NJ, 16, W), _BF16),
            pltpu.VMEM((NC, DP // 2, W), _U32),
            pltpu.VMEM((NG, NJ, GI, 16, W), _F32),
            pltpu.VMEM((D, H * Dh), _BF16),
            pltpu.VMEM((H * Dh, D), _BF16),
            pltpu.VMEM((D, F), _BF16),
            pltpu.VMEM((D, F), _BF16),
            pltpu.VMEM((F, D), _BF16),
            pltpu.VMEM((D // 2, H * Dh), _U32),
            pltpu.VMEM((NG, NJ, GI * 8, D), _U32),
            pltpu.VMEM((D // 2, F), _U32),
            pltpu.VMEM((D // 2, F), _U32),
            pltpu.VMEM((F // 2, D), _U32),
            pltpu.VMEM((max(len(wqf_slot), 1), 128, DP), _F32),
            pltpu.VMEM((max(len(wof_slot), 1), 128, D + 128), _F32),
            pltpu.VMEM((NJ, GI, 16, D + 128), _F32),
            pltpu.VMEM((GI - IA, 16, 2 * FM1), _F32),
            pltpu.VMEM((max(NR, 1) * 128, D + 128), _F32),
            pltpu.VMEM((max(len(wt_slot), 1), 128, D), _F32),
            pltpu.VMEM((B, D), _BF16),
            pltpu.VMEM((D,), _BF16),
            pltpu.VMEM((8, D), _F32),
            pltpu.VMEM((8, H * Dh), _F32),
            pltpu.VMEM((GP, 16, W), _F32),
            pltpu.VMEM((8, H * Dh), _F32),
            pltpu.VMEM((8, F), _F32),
            pltpu.SemaphoreType.DMA((NS,)),
            pltpu.SemaphoreType.DMA((NS,)),
            pltpu.SemaphoreType.DMA((len(last_parts),)),
        ],
        compiler_params=_compiler_params(),
    )(
        A_x.reshape(B, D),
        jnp.swapaxes(A_k_cache, 2, 3).reshape(B, NG, GI, NJ, 16, Sk),
        jnp.swapaxes(A_v_cache, 2, 3).reshape(B, NG, GI, NJ, 16, Sk),
        A_wq, A_wo, B_w_r, B_w_gate, B_w_up, B_w_down,
    )
    return out.reshape(B, Sq, D)


@jax.jit
def pallas_interleave_layers__sliding_block_cached__moe_arch_mod__decode_kernel(
    A_x: jax.Array,
    A_k_cache: jax.Array,
    A_v_cache: jax.Array,
    A_wq: jax.Array,
    A_wo: jax.Array,
    B_x: jax.Array,
    B_w_r: jax.Array,
    B_w_gate: jax.Array,
    B_w_up: jax.Array,
    B_w_down: jax.Array,
):
    return _forward(_CFG, A_x, A_k_cache, A_v_cache, A_wq, A_wo,
                    B_w_r, B_w_gate, B_w_up, B_w_down)
```

```python
import jax
import jax.numpy as jnp
from jax import lax
import jax.experimental.pallas as pl
import jax.experimental.pallas.tpu as pltpu

_F32 = jnp.float32
_BF16 = jnp.bfloat16
_U32 = jnp.uint32
_LOG2E = 1.4426950408889634

_CFG = dict(
    SA=5, SB=4, SM=2, SS=1, order="MSCDAB",
    rot=6,
    ka="0012011212110111",
    bd="2301032211121002",
    sd="0003142523640244",
    LM=3,
    NJ=6,
    cuts=(0, 5, 8),
    nv=5, nr=2, fgrp=3,
    nv1=2, nr1=3,
)


def _pack(x):
    return pltpu.bitcast(x, _U32)


def _unpack(x):
    return pltpu.bitcast(x, _BF16)


def _dot(a, b):
    return jnp.dot(a, b, preferred_element_type=_F32)


def _dot_t(a, b):
    return lax.dot_general(a, b, (((1,), (1,)), ((), ())), preferred_element_type=_F32)


def _lhs(x8):
    return jnp.concatenate([x8, x8], axis=0).astype(_BF16)


def _lane_fold(x):
    a = x[:, 0:128]
    for j in range(1, x.shape[1] // 128):
        a = a + x[:, j * 128:(j + 1) * 128]
    return a


def _row_sums(parts):
    return jnp.sum(jnp.concatenate(parts, axis=0).T, axis=0, keepdims=True)


def _row_sums8(parts):
    t = jnp.concatenate(parts, axis=0).T
    a = t[0:8]
    for i in range(1, 16):
        a = a + t[i * 8:(i + 1) * 8]
    return a


def _rstd(xc):
    return lax.rsqrt(jnp.mean(xc * xc, axis=-1, keepdims=True) + 1e-5)


def _compiler_params():
    limit = 120 * 1024 * 1024
    try:
        return pltpu.CompilerParams(vmem_limit_bytes=limit, disable_semaphore_checks=True)
    except TypeError:
        return pltpu.CompilerParams(vmem_limit_bytes=limit)


def _forward(cfg, A_x, A_k_cache, A_v_cache, A_wq, A_wo, B_w_r, B_w_gate, B_w_up, B_w_down):
    B, Sq, D = A_x.shape
    _, H, Sk, Dh = A_k_cache.shape
    F = B_w_gate.shape[1]
    W = min(4096, max(256, Sk // 4))
    assert Sq == 1 and H == 32 and Dh == 192 and B <= 8 and D % 128 == 0 and F % 128 == 0
    DP = 2 * Dh
    NC = H // 2
    DT = D // 128
    FT = F // 128
    NJ = cfg["NJ"]
    GP = 2
    NG = NC // GP
    GI = GP * DP // (16 * NJ)
    PI = GI // GP
    HI = PI // 2
    PT = DP // 16
    NS = 4
    cuts = cfg["cuts"]
    IA = cuts[-2]
    last_parts = [(j, 0, GI) for j in range(NJ - 1)]
    last_parts += [(NJ - 1, i0, i1) for i0, i1 in zip(cuts[:-1], cuts[1:])]
    qscale = float(Dh) ** -0.5 * _LOG2E

    perm = [(cfg["rot"] + n) % NC for n in range(NC)]
    ka = {perm[n]: int(c) for n, c in enumerate(cfg["ka"])}
    bd = {perm[n]: int(c) for n, c in enumerate(cfg["bd"])}
    dpos = [n + int(c, 16) for n, c in enumerate(cfg["sd"])]
    nv, nr, nv1, nr1 = cfg["nv"], cfg["nr"], cfg["nv1"], cfg["nr1"]
    NR = max(nr, nr1)
    FM1 = (FT - nv1 - nr1) * 128

    def slots(keys):
        return {key: n for n, key in enumerate(keys)}
    wqf_slot = slots((c, i) for c in range(NC) for i in range(DT - ka[c], DT))
    wof_slot = slots((c, i) for c in range(NC) for i in range(3 - bd[c], 3))
    wt_slot = slots((w, n) for n in range(FT - max(nv + nr, nv1 + nr1), FT) for w in "gu")

    def chunk_pos(c, t):
        return c // GP, t % NJ, (c % GP) * PI + t // NJ

    def kernel(x_hbm, k_hbm, v_hbm, wq_hbm, wo_hbm, wr_hbm, wg_hbm, wu_hbm, wd_hbm,
               o_ref,
               kraw, vraw, kp, vf,
               wq_r, wo_r, wg_r, wu_r, wd_r,
               wq_p, wo_p, wg_p, wu_p, wd_p, wq_f, wo_f, wl_f, wl2_f, wd_f, w_t,
               x_v, wr_v, xs_v, q1_v, p_v, rmo_v, rmd_v,
               ksem, vsem, lsem):

        def k_copies(b, g):
            s = g % NS
            return [pltpu.make_async_copy(
                k_hbm.at[b, g, :, j, :, pl.ds(Sk - W, W)], kraw.at[s, :, j],
                ksem.at[s]) for j in range(NJ)]

        def v_copies(b, g):
            s = g % NS
            return [pltpu.make_async_copy(
                v_hbm.at[b, g, :, j, :, pl.ds(Sk - W, W)], vraw.at[s, :, j],
                vsem.at[s]) for j in range(NJ)]

        def v_last_copies(b):
            g = NG - 1
            return [pltpu.make_async_copy(
                v_hbm.at[b, g, pl.ds(i0, i1 - i0), j, :, pl.ds(Sk - W, W)],
                vraw.at[g % NS, pl.ds(i0, i1 - i0), j], lsem.at[e])
                for e, (j, i0, i1) in enumerate(last_parts)]

        def start_next(copies, b, g):
            n = b * NG + g + NS

            @pl.when(n < B * NG)
            def _():
                for cp in copies(n // NG, n % NG):
                    cp.start()

        w_sets = [
            [(wq_hbm, wq_r), (x_hbm, x_v), (wr_hbm, wr_v)],
            [(wo_hbm, wo_r)],
            [(wg_hbm, wg_r), (wu_hbm, wu_r), (wd_hbm, wd_r)],
        ]
        w_copies = [[pltpu.make_async_copy(src, dst, lsem.at[i]) for src, dst in ws]
                    for i, ws in enumerate(w_sets)]
        for ws in w_copies:
            for cp in ws:
                cp.start()

        def start0(g, _):
            for cp in k_copies(0, g) + v_copies(0, g):
                cp.start()
            return 0
        lax.fori_loop(0, NS, start0, 0)

        def repack(raw, packed, rows):
            def go(i, _):
                r = pl.multiple_of(i * rows, rows)
                r2 = pl.multiple_of(i * (rows // 2), rows // 2)
                packed[pl.ds(r2, rows // 2), :] = _pack(raw[pl.ds(r, rows), :])
                return 0
            lax.fori_loop(0, raw.shape[0] // rows, go, 0)

        def transpose_blocks(raw, name):
            keys = [key for key in wt_slot if key[0] == name]
            if keys:
                def go(i, _):
                    r = pl.multiple_of(i * 128, 128)
                    for key in keys:
                        blk = raw[pl.ds(r, 128), key[1] * 128:(key[1] + 1) * 128]
                        w_t[wt_slot[key], :, pl.ds(r, 128)] = blk.astype(_F32).T
                    return 0
                lax.fori_loop(0, DT, go, 0)

        def row_means(raw, dst):
            ones = jnp.ones((16, D), _BF16)

            def go(i, _):
                r = pl.multiple_of(i * 512, 512)
                dst[:, pl.ds(r, 512)] = _dot_t(ones, raw[pl.ds(r, 512), :])[0:8] * (1.0 / D)
                return 0
            lax.fori_loop(0, raw.shape[0] // 512, go, 0)

        def with_mean(rows):
            w = rows.astype(_F32)
            m = jnp.mean(w, axis=-1, keepdims=True)
            return jnp.concatenate([w, jnp.broadcast_to(m, (w.shape[0], 128))], axis=1)

        low_half = lax.broadcasted_iota(jnp.int32, (8, 128), 1) < 64

        def tile_d(m):
            return jnp.concatenate([m] * DT, axis=1)

        def lane_mean_part(x):
            return jnp.broadcast_to(jnp.sum(_lane_fold(x), axis=-1, keepdims=True), (8, 128))

        def scores(q, kk):
            mid = q[:, 128:256]
            mid = jnp.concatenate([jnp.where(low_half, mid, 0.0), jnp.where(low_half, 0.0, mid)],
                                  axis=0).astype(_BF16)
            s0 = _dot(_lhs(q[:, 0:128]), kk[0:128])
            s1 = _dot(mid, kk[128:256])
            s2 = _dot(_lhs(q[:, 256:384]), kk[256:384])
            return s1 + jnp.concatenate([s0[0:8], s2[8:16]], axis=0)

        def probs(s):
            return jnp.exp2(s - jnp.max(s, axis=-1, keepdims=True))

        def inv_sum(p):
            l = jnp.sum(p, axis=-1, keepdims=True)
            r = pl.reciprocal(l, approx=True)
            return r * (2.0 - l * r)

        def pv_chunk(pp, vv):
            return _lane_fold(vv * jnp.concatenate([pp, pp], axis=0))

        def vpu_out(part, w):
            cc = jnp.sum(part, axis=1, keepdims=True) * w
            return cc[0:8] + cc[8:16]

        def vpu_cols(xc, key):
            parts = [_lane_fold(w_t[wt_slot[key], t * 8:(t + 1) * 8, :] * xc) for t in range(16)]
            return jnp.broadcast_to(_row_sums(parts), (8, 128))

        def ffn(x, m, wr, nv, nr, early=None):
            xc = x - tile_d(m)
            rstd = _rstd(xc)
            half = 0.5 * rstd
            gate = jax.nn.sigmoid(jnp.sum(xc * wr, axis=-1, keepdims=True) * rstd)

            def hidden(g, u):
                a = g * half
                return (a + a * jnp.tanh(a)) * u

            xb = _lhs(xc if early is None else early[0])
            nm = FT - nv - nr
            hs = []
            for n0 in range(0, nm, cfg["fgrp"]):
                n1 = min(nm, n0 + cfg["fgrp"])
                g = _dot(xb, _unpack(wg_p[:, n0 * 128:n1 * 128]))[0:8]
                u = _dot(xb, _unpack(wu_p[:, n0 * 128:n1 * 128]))[0:8]
                if early is not None:
                    g = g + early[1][:, n0 * 128:n1 * 128]
                    u = u + early[1][:, FM1 + n0 * 128:FM1 + n1 * 128]
                hs.append((n0, n1, _lhs(hidden(g, u))))
            for n in range(nm, nm + nv):
                hs.append((n, n + 1, _lhs(hidden(vpu_cols(xc, ("g", n)), vpu_cols(xc, ("u", n))))))
            yv = None
            for n in range(FT - nr, FT):
                for t in range(16):
                    g, u = [jnp.sum(w_t[wt_slot[w, n], t * 8:(t + 1) * 8, :] * xc,
                                    axis=-1, keepdims=True) for w in "gu"]
                    r = (n - FT + NR) * 128 + t * 8
                    cc = hidden(g, u) * wd_f[r:r + 8, :]
                    yv = cc if yv is None else yv + cc
            y = None
            for n0, n1, h in hs:
                d = _dot(h, _unpack(wd_p[n0 * 64:n1 * 64, :]))[0:8]
                y = d if y is None else y + d
            hall = jnp.concatenate([h[0:8].astype(_F32) for _, _, h in hs], axis=1)
            my = lane_mean_part(hall * rmd_v[:, 0:(FT - nr) * 128])
            if yv is not None:
                yv = jnp.sum(yv, axis=0, keepdims=True)
                y = y + yv[:, 0:D]
                my = my + yv[:, D:]
            gate = gate * rstd
            return x + xc * rstd + y * gate, m + my * gate

        for cp in w_copies[0]:
            cp.wait()
        repack(wq_r, wq_p, 16)

        def wqf_go(t, _):
            for (c, i), n in wqf_slot.items():
                r = pl.multiple_of(i * 128 + t * 16, 16)
                wq_f[n, pl.ds(pl.multiple_of(t * 16, 16), 16), :] = (
                    wq_r[pl.ds(r, 16), c * DP:(c + 1) * DP].astype(_F32))
            return 0
        lax.fori_loop(0, 8, wqf_go, 0)

        xs_v[...] = jnp.zeros(xs_v.shape, _F32)
        xs_v[0:B, :] = x_v[...].astype(_F32)
        wr = wr_v[...].astype(_F32).reshape(1, D)
        xc0 = xs_v[...] - jnp.mean(xs_v[...], axis=-1, keepdims=True)
        qs0 = _rstd(xc0) * qscale
        xb0 = _lhs(xc0)

        def q1_go(g, _):
            col = pl.ds(pl.multiple_of(g * GP * DP, 128), GP * DP)
            q1_v[:, col] = _dot(xb0, _unpack(wq_p[:, col]))[0:8] * qs0
            return 0
        lax.fori_loop(0, NG, q1_go, 0)

        for cp in w_copies[1]:
            cp.wait()

        def wo_go(n, _):
            g = n // GI
            i = n % GI
            for j in range(NJ):
                r = pl.multiple_of((n * NJ + j) * 16, 16)
                wo_p[g, j, pl.ds(pl.multiple_of(i * 8, 8), 8), :] = _pack(wo_r[pl.ds(r, 16), :])
            return 0
        lax.fori_loop(0, NG * GI, wo_go, 0)

        def wof_go(t, _):
            for (c, i), n in wof_slot.items():
                r = pl.multiple_of(c * DP + i * 128 + t * 16, 16)
                wo_f[n, pl.ds(pl.multiple_of(t * 16, 16), 16), :] = with_mean(wo_r[pl.ds(r, 16), :])
            return 0
        lax.fori_loop(0, 8, wof_go, 0)

        def wlf_go(i, _):
            for j in range(NJ):
                r = pl.multiple_of((((NG - 1) * GI + i) * NJ + j) * 16, 16)
                wl_f[j, i] = with_mean(wo_r[pl.ds(r, 16), :])
            return 0
        lax.fori_loop(0, GI, wlf_go, 0)
        row_means(wo_r, rmo_v)

        for cp in w_copies[2]:
            cp.wait()
        repack(wg_r, wg_p, 64)
        repack(wu_r, wu_p, 64)
        repack(wd_r, wd_p, 128)
        transpose_blocks(wg_r, "g")
        transpose_blocks(wu_r, "u")
        row_means(wd_r, rmd_v)

        def wdf_go(i, _):
            r = pl.multiple_of(i * 128, 128)
            wd_f[pl.ds(r, 128), :] = with_mean(wd_r[pl.ds(F - NR * 128 + r, 128), :])
            return 0
        lax.fori_loop(0, NR, wdf_go, 0)

        rows = [wo_r[pl.ds((((NG - 1) * GI + i) * NJ + NJ - 1) * 16, 16), :] for i in range(IA, GI)]
        rows = jnp.concatenate(rows + [jnp.ones((16, D), _BF16)], axis=0)

        def wl2_go(n, _):
            col = pl.multiple_of(n * 128, 128)
            for e, w_p in enumerate((wg_p, wu_p)):
                prod = _dot(rows, _unpack(w_p[:, pl.ds(col, 128)]))
                for i in range(GI - IA):
                    wl2_f[i, :, pl.ds(pl.multiple_of(e * FM1 + col, 128), 128)] = (
                        prod[i * 16:(i + 1) * 16]
                        - wl_f[NJ - 1, IA + i, :, D:] * prod[(GI - IA) * 16:])
            return 0
        lax.fori_loop(0, FM1 // 128, wl2_go, 0)

        def attention3(x, m):
            xc = x - tile_d(m)
            qs8 = _rstd(xc) * qscale
            xb = _lhs(xc)
            xcol = {i: jnp.broadcast_to(xc[0:1, i * 128:(i + 1) * 128], (128, 128)).T
                    for i in range(DT - max(ka.values()), DT)}

            def stage_a(c):
                km = (DT - ka[c]) * 128
                q = _dot(xb[:, 0:km], _unpack(wq_p[0:km // 2, c * DP:(c + 1) * DP]))[0:8]
                if ka[c]:
                    a = None
                    for i in range(DT - ka[c], DT):
                        for t in range(16):
                            xx = xcol[i][t * 8:(t + 1) * 8, :]
                            cc = (jnp.concatenate([xx] * (DP // 128), axis=1)
                                  * wq_f[wqf_slot[c, i], t * 8:(t + 1) * 8, :])
                            a = cc if a is None else a + cc
                    q = q + jnp.sum(a, axis=0, keepdims=True)
                return q * qs8

            def v_rows(c, t):
                g, j, i = chunk_pos(c, t)
                if g == NG - 1 and j == NJ - 1 and i >= IA:
                    return vraw[g % NS, i, j].astype(_F32)
                return vf[g, j, i]

            def stage_c(p, linv, c, wide):
                nt = (3 - bd[c]) * 8
                head = lambda t: t // (PT // 2)
                chunk = lambda t: pv_chunk(p[head(t) * 8:head(t) * 8 + 8], v_rows(c, t))
                o = None
                if nt:
                    l0 = jnp.broadcast_to(linv[0:8], (8, 128))
                    l1 = jnp.broadcast_to(linv[8:16], (8, 128))
                    li = [l0, jnp.where(low_half, l0, l1), l1][0:nt // 8]
                    o = _lhs(_row_sums8([chunk(t) for t in range(nt)])
                             * jnp.concatenate(li, axis=1))
                tot = None
                for hh in range(2):
                    a = None
                    for t in range(nt, PT):
                        if head(t) != hh:
                            continue
                        r = (t % 8) * 16
                        cc = vpu_out(chunk(t), wo_f[wof_slot[c, t // 8], r:r + 16, 0:wide])
                        a = cc if a is None else a + cc
                    if a is not None:
                        a = a * linv[hh * 8:hh * 8 + 8]
                        tot = a if tot is None else tot + a
                return o, tot

            def stage_d(o, c):
                ws = []
                for t in range(o.shape[1] // 16):
                    g, j, i = chunk_pos(c, t)
                    ws.append(wo_p[g, j, i * 8:(i + 1) * 8, :])
                return _dot(o, _unpack(jnp.concatenate(ws, axis=0)))[0:8]

            def add(a, b):
                return b if a is None else a + b

            acc = accl = accm = accw = None
            qs, ss, ps, ls, os_ = {}, {}, {}, {}, {}
            off = dict(A=cfg["SA"], B=cfg["SB"], M=cfg["SM"], S=cfg["SS"], C=0)
            for step in range(-cfg["SA"], max(dpos) + 1):
                for st in cfg["order"]:
                    if st == "D":
                        for n in range(NC):
                            if dpos[n] == step and os_[n] is not None:
                                o, c = os_[n], perm[n]
                                accl = add(accl, stage_d(o, c))
                                rm = rmo_v[:, c * DP:c * DP + o.shape[1]]
                                accm = add(accm, _lane_fold(o[0:8].astype(_F32) * rm))
                        continue
                    n = step + off[st]
                    if not 0 <= n < NC:
                        continue
                    c = perm[n]
                    if st == "A":
                        qs[n] = stage_a(c)
                    elif st == "B":
                        ss[n] = scores(qs[n], _unpack(kp[c]))
                    elif st == "M":
                        ps[n] = probs(ss[n])
                    elif st == "S":
                        ls[n] = inv_sum(ps[n])
                    elif st == "C":
                        late = n >= NC - cfg["LM"]
                        os_[n], part = stage_c(ps[n], ls[n], c, D + 128 if late else D)
                        if part is not None and late:
                            accw = add(accw, part)
                        elif part is not None:
                            acc = add(acc, part)
            if acc is not None:
                accm = accm + _lane_fold(acc) * (1.0 / D)
                accl = accl + acc
            tot = jnp.concatenate([accl, lane_mean_part(accm)], axis=1)
            if accw is not None:
                tot = tot + accw
            tot = jnp.sum(tot, axis=0, keepdims=True)
            return x + tot[:, 0:D], m + tot[:, D:]

        def batch(b, _):
            @pl.when(b > 0)
            def _():
                for cp in v_copies(b, (NG - 1 + NS) % NG):
                    cp.start()

            def group_probs(g, s, static):
                for cp in k_copies(b, g):
                    cp.wait()
                linvs = []
                for i in range(GP):
                    c = g * GP + i
                    col = c * DP if static else pl.multiple_of(c * DP, 128)
                    q = jnp.broadcast_to(q1_v[pl.ds(b, 1), pl.ds(col, DP)], (8, DP))
                    kk = kraw[s, i * PI:(i + 1) * PI].reshape(DP, W)
                    kp[c] = _pack(kk)
                    p = probs(scores(q, kk))
                    p_v[i] = p
                    linvs.append(inv_sum(p))
                start_next(k_copies, b, g)
                return linvs

            def head_probs(i):
                h = i // HI
                return p_v[h // 2, (h % 2) * 8:(h % 2) * 8 + 8, :]

            def piece(g, s, j, li):
                parts = []
                for i in range(GI):
                    vv = vraw[s, i, j].astype(_F32)
                    vf[g, j, i] = vv
                    parts.append(pv_chunk(head_probs(i), vv))
                o = _lhs(_row_sums(parts) * li)
                return _dot(o, _unpack(wo_p[g, j]))[0:8]

            def group(g, acc):
                s = g % NS
                linvs = group_probs(g, s, False)
                lane = lax.broadcasted_iota(jnp.int32, (8, GI * 16), 1)
                li = jnp.broadcast_to(linvs[0][0:8], (8, GI * 16))
                for h in range(1, 2 * GP):
                    li = jnp.where(lane >= h * HI * 16,
                                   linvs[h // 2][(h % 2) * 8:(h % 2) * 8 + 8], li)
                for cp in v_copies(b, g):
                    cp.wait()
                for j in range(NJ):
                    acc = acc + piece(g, s, j, li)

                @pl.when(g == NG - 1 - NS)
                def _():
                    for cp in v_last_copies(b):
                        cp.start()

                @pl.when(g != NG - 1 - NS)
                def _():
                    start_next(v_copies, b, g)
                return acc

            x = lax.fori_loop(0, NG - 1, group, jnp.broadcast_to(xs_v[pl.ds(b, 1), :], (8, D)))
            g = NG - 1
            s = g % NS
            m = lane_mean_part(x) * (1.0 / D)
            linvs = group_probs(g, s, True)
            tot = None
            for cp, (j, i0, i1) in zip(v_last_copies(b), last_parts):
                final = j == NJ - 1 and i0 == IA
                if final:
                    tot = jnp.sum(tot, axis=0, keepdims=True)
                    x = x + tot[:, 0:D]
                    m = m + tot[:, D:]
                    xc_early = x - tile_d(m)
                    tot = None
                cp.wait()
                for h in range(GI // HI):
                    a = None
                    for i in range(max(i0, h * HI), min(i1, (h + 1) * HI)):
                        vv = vraw[s, i, j].astype(_F32)
                        w = wl_f[j, i]
                        if final:
                            w = jnp.concatenate([w, wl2_f[i - IA]], axis=1)
                        else:
                            vf[g, j, i] = vv
                        cc = vpu_out(pv_chunk(head_probs(i), vv), w)
                        a = cc if a is None else a + cc
                    if a is not None:
                        a = a * linvs[h // 2][(h % 2) * 8:(h % 2) * 8 + 8]
                        tot = a if tot is None else tot + a
            tot = jnp.sum(tot, axis=0, keepdims=True)
            x = x + tot[:, 0:D]
            m = m + tot[:, D:D + 128]

            x, m = ffn(x, m, wr, nv1, nr1, (xc_early, tot[:, D + 128:]))
            x, m = attention3(x, m)
            x, _ = ffn(x, m, wr, nv, nr)
            xs = jnp.where(lax.broadcasted_iota(jnp.int32, (8, D), 0) == b, x, xs_v[...])
            xs_v[...] = xs
            o_ref[...] = xs[0:B].astype(o_ref.dtype)
            return 0

        lax.fori_loop(0, B, batch, 0)

    any_spec = pl.BlockSpec(memory_space=pl.ANY)
    out = pl.pallas_call(
        kernel,
        in_specs=[any_spec] * 9,
        out_specs=pl.BlockSpec(memory_space=pltpu.VMEM),
        out_shape=jax.ShapeDtypeStruct((B, D), A_x.dtype),
        scratch_shapes=[
            pltpu.VMEM((NS, GI, NJ, 16, W), _BF16),
            pltpu.VMEM((NS, GI, NJ, 16, W), _BF16),
            pltpu.VMEM((NC, DP // 2, W), _U32),
            pltpu.VMEM((NG, NJ, GI, 16, W), _F32),
            pltpu.VMEM((D, H * Dh), _BF16),
            pltpu.VMEM((H * Dh, D), _BF16),
            pltpu.VMEM((D, F), _BF16),
            pltpu.VMEM((D, F), _BF16),
            pltpu.VMEM((F, D), _BF16),
            pltpu.VMEM((D // 2, H * Dh), _U32),
            pltpu.VMEM((NG, NJ, GI * 8, D), _U32),
            pltpu.VMEM((D // 2, F), _U32),
            pltpu.VMEM((D // 2, F), _U32),
            pltpu.VMEM((F // 2, D), _U32),
            pltpu.VMEM((max(len(wqf_slot), 1), 128, DP), _F32),
            pltpu.VMEM((max(len(wof_slot), 1), 128, D + 128), _F32),
            pltpu.VMEM((NJ, GI, 16, D + 128), _F32),
            pltpu.VMEM((GI - IA, 16, 2 * FM1), _F32),
            pltpu.VMEM((max(NR, 1) * 128, D + 128), _F32),
            pltpu.VMEM((max(len(wt_slot), 1), 128, D), _F32),
            pltpu.VMEM((B, D), _BF16),
            pltpu.VMEM((D,), _BF16),
            pltpu.VMEM((8, D), _F32),
            pltpu.VMEM((8, H * Dh), _F32),
            pltpu.VMEM((GP, 16, W), _F32),
            pltpu.VMEM((8, H * Dh), _F32),
            pltpu.VMEM((8, F), _F32),
            pltpu.SemaphoreType.DMA((NS,)),
            pltpu.SemaphoreType.DMA((NS,)),
            pltpu.SemaphoreType.DMA((len(last_parts),)),
        ],
        compiler_params=_compiler_params(),
    )(
        A_x.reshape(B, D),
        jnp.swapaxes(A_k_cache, 2, 3).reshape(B, NG, GI, NJ, 16, Sk),
        jnp.swapaxes(A_v_cache, 2, 3).reshape(B, NG, GI, NJ, 16, Sk),
        A_wq, A_wo, B_w_r, B_w_gate, B_w_up, B_w_down,
    )
    return out.reshape(B, Sq, D)


@jax.jit
def pallas_interleave_layers__sliding_block_cached__moe_arch_mod__decode_kernel(
    A_x: jax.Array,
    A_k_cache: jax.Array,
    A_v_cache: jax.Array,
    A_wq: jax.Array,
    A_wo: jax.Array,
    B_x: jax.Array,
    B_w_r: jax.Array,
    B_w_gate: jax.Array,
    B_w_up: jax.Array,
    B_w_down: jax.Array,
):
    return _forward(_CFG, A_x, A_k_cache, A_v_cache, A_wq, A_wo,
                    B_w_r, B_w_gate, B_w_up, B_w_down)
```

```python
import jax
import jax.numpy as jnp
from jax import lax
import jax.experimental.pallas as pl
import jax.experimental.pallas.tpu as pltpu

_F32 = jnp.float32
_BF16 = jnp.bfloat16
_U32 = jnp.uint32
_LOG2E = 1.4426950408889634

_CFG = dict(
    SA=4, SB=3, SM=2, SS=0, order="MSCADB",
    rot=10,
    ka="0212011001211011",
    bd="2112031210111203",
    sd="3241372502331263",
    LM=1,
    NJ=6,
    cuts=(0, 3, 8),
    nv=5, nr=2, fgrp=3,
    nv1=2, nr1=3,
)


def _pack(x):
    return pltpu.bitcast(x, _U32)


def _unpack(x):
    return pltpu.bitcast(x, _BF16)


def _dot(a, b):
    return jnp.dot(a, b, preferred_element_type=_F32)


def _dot_t(a, b):
    return lax.dot_general(a, b, (((1,), (1,)), ((), ())), preferred_element_type=_F32)


def _lhs(x8):
    return jnp.concatenate([x8, x8], axis=0).astype(_BF16)


def _lane_fold(x):
    a = x[:, 0:128]
    for j in range(1, x.shape[1] // 128):
        a = a + x[:, j * 128:(j + 1) * 128]
    return a


def _row_sums(parts):
    return jnp.sum(jnp.concatenate(parts, axis=0).T, axis=0, keepdims=True)


def _row_sums8(parts):
    t = jnp.concatenate(parts, axis=0).T
    a = t[0:8]
    for i in range(1, 16):
        a = a + t[i * 8:(i + 1) * 8]
    return a


def _rstd(xc):
    return lax.rsqrt(jnp.mean(xc * xc, axis=-1, keepdims=True) + 1e-5)


def _compiler_params():
    limit = 120 * 1024 * 1024
    try:
        return pltpu.CompilerParams(vmem_limit_bytes=limit, disable_semaphore_checks=True)
    except TypeError:
        return pltpu.CompilerParams(vmem_limit_bytes=limit)


def _forward(cfg, A_x, A_k_cache, A_v_cache, A_wq, A_wo, B_w_r, B_w_gate, B_w_up, B_w_down):
    B, Sq, D = A_x.shape
    _, H, Sk, Dh = A_k_cache.shape
    F = B_w_gate.shape[1]
    W = min(4096, max(256, Sk // 4))
    assert Sq == 1 and H == 32 and Dh == 192 and B <= 8 and D % 128 == 0 and F % 128 == 0
    DP = 2 * Dh
    NC = H // 2
    DT = D // 128
    FT = F // 128
    NJ = cfg["NJ"]
    GP = 2
    NG = NC // GP
    GI = GP * DP // (16 * NJ)
    PI = GI // GP
    HI = PI // 2
    PT = DP // 16
    NS = 4
    cuts = cfg["cuts"]
    IA = cuts[-2]
    last_parts = [(j, 0, GI) for j in range(NJ - 1)]
    last_parts += [(NJ - 1, i0, i1) for i0, i1 in zip(cuts[:-1], cuts[1:])]
    qscale = float(Dh) ** -0.5 * _LOG2E

    perm = [(cfg["rot"] + n) % NC for n in range(NC)]
    ka = {perm[n]: int(c) for n, c in enumerate(cfg["ka"])}
    bd = {perm[n]: int(c) for n, c in enumerate(cfg["bd"])}
    dpos = [n + int(c, 16) for n, c in enumerate(cfg["sd"])]
    nv, nr, nv1, nr1 = cfg["nv"], cfg["nr"], cfg["nv1"], cfg["nr1"]
    NR = max(nr, nr1)
    FM1 = (FT - nv1 - nr1) * 128

    def slots(keys):
        return {key: n for n, key in enumerate(keys)}
    wqf_slot = slots((c, i) for c in range(NC) for i in range(DT - ka[c], DT))
    wof_slot = slots((c, i) for c in range(NC) for i in range(3 - bd[c], 3))
    wt_slot = slots((w, n) for n in range(FT - max(nv + nr, nv1 + nr1), FT) for w in "gu")

    def chunk_pos(c, t):
        return c // GP, t % NJ, (c % GP) * PI + t // NJ

    def kernel(x_hbm, k_hbm, v_hbm, wq_hbm, wo_hbm, wr_hbm, wg_hbm, wu_hbm, wd_hbm,
               o_ref,
               kraw, vraw, kp, vf,
               wq_r, wo_r, wg_r, wu_r, wd_r,
               wq_p, wo_p, wg_p, wu_p, wd_p, wq_f, wo_f, wl_f, wl2_f, wd_f, w_t,
               x_v, wr_v, xs_v, q1_v, p_v, rmo_v, rmd_v,
               ksem, vsem, lsem):

        def k_copies(b, g):
            s = g % NS
            return [pltpu.make_async_copy(
                k_hbm.at[b, g, :, j, :, pl.ds(Sk - W, W)], kraw.at[s, :, j],
                ksem.at[s]) for j in range(NJ)]

        def v_copies(b, g):
            s = g % NS
            return [pltpu.make_async_copy(
                v_hbm.at[b, g, :, j, :, pl.ds(Sk - W, W)], vraw.at[s, :, j],
                vsem.at[s]) for j in range(NJ)]

        def v_last_copies(b):
            g = NG - 1
            return [pltpu.make_async_copy(
                v_hbm.at[b, g, pl.ds(i0, i1 - i0), j, :, pl.ds(Sk - W, W)],
                vraw.at[g % NS, pl.ds(i0, i1 - i0), j], lsem.at[e])
                for e, (j, i0, i1) in enumerate(last_parts)]

        def start_next(copies, b, g):
            n = b * NG + g + NS

            @pl.when(n < B * NG)
            def _():
                for cp in copies(n // NG, n % NG):
                    cp.start()

        w_sets = [
            [(wq_hbm, wq_r), (x_hbm, x_v), (wr_hbm, wr_v)],
            [(wo_hbm, wo_r)],
            [(wg_hbm, wg_r), (wu_hbm, wu_r), (wd_hbm, wd_r)],
        ]
        w_copies = [[pltpu.make_async_copy(src, dst, lsem.at[i]) for src, dst in ws]
                    for i, ws in enumerate(w_sets)]
        for ws in w_copies:
            for cp in ws:
                cp.start()

        def start0(g, _):
            for cp in k_copies(0, g) + v_copies(0, g):
                cp.start()
            return 0
        lax.fori_loop(0, NS, start0, 0)

        def repack(raw, packed, rows):
            def go(i, _):
                r = pl.multiple_of(i * rows, rows)
                r2 = pl.multiple_of(i * (rows // 2), rows // 2)
                packed[pl.ds(r2, rows // 2), :] = _pack(raw[pl.ds(r, rows), :])
                return 0
            lax.fori_loop(0, raw.shape[0] // rows, go, 0)

        def transpose_blocks(raw, name):
            keys = [key for key in wt_slot if key[0] == name]
            if keys:
                def go(i, _):
                    r = pl.multiple_of(i * 128, 128)
                    for key in keys:
                        blk = raw[pl.ds(r, 128), key[1] * 128:(key[1] + 1) * 128]
                        w_t[wt_slot[key], :, pl.ds(r, 128)] = blk.astype(_F32).T
                    return 0
                lax.fori_loop(0, DT, go, 0)

        def row_means(raw, dst):
            ones = jnp.ones((16, D), _BF16)

            def go(i, _):
                r = pl.multiple_of(i * 512, 512)
                dst[:, pl.ds(r, 512)] = _dot_t(ones, raw[pl.ds(r, 512), :])[0:8] * (1.0 / D)
                return 0
            lax.fori_loop(0, raw.shape[0] // 512, go, 0)

        def with_mean(rows):
            w = rows.astype(_F32)
            m = jnp.mean(w, axis=-1, keepdims=True)
            return jnp.concatenate([w, jnp.broadcast_to(m, (w.shape[0], 128))], axis=1)

        low_half = lax.broadcasted_iota(jnp.int32, (8, 128), 1) < 64

        def tile_d(m):
            return jnp.concatenate([m] * DT, axis=1)

        def lane_mean_part(x):
            return jnp.broadcast_to(jnp.sum(_lane_fold(x), axis=-1, keepdims=True), (8, 128))

        def scores(q, kk):
            mid = q[:, 128:256]
            mid = jnp.concatenate([jnp.where(low_half, mid, 0.0), jnp.where(low_half, 0.0, mid)],
                                  axis=0).astype(_BF16)
            s0 = _dot(_lhs(q[:, 0:128]), kk[0:128])
            s1 = _dot(mid, kk[128:256])
            s2 = _dot(_lhs(q[:, 256:384]), kk[256:384])
            return s1 + jnp.concatenate([s0[0:8], s2[8:16]], axis=0)

        def probs(s):
            return jnp.exp2(s - jnp.max(s, axis=-1, keepdims=True))

        def inv_sum(p):
            l = jnp.sum(p, axis=-1, keepdims=True)
            r = pl.reciprocal(l, approx=True)
            return r * (2.0 - l * r)

        def pv_chunk(pp, vv):
            return _lane_fold(vv * jnp.concatenate([pp, pp], axis=0))

        def vpu_out(part, w):
            cc = jnp.sum(part, axis=1, keepdims=True) * w
            return cc[0:8] + cc[8:16]

        def vpu_cols(xc, key):
            parts = [_lane_fold(w_t[wt_slot[key], t * 8:(t + 1) * 8, :] * xc) for t in range(16)]
            return jnp.broadcast_to(_row_sums(parts), (8, 128))

        def ffn(x, m, wr, nv, nr, early=None):
            xc = x - tile_d(m)
            rstd = _rstd(xc)
            half = 0.5 * rstd
            gate = jax.nn.sigmoid(jnp.sum(xc * wr, axis=-1, keepdims=True) * rstd)

            def hidden(g, u):
                a = g * half
                return (a + a * jnp.tanh(a)) * u

            xb = _lhs(xc if early is None else early[0])
            nm = FT - nv - nr
            hs = []
            for n0 in range(0, nm, cfg["fgrp"]):
                n1 = min(nm, n0 + cfg["fgrp"])
                g = _dot(xb, _unpack(wg_p[:, n0 * 128:n1 * 128]))[0:8]
                u = _dot(xb, _unpack(wu_p[:, n0 * 128:n1 * 128]))[0:8]
                if early is not None:
                    g = g + early[1][:, n0 * 128:n1 * 128]
                    u = u + early[1][:, FM1 + n0 * 128:FM1 + n1 * 128]
                hs.append((n0, n1, _lhs(hidden(g, u))))
            for n in range(nm, nm + nv):
                hs.append((n, n + 1, _lhs(hidden(vpu_cols(xc, ("g", n)), vpu_cols(xc, ("u", n))))))
            yv = None
            for n in range(FT - nr, FT):
                for t in range(16):
                    g, u = [jnp.sum(w_t[wt_slot[w, n], t * 8:(t + 1) * 8, :] * xc,
                                    axis=-1, keepdims=True) for w in "gu"]
                    r = (n - FT + NR) * 128 + t * 8
                    cc = hidden(g, u) * wd_f[r:r + 8, :]
                    yv = cc if yv is None else yv + cc
            y = None
            for n0, n1, h in hs:
                d = _dot(h, _unpack(wd_p[n0 * 64:n1 * 64, :]))[0:8]
                y = d if y is None else y + d
            hall = jnp.concatenate([h[0:8].astype(_F32) for _, _, h in hs], axis=1)
            my = lane_mean_part(hall * rmd_v[:, 0:(FT - nr) * 128])
            if yv is not None:
                yv = jnp.sum(yv, axis=0, keepdims=True)
                y = y + yv[:, 0:D]
                my = my + yv[:, D:]
            gate = gate * rstd
            return x + xc * rstd + y * gate, m + my * gate

        for cp in w_copies[0]:
            cp.wait()
        repack(wq_r, wq_p, 16)

        def wqf_go(t, _):
            for (c, i), n in wqf_slot.items():
                r = pl.multiple_of(i * 128 + t * 16, 16)
                wq_f[n, pl.ds(pl.multiple_of(t * 16, 16), 16), :] = (
                    wq_r[pl.ds(r, 16), c * DP:(c + 1) * DP].astype(_F32))
            return 0
        lax.fori_loop(0, 8, wqf_go, 0)

        xs_v[...] = jnp.zeros(xs_v.shape, _F32)
        xs_v[0:B, :] = x_v[...].astype(_F32)
        wr = wr_v[...].astype(_F32).reshape(1, D)
        xc0 = xs_v[...] - jnp.mean(xs_v[...], axis=-1, keepdims=True)
        qs0 = _rstd(xc0) * qscale
        xb0 = _lhs(xc0)

        def q1_go(g, _):
            col = pl.ds(pl.multiple_of(g * GP * DP, 128), GP * DP)
            q1_v[:, col] = _dot(xb0, _unpack(wq_p[:, col]))[0:8] * qs0
            return 0
        lax.fori_loop(0, NG, q1_go, 0)

        for cp in w_copies[1]:
            cp.wait()

        def wo_go(n, _):
            g = n // GI
            i = n % GI
            for j in range(NJ):
                r = pl.multiple_of((n * NJ + j) * 16, 16)
                wo_p[g, j, pl.ds(pl.multiple_of(i * 8, 8), 8), :] = _pack(wo_r[pl.ds(r, 16), :])
            return 0
        lax.fori_loop(0, NG * GI, wo_go, 0)

        def wof_go(t, _):
            for (c, i), n in wof_slot.items():
                r = pl.multiple_of(c * DP + i * 128 + t * 16, 16)
                wo_f[n, pl.ds(pl.multiple_of(t * 16, 16), 16), :] = with_mean(wo_r[pl.ds(r, 16), :])
            return 0
        lax.fori_loop(0, 8, wof_go, 0)

        def wlf_go(i, _):
            for j in range(NJ):
                r = pl.multiple_of((((NG - 1) * GI + i) * NJ + j) * 16, 16)
                wl_f[j, i] = with_mean(wo_r[pl.ds(r, 16), :])
            return 0
        lax.fori_loop(0, GI, wlf_go, 0)
        row_means(wo_r, rmo_v)

        for cp in w_copies[2]:
            cp.wait()
        repack(wg_r, wg_p, 64)
        repack(wu_r, wu_p, 64)
        repack(wd_r, wd_p, 128)
        transpose_blocks(wg_r, "g")
        transpose_blocks(wu_r, "u")
        row_means(wd_r, rmd_v)

        def wdf_go(i, _):
            r = pl.multiple_of(i * 128, 128)
            wd_f[pl.ds(r, 128), :] = with_mean(wd_r[pl.ds(F - NR * 128 + r, 128), :])
            return 0
        lax.fori_loop(0, NR, wdf_go, 0)

        rows = [wo_r[pl.ds((((NG - 1) * GI + i) * NJ + NJ - 1) * 16, 16), :] for i in range(IA, GI)]
        rows = jnp.concatenate(rows + [jnp.ones((16, D), _BF16)], axis=0)

        def wl2_go(n, _):
            col = pl.multiple_of(n * 128, 128)
            for e, w_p in enumerate((wg_p, wu_p)):
                prod = _dot(rows, _unpack(w_p[:, pl.ds(col, 128)]))
                for i in range(GI - IA):
                    wl2_f[i, :, pl.ds(pl.multiple_of(e * FM1 + col, 128), 128)] = (
                        prod[i * 16:(i + 1) * 16]
                        - wl_f[NJ - 1, IA + i, :, D:] * prod[(GI - IA) * 16:])
            return 0
        lax.fori_loop(0, FM1 // 128, wl2_go, 0)

        def attention3(x, m):
            xc = x - tile_d(m)
            qs8 = _rstd(xc) * qscale
            xb = _lhs(xc)
            xcol = {i: jnp.broadcast_to(xc[0:1, i * 128:(i + 1) * 128], (128, 128)).T
                    for i in range(DT - max(ka.values()), DT)}

            def stage_a(c):
                km = (DT - ka[c]) * 128
                q = _dot(xb[:, 0:km], _unpack(wq_p[0:km // 2, c * DP:(c + 1) * DP]))[0:8]
                if ka[c]:
                    a = None
                    for i in range(DT - ka[c], DT):
                        for t in range(16):
                            xx = xcol[i][t * 8:(t + 1) * 8, :]
                            cc = (jnp.concatenate([xx] * (DP // 128), axis=1)
                                  * wq_f[wqf_slot[c, i], t * 8:(t + 1) * 8, :])
                            a = cc if a is None else a + cc
                    q = q + jnp.sum(a, axis=0, keepdims=True)
                return q * qs8

            def v_rows(c, t):
                g, j, i = chunk_pos(c, t)
                if g == NG - 1 and j == NJ - 1 and i >= IA:
                    return vraw[g % NS, i, j].astype(_F32)
                return vf[g, j, i]

            def stage_c(p, linv, c, wide):
                nt = (3 - bd[c]) * 8
                head = lambda t: t // (PT // 2)
                chunk = lambda t: pv_chunk(p[head(t) * 8:head(t) * 8 + 8], v_rows(c, t))
                o = None
                if nt:
                    l0 = jnp.broadcast_to(linv[0:8], (8, 128))
                    l1 = jnp.broadcast_to(linv[8:16], (8, 128))
                    li = [l0, jnp.where(low_half, l0, l1), l1][0:nt // 8]
                    o = _lhs(_row_sums8([chunk(t) for t in range(nt)])
                             * jnp.concatenate(li, axis=1))
                tot = None
                for hh in range(2):
                    a = None
                    for t in range(nt, PT):
                        if head(t) != hh:
                            continue
                        r = (t % 8) * 16
                        cc = vpu_out(chunk(t), wo_f[wof_slot[c, t // 8], r:r + 16, 0:wide])
                        a = cc if a is None else a + cc
                    if a is not None:
                        a = a * linv[hh * 8:hh * 8 + 8]
                        tot = a if tot is None else tot + a
                return o, tot

            def stage_d(o, c):
                ws = []
                for t in range(o.shape[1] // 16):
                    g, j, i = chunk_pos(c, t)
                    ws.append(wo_p[g, j, i * 8:(i + 1) * 8, :])
                return _dot(o, _unpack(jnp.concatenate(ws, axis=0)))[0:8]

            def add(a, b):
                return b if a is None else a + b

            acc = accl = accm = accw = None
            qs, ss, ps, ls, os_ = {}, {}, {}, {}, {}
            off = dict(A=cfg["SA"], B=cfg["SB"], M=cfg["SM"], S=cfg["SS"], C=0)
            for step in range(-cfg["SA"], max(dpos) + 1):
                for st in cfg["order"]:
                    if st == "D":
                        for n in range(NC):
                            if dpos[n] == step and os_[n] is not None:
                                o, c = os_[n], perm[n]
                                accl = add(accl, stage_d(o, c))
                                rm = rmo_v[:, c * DP:c * DP + o.shape[1]]
                                accm = add(accm, _lane_fold(o[0:8].astype(_F32) * rm))
                        continue
                    n = step + off[st]
                    if not 0 <= n < NC:
                        continue
                    c = perm[n]
                    if st == "A":
                        qs[n] = stage_a(c)
                    elif st == "B":
                        ss[n] = scores(qs[n], _unpack(kp[c]))
                    elif st == "M":
                        ps[n] = probs(ss[n])
                    elif st == "S":
                        ls[n] = inv_sum(ps[n])
                    elif st == "C":
                        late = n >= NC - cfg["LM"]
                        os_[n], part = stage_c(ps[n], ls[n], c, D + 128 if late else D)
                        if part is not None and late:
                            accw = add(accw, part)
                        elif part is not None:
                            acc = add(acc, part)
            if acc is not None:
                accm = accm + _lane_fold(acc) * (1.0 / D)
                accl = accl + acc
            tot = jnp.concatenate([accl, lane_mean_part(accm)], axis=1)
            if accw is not None:
                tot = tot + accw
            tot = jnp.sum(tot, axis=0, keepdims=True)
            return x + tot[:, 0:D], m + tot[:, D:]

        def batch(b, _):
            @pl.when(b > 0)
            def _():
                for cp in v_copies(b, (NG - 1 + NS) % NG):
                    cp.start()

            def group_probs(g, s, static):
                for cp in k_copies(b, g):
                    cp.wait()
                linvs = []
                for i in range(GP):
                    c = g * GP + i
                    col = c * DP if static else pl.multiple_of(c * DP, 128)
                    q = jnp.broadcast_to(q1_v[pl.ds(b, 1), pl.ds(col, DP)], (8, DP))
                    kk = kraw[s, i * PI:(i + 1) * PI].reshape(DP, W)
                    kp[c] = _pack(kk)
                    p = probs(scores(q, kk))
                    p_v[i] = p
                    linvs.append(inv_sum(p))
                start_next(k_copies, b, g)
                return linvs

            def head_probs(i):
                h = i // HI
                return p_v[h // 2, (h % 2) * 8:(h % 2) * 8 + 8, :]

            def piece(g, s, j, li):
                parts = []
                for i in range(GI):
                    vv = vraw[s, i, j].astype(_F32)
                    vf[g, j, i] = vv
                    parts.append(pv_chunk(head_probs(i), vv))
                o = _lhs(_row_sums(parts) * li)
                return _dot(o, _unpack(wo_p[g, j]))[0:8]

            def group(g, acc):
                s = g % NS
                linvs = group_probs(g, s, False)
                lane = lax.broadcasted_iota(jnp.int32, (8, GI * 16), 1)
                li = jnp.broadcast_to(linvs[0][0:8], (8, GI * 16))
                for h in range(1, 2 * GP):
                    li = jnp.where(lane >= h * HI * 16,
                                   linvs[h // 2][(h % 2) * 8:(h % 2) * 8 + 8], li)
                for cp in v_copies(b, g):
                    cp.wait()
                for j in range(NJ):
                    acc = acc + piece(g, s, j, li)

                @pl.when(g == NG - 1 - NS)
                def _():
                    for cp in v_last_copies(b):
                        cp.start()

                @pl.when(g != NG - 1 - NS)
                def _():
                    start_next(v_copies, b, g)
                return acc

            x = lax.fori_loop(0, NG - 1, group, jnp.broadcast_to(xs_v[pl.ds(b, 1), :], (8, D)))
            g = NG - 1
            s = g % NS
            m = lane_mean_part(x) * (1.0 / D)
            linvs = group_probs(g, s, True)
            tot = None
            for cp, (j, i0, i1) in zip(v_last_copies(b), last_parts):
                final = j == NJ - 1 and i0 == IA
                if final:
                    tot = jnp.sum(tot, axis=0, keepdims=True)
                    x = x + tot[:, 0:D]
                    m = m + tot[:, D:]
                    xc_early = x - tile_d(m)
                    tot = None
                cp.wait()
                for h in range(GI // HI):
                    a = None
                    for i in range(max(i0, h * HI), min(i1, (h + 1) * HI)):
                        vv = vraw[s, i, j].astype(_F32)
                        w = wl_f[j, i]
                        if final:
                            w = jnp.concatenate([w, wl2_f[i - IA]], axis=1)
                        else:
                            vf[g, j, i] = vv
                        cc = vpu_out(pv_chunk(head_probs(i), vv), w)
                        a = cc if a is None else a + cc
                    if a is not None:
                        a = a * linvs[h // 2][(h % 2) * 8:(h % 2) * 8 + 8]
                        tot = a if tot is None else tot + a
            tot = jnp.sum(tot, axis=0, keepdims=True)
            x = x + tot[:, 0:D]
            m = m + tot[:, D:D + 128]

            x, m = ffn(x, m, wr, nv1, nr1, (xc_early, tot[:, D + 128:]))
            x, m = attention3(x, m)
            x, _ = ffn(x, m, wr, nv, nr)
            xs = jnp.where(lax.broadcasted_iota(jnp.int32, (8, D), 0) == b, x, xs_v[...])
            xs_v[...] = xs
            o_ref[...] = xs[0:B].astype(o_ref.dtype)
            return 0

        lax.fori_loop(0, B, batch, 0)

    any_spec = pl.BlockSpec(memory_space=pl.ANY)
    out = pl.pallas_call(
        kernel,
        in_specs=[any_spec] * 9,
        out_specs=pl.BlockSpec(memory_space=pltpu.VMEM),
        out_shape=jax.ShapeDtypeStruct((B, D), A_x.dtype),
        scratch_shapes=[
            pltpu.VMEM((NS, GI, NJ, 16, W), _BF16),
            pltpu.VMEM((NS, GI, NJ, 16, W), _BF16),
            pltpu.VMEM((NC, DP // 2, W), _U32),
            pltpu.VMEM((NG, NJ, GI, 16, W), _F32),
            pltpu.VMEM((D, H * Dh), _BF16),
            pltpu.VMEM((H * Dh, D), _BF16),
            pltpu.VMEM((D, F), _BF16),
            pltpu.VMEM((D, F), _BF16),
            pltpu.VMEM((F, D), _BF16),
            pltpu.VMEM((D // 2, H * Dh), _U32),
            pltpu.VMEM((NG, NJ, GI * 8, D), _U32),
            pltpu.VMEM((D // 2, F), _U32),
            pltpu.VMEM((D // 2, F), _U32),
            pltpu.VMEM((F // 2, D), _U32),
            pltpu.VMEM((max(len(wqf_slot), 1), 128, DP), _F32),
            pltpu.VMEM((max(len(wof_slot), 1), 128, D + 128), _F32),
            pltpu.VMEM((NJ, GI, 16, D + 128), _F32),
            pltpu.VMEM((GI - IA, 16, 2 * FM1), _F32),
            pltpu.VMEM((max(NR, 1) * 128, D + 128), _F32),
            pltpu.VMEM((max(len(wt_slot), 1), 128, D), _F32),
            pltpu.VMEM((B, D), _BF16),
            pltpu.VMEM((D,), _BF16),
            pltpu.VMEM((8, D), _F32),
            pltpu.VMEM((8, H * Dh), _F32),
            pltpu.VMEM((GP, 16, W), _F32),
            pltpu.VMEM((8, H * Dh), _F32),
            pltpu.VMEM((8, F), _F32),
            pltpu.SemaphoreType.DMA((NS,)),
            pltpu.SemaphoreType.DMA((NS,)),
            pltpu.SemaphoreType.DMA((len(last_parts),)),
        ],
        compiler_params=_compiler_params(),
    )(
        A_x.reshape(B, D),
        jnp.swapaxes(A_k_cache, 2, 3).reshape(B, NG, GI, NJ, 16, Sk),
        jnp.swapaxes(A_v_cache, 2, 3).reshape(B, NG, GI, NJ, 16, Sk),
        A_wq, A_wo, B_w_r, B_w_gate, B_w_up, B_w_down,
    )
    return out.reshape(B, Sq, D)


@jax.jit
def pallas_interleave_layers__sliding_block_cached__moe_arch_mod__decode_kernel(
    A_x: jax.Array,
    A_k_cache: jax.Array,
    A_v_cache: jax.Array,
    A_wq: jax.Array,
    A_wo: jax.Array,
    B_x: jax.Array,
    B_w_r: jax.Array,
    B_w_gate: jax.Array,
    B_w_up: jax.Array,
    B_w_down: jax.Array,
):
    return _forward(_CFG, A_x, A_k_cache, A_v_cache, A_wq, A_wo,
                    B_w_r, B_w_gate, B_w_up, B_w_down)
```

```python
import jax
import jax.numpy as jnp
from jax import lax
import jax.experimental.pallas as pl
import jax.experimental.pallas.tpu as pltpu

_F32 = jnp.float32
_BF16 = jnp.bfloat16
_U32 = jnp.uint32
_LOG2E = 1.4426950408889634

_CFG = dict(
    SA=4, SB=3, SM=2, SS=0, order="MSCADB",
    rot=6,
    ka="0212011001211011",
    bd="2112031211122103",
    sd="3241371504331463",
    LM=1,
    cuts=(0, 7, 12),
    nv=5, nr=2, fgrp=3,
    nv1=2, nr1=3,
)


def _pack(x):
    return pltpu.bitcast(x, _U32)


def _unpack(x):
    return pltpu.bitcast(x, _BF16)


def _dot(a, b):
    return jnp.dot(a, b, preferred_element_type=_F32)


def _dot_t(a, b):
    return lax.dot_general(a, b, (((1,), (1,)), ((), ())), preferred_element_type=_F32)


def _lhs(x8):
    return jnp.concatenate([x8, x8], axis=0).astype(_BF16)


def _lane_fold(x):
    a = x[:, 0:128]
    for j in range(1, x.shape[1] // 128):
        a = a + x[:, j * 128:(j + 1) * 128]
    return a


def _row_sums(parts):
    return jnp.sum(jnp.concatenate(parts, axis=0).T, axis=0, keepdims=True)


def _row_sums8(parts):
    t = jnp.concatenate(parts, axis=0).T
    a = t[0:8]
    for i in range(1, 16):
        a = a + t[i * 8:(i + 1) * 8]
    return a


def _rstd(xc):
    return lax.rsqrt(jnp.mean(xc * xc, axis=-1, keepdims=True) + 1e-5)


def _compiler_params():
    limit = 120 * 1024 * 1024
    try:
        return pltpu.CompilerParams(vmem_limit_bytes=limit, disable_semaphore_checks=True)
    except TypeError:
        return pltpu.CompilerParams(vmem_limit_bytes=limit)


def _forward(cfg, A_x, A_k_cache, A_v_cache, A_wq, A_wo, B_w_r, B_w_gate, B_w_up, B_w_down):
    B, Sq, D = A_x.shape
    _, H, Sk, Dh = A_k_cache.shape
    F = B_w_gate.shape[1]
    W = min(4096, max(256, Sk // 4))
    assert Sq == 1 and H == 32 and Dh == 192 and B <= 8 and D % 128 == 0 and F % 128 == 0
    DP = 2 * Dh
    NC = H // 2
    DT = D // 128
    FT = F // 128
    RT = 8
    NJ = RT // 2
    GP = 2
    NG = NC // GP
    GI = GP * DP // (8 * RT)
    PI = GI // GP
    HI = PI // 2
    PT = DP // 16
    NS = 4
    cuts = cfg["cuts"]
    IA = cuts[-2]
    last_parts = [(j, 0, GI) for j in range(NJ - 1)]
    last_parts += [(NJ - 1, i0, i1) for i0, i1 in zip(cuts[:-1], cuts[1:])]
    qscale = float(Dh) ** -0.5 * _LOG2E

    perm = [(cfg["rot"] + n) % NC for n in range(NC)]
    ka = {perm[n]: int(c) for n, c in enumerate(cfg["ka"])}
    bd = {perm[n]: int(c) for n, c in enumerate(cfg["bd"])}
    dpos = [n + int(c, 16) for n, c in enumerate(cfg["sd"])]
    nv, nr, nv1, nr1 = cfg["nv"], cfg["nr"], cfg["nv1"], cfg["nr1"]
    NR = max(nr, nr1)
    FM1 = (FT - nv1 - nr1) * 128

    def slots(keys):
        return {key: n for n, key in enumerate(keys)}
    wqf_slot = slots((c, i) for c in range(NC) for i in range(DT - ka[c], DT))
    wof_slot = slots((c, i) for c in range(NC) for i in range(3 - bd[c], 3))
    wt_slot = slots((w, n) for n in range(FT - max(nv + nr, nv1 + nr1), FT) for w in "gu")

    def kernel(x_hbm, k_hbm, v_hbm, wq_hbm, wo_hbm, wr_hbm, wg_hbm, wu_hbm, wd_hbm,
               o_ref,
               kraw, vraw, kp, vf,
               wq_r, wo_r, wg_r, wu_r, wd_r,
               wq_p, wo_p, wg_p, wu_p, wd_p, wq_f, wo_f, wl_f, wl2_f, wd_f, w_t,
               x_v, wr_v, xs_v, q1_v, p_v, rmo_v, rmd_v,
               ksem, vsem, lsem):

        def k_copies(b, g):
            s = g % NS
            return [pltpu.make_async_copy(
                k_hbm.at[b, g, :, j, :, pl.ds(Sk - W, W)], kraw.at[s, :, j],
                ksem.at[s]) for j in range(RT)]

        def v_copies(b, g):
            s = g % NS
            return [pltpu.make_async_copy(
                v_hbm.at[b, g, :, j, :, pl.ds(Sk - W, W)], vraw.at[s, :, j],
                vsem.at[s]) for j in range(RT)]

        def v_last_copies(b):
            g = NG - 1
            return [[pltpu.make_async_copy(
                v_hbm.at[b, g, pl.ds(i0, i1 - i0), t, :, pl.ds(Sk - W, W)],
                vraw.at[g % NS, pl.ds(i0, i1 - i0), t], lsem.at[e]) for t in (2 * j, 2 * j + 1)]
                for e, (j, i0, i1) in enumerate(last_parts)]

        def v_chunk(s, i, j):
            return jnp.concatenate([vraw[s, i, t].astype(_F32) for t in (2 * j, 2 * j + 1)], axis=0)

        def start_next(copies, b, g):
            n = b * NG + g + NS

            @pl.when(n < B * NG)
            def _():
                for cp in copies(n // NG, n % NG):
                    cp.start()

        w_sets = [
            [(wq_hbm, wq_r), (x_hbm, x_v), (wr_hbm, wr_v)],
            [(wo_hbm, wo_r)],
            [(wg_hbm, wg_r), (wu_hbm, wu_r), (wd_hbm, wd_r)],
        ]
        w_copies = [[pltpu.make_async_copy(src, dst, lsem.at[i]) for src, dst in ws]
                    for i, ws in enumerate(w_sets)]
        for ws in w_copies:
            for cp in ws:
                cp.start()

        def start0(g, _):
            for cp in k_copies(0, g) + v_copies(0, g):
                cp.start()
            return 0
        lax.fori_loop(0, NS, start0, 0)

        def repack(raw, packed, rows):
            def go(i, _):
                r = pl.multiple_of(i * rows, rows)
                r2 = pl.multiple_of(i * (rows // 2), rows // 2)
                packed[pl.ds(r2, rows // 2), :] = _pack(raw[pl.ds(r, rows), :])
                return 0
            lax.fori_loop(0, raw.shape[0] // rows, go, 0)

        def transpose_blocks(raw, name):
            keys = [key for key in wt_slot if key[0] == name]
            if keys:
                def go(i, _):
                    r = pl.multiple_of(i * 128, 128)
                    for key in keys:
                        blk = raw[pl.ds(r, 128), key[1] * 128:(key[1] + 1) * 128]
                        w_t[wt_slot[key], :, pl.ds(r, 128)] = blk.astype(_F32).T
                    return 0
                lax.fori_loop(0, DT, go, 0)

        def row_means(raw, dst):
            ones = jnp.ones((16, D), _BF16)

            def go(i, _):
                r = pl.multiple_of(i * 512, 512)
                dst[:, pl.ds(r, 512)] = _dot_t(ones, raw[pl.ds(r, 512), :])[0:8] * (1.0 / D)
                return 0
            lax.fori_loop(0, raw.shape[0] // 512, go, 0)

        def with_mean(rows):
            w = rows.astype(_F32)
            m = jnp.mean(w, axis=-1, keepdims=True)
            return jnp.concatenate([w, jnp.broadcast_to(m, (w.shape[0], 128))], axis=1)

        low_half = lax.broadcasted_iota(jnp.int32, (8, 128), 1) < 64

        def tile_d(m):
            return jnp.concatenate([m] * DT, axis=1)

        def lane_mean_part(x):
            return jnp.broadcast_to(jnp.sum(_lane_fold(x), axis=-1, keepdims=True), (8, 128))

        def scores(q, kk):
            mid = q[:, 128:256]
            mid = jnp.concatenate([jnp.where(low_half, mid, 0.0), jnp.where(low_half, 0.0, mid)],
                                  axis=0).astype(_BF16)
            s0 = _dot(_lhs(q[:, 0:128]), kk[0:128])
            s1 = _dot(mid, kk[128:256])
            s2 = _dot(_lhs(q[:, 256:384]), kk[256:384])
            return s1 + jnp.concatenate([s0[0:8], s2[8:16]], axis=0)

        def probs(s):
            return jnp.exp2(s - jnp.max(s, axis=-1, keepdims=True))

        def inv_sum(p):
            l = jnp.sum(p, axis=-1, keepdims=True)
            r = pl.reciprocal(l, approx=True)
            return r * (2.0 - l * r)

        def pair_scale(linv):
            l0 = jnp.broadcast_to(linv[0:8], (8, 128))
            l1 = jnp.broadcast_to(linv[8:16], (8, 128))
            return jnp.concatenate([l0, jnp.where(low_half, l0, l1), l1], axis=1)

        def pv_chunk(pp, vv):
            return _lane_fold(vv * jnp.concatenate([pp, pp], axis=0))

        def vpu_out(part, w):
            cc = jnp.sum(part, axis=1, keepdims=True) * w
            return cc[0:8] + cc[8:16]

        def vpu_cols(xc, key):
            parts = [_lane_fold(w_t[wt_slot[key], t * 8:(t + 1) * 8, :] * xc) for t in range(16)]
            return jnp.broadcast_to(_row_sums(parts), (8, 128))

        def ffn(x, m, wr, nv, nr, early=None):
            xc = x - tile_d(m)
            rstd = _rstd(xc)
            half = 0.5 * rstd
            gate = jax.nn.sigmoid(jnp.sum(xc * wr, axis=-1, keepdims=True) * rstd)

            def hidden(g, u):
                a = g * half
                return (a + a * jnp.tanh(a)) * u

            xb = _lhs(xc if early is None else early[0])
            nm = FT - nv - nr
            hs = []
            for n0 in range(0, nm, cfg["fgrp"]):
                n1 = min(nm, n0 + cfg["fgrp"])
                g = _dot(xb, _unpack(wg_p[:, n0 * 128:n1 * 128]))[0:8]
                u = _dot(xb, _unpack(wu_p[:, n0 * 128:n1 * 128]))[0:8]
                if early is not None:
                    g = g + early[1][:, n0 * 128:n1 * 128]
                    u = u + early[1][:, FM1 + n0 * 128:FM1 + n1 * 128]
                hs.append((n0, n1, _lhs(hidden(g, u))))
            for n in range(nm, nm + nv):
                hs.append((n, n + 1, _lhs(hidden(vpu_cols(xc, ("g", n)), vpu_cols(xc, ("u", n))))))
            yv = None
            for n in range(FT - nr, FT):
                for t in range(16):
                    g, u = [jnp.sum(w_t[wt_slot[w, n], t * 8:(t + 1) * 8, :] * xc,
                                    axis=-1, keepdims=True) for w in "gu"]
                    r = (n - FT + NR) * 128 + t * 8
                    cc = hidden(g, u) * wd_f[r:r + 8, :]
                    yv = cc if yv is None else yv + cc
            y = None
            for n0, n1, h in hs:
                d = _dot(h, _unpack(wd_p[n0 * 64:n1 * 64, :]))[0:8]
                y = d if y is None else y + d
            hall = jnp.concatenate([h[0:8].astype(_F32) for _, _, h in hs], axis=1)
            my = lane_mean_part(hall * rmd_v[:, 0:(FT - nr) * 128])
            if yv is not None:
                yv = jnp.sum(yv, axis=0, keepdims=True)
                y = y + yv[:, 0:D]
                my = my + yv[:, D:]
            gate = gate * rstd
            return x + xc * rstd + y * gate, m + my * gate

        for cp in w_copies[0]:
            cp.wait()
        repack(wq_r, wq_p, 16)

        def wqf_go(t, _):
            for (c, i), n in wqf_slot.items():
                r = pl.multiple_of(i * 128 + t * 16, 16)
                wq_f[n, pl.ds(pl.multiple_of(t * 16, 16), 16), :] = (
                    wq_r[pl.ds(r, 16), c * DP:(c + 1) * DP].astype(_F32))
            return 0
        lax.fori_loop(0, 8, wqf_go, 0)

        xs_v[...] = jnp.zeros(xs_v.shape, _F32)
        xs_v[0:B, :] = x_v[...].astype(_F32)
        wr = wr_v[...].astype(_F32).reshape(1, D)
        xc0 = xs_v[...] - jnp.mean(xs_v[...], axis=-1, keepdims=True)
        qs0 = _rstd(xc0) * qscale
        xb0 = _lhs(xc0)

        def q1_go(g, _):
            col = pl.ds(pl.multiple_of(g * GP * DP, 128), GP * DP)
            q1_v[:, col] = _dot(xb0, _unpack(wq_p[:, col]))[0:8] * qs0
            return 0
        lax.fori_loop(0, NG, q1_go, 0)

        for cp in w_copies[1]:
            cp.wait()

        repack(wo_r, wo_p, 128)

        def wof_go(t, _):
            for (c, i), n in wof_slot.items():
                r = pl.multiple_of(c * DP + i * 128 + t * 16, 16)
                wo_f[n, pl.ds(pl.multiple_of(t * 16, 16), 16), :] = with_mean(wo_r[pl.ds(r, 16), :])
            return 0
        lax.fori_loop(0, 8, wof_go, 0)

        def wlf_go(i, _):
            for j in range(NJ):
                r = pl.multiple_of((((NG - 1) * GI + i) * NJ + j) * 16, 16)
                wl_f[j, i] = with_mean(wo_r[pl.ds(r, 16), :])
            return 0
        lax.fori_loop(0, GI, wlf_go, 0)
        row_means(wo_r, rmo_v)

        for cp in w_copies[2]:
            cp.wait()
        repack(wg_r, wg_p, 64)
        repack(wu_r, wu_p, 64)
        repack(wd_r, wd_p, 128)
        transpose_blocks(wg_r, "g")
        transpose_blocks(wu_r, "u")
        row_means(wd_r, rmd_v)

        def wdf_go(i, _):
            r = pl.multiple_of(i * 128, 128)
            wd_f[pl.ds(r, 128), :] = with_mean(wd_r[pl.ds(F - NR * 128 + r, 128), :])
            return 0
        lax.fori_loop(0, NR, wdf_go, 0)

        rows = [wo_r[pl.ds((((NG - 1) * GI + i) * NJ + NJ - 1) * 16, 16), :] for i in range(IA, GI)]
        rows = jnp.concatenate(rows + [jnp.ones((16, D), _BF16)], axis=0)

        def wl2_go(n, _):
            col = pl.multiple_of(n * 128, 128)
            for e, w_p in enumerate((wg_p, wu_p)):
                prod = _dot(rows, _unpack(w_p[:, pl.ds(col, 128)]))
                for i in range(GI - IA):
                    wl2_f[i, :, pl.ds(pl.multiple_of(e * FM1 + col, 128), 128)] = (
                        prod[i * 16:(i + 1) * 16]
                        - wl_f[NJ - 1, IA + i, :, D:] * prod[(GI - IA) * 16:])
            return 0
        lax.fori_loop(0, FM1 // 128, wl2_go, 0)

        def attention3(x, m):
            xc = x - tile_d(m)
            qs8 = _rstd(xc) * qscale
            xb = _lhs(xc)
            xcol = {i: jnp.broadcast_to(xc[0:1, i * 128:(i + 1) * 128], (128, 128)).T
                    for i in range(DT - max(ka.values()), DT)}

            def stage_a(c):
                km = (DT - ka[c]) * 128
                q = _dot(xb[:, 0:km], _unpack(wq_p[0:km // 2, c * DP:(c + 1) * DP]))[0:8]
                if ka[c]:
                    a = None
                    for i in range(DT - ka[c], DT):
                        for t in range(16):
                            xx = xcol[i][t * 8:(t + 1) * 8, :]
                            cc = (jnp.concatenate([xx] * (DP // 128), axis=1)
                                  * wq_f[wqf_slot[c, i], t * 8:(t + 1) * 8, :])
                            a = cc if a is None else a + cc
                    q = q + jnp.sum(a, axis=0, keepdims=True)
                return q * qs8

            def v_rows(c, t):
                i = (c % GP) * PI + t // NJ
                if c // GP == NG - 1 and t % NJ == NJ - 1 and i >= IA:
                    return v_chunk((NG - 1) % NS, i, NJ - 1)
                return vf[c, t]

            def stage_c(p, linv, c, wide):
                nt = (3 - bd[c]) * 8
                head = lambda t: t // (PT // 2)
                chunk = lambda t: pv_chunk(p[head(t) * 8:head(t) * 8 + 8], v_rows(c, t))
                o = None
                if nt:
                    o = _lhs(_row_sums8([chunk(t) for t in range(nt)])
                             * pair_scale(linv)[:, 0:nt * 16])
                tot = None
                for hh in range(2):
                    a = None
                    for t in range(nt, PT):
                        if head(t) != hh:
                            continue
                        r = (t % 8) * 16
                        cc = vpu_out(chunk(t), wo_f[wof_slot[c, t // 8], r:r + 16, 0:wide])
                        a = cc if a is None else a + cc
                    if a is not None:
                        a = a * linv[hh * 8:hh * 8 + 8]
                        tot = a if tot is None else tot + a
                return o, tot

            def stage_d(o, c):
                r = c * DP // 2
                return _dot(o, _unpack(wo_p[r:r + o.shape[1] // 2, :]))[0:8]

            def add(a, b):
                return b if a is None else a + b

            acc = accl = accm = accw = None
            qs, ss, ps, ls, os_ = {}, {}, {}, {}, {}
            off = dict(A=cfg["SA"], B=cfg["SB"], M=cfg["SM"], S=cfg["SS"], C=0)
            for step in range(-cfg["SA"], max(dpos) + 1):
                for st in cfg["order"]:
                    if st == "D":
                        for n in range(NC):
                            if dpos[n] == step and os_[n] is not None:
                                o, c = os_[n], perm[n]
                                accl = add(accl, stage_d(o, c))
                                rm = rmo_v[:, c * DP:c * DP + o.shape[1]]
                                accm = add(accm, _lane_fold(o[0:8].astype(_F32) * rm))
                        continue
                    n = step + off[st]
                    if not 0 <= n < NC:
                        continue
                    c = perm[n]
                    if st == "A":
                        qs[n] = stage_a(c)
                    elif st == "B":
                        ss[n] = scores(qs[n], _unpack(kp[c]))
                    elif st == "M":
                        ps[n] = probs(ss[n])
                    elif st == "S":
                        ls[n] = inv_sum(ps[n])
                    elif st == "C":
                        late = n >= NC - cfg["LM"]
                        os_[n], part = stage_c(ps[n], ls[n], c, D + 128 if late else D)
                        if part is not None and late:
                            accw = add(accw, part)
                        elif part is not None:
                            acc = add(acc, part)
            if acc is not None:
                accm = accm + _lane_fold(acc) * (1.0 / D)
                accl = accl + acc
            tot = jnp.concatenate([accl, lane_mean_part(accm)], axis=1)
            if accw is not None:
                tot = tot + accw
            tot = jnp.sum(tot, axis=0, keepdims=True)
            return x + tot[:, 0:D], m + tot[:, D:]

        def batch(b, _):
            @pl.when(b > 0)
            def _():
                for cp in v_copies(b, (NG - 1 + NS) % NG):
                    cp.start()

            def group_probs(g, s, static):
                for cp in k_copies(b, g):
                    cp.wait()
                linvs = []
                for i in range(GP):
                    c = g * GP + i
                    col = c * DP if static else pl.multiple_of(c * DP, 128)
                    q = jnp.broadcast_to(q1_v[pl.ds(b, 1), pl.ds(col, DP)], (8, DP))
                    kk = kraw[s, i * PI:(i + 1) * PI].reshape(DP, W)
                    kp[c] = _pack(kk)
                    p = probs(scores(q, kk))
                    p_v[i] = p
                    linvs.append(inv_sum(p))
                start_next(k_copies, b, g)
                return linvs

            def head_probs(i):
                h = i // HI
                return p_v[h // 2, (h % 2) * 8:(h % 2) * 8 + 8, :]

            def group(g, acc):
                s = g % NS
                linvs = group_probs(g, s, False)
                for cp in v_copies(b, g):
                    cp.wait()
                for e in range(GP):
                    c = g * GP + e
                    parts = []
                    for t in range(PT):
                        i = e * PI + t // NJ
                        vv = v_chunk(s, i, t % NJ)
                        vf[c, t] = vv
                        parts.append(pv_chunk(head_probs(i), vv))
                    o = _lhs(_row_sums(parts) * pair_scale(linvs[e]))
                    r = pl.multiple_of(c * (DP // 2), 8)
                    acc = acc + _dot(o, _unpack(wo_p[pl.ds(r, DP // 2), :]))[0:8]

                @pl.when(g == NG - 1 - NS)
                def _():
                    for cps in v_last_copies(b):
                        for cp in cps:
                            cp.start()

                @pl.when(g != NG - 1 - NS)
                def _():
                    start_next(v_copies, b, g)
                return acc

            x = lax.fori_loop(0, NG - 1, group, jnp.broadcast_to(xs_v[pl.ds(b, 1), :], (8, D)))
            g = NG - 1
            s = g % NS
            m = lane_mean_part(x) * (1.0 / D)
            linvs = group_probs(g, s, True)
            tot = None
            for cps, (j, i0, i1) in zip(v_last_copies(b), last_parts):
                final = j == NJ - 1 and i0 == IA
                if final:
                    tot = jnp.sum(tot, axis=0, keepdims=True)
                    x = x + tot[:, 0:D]
                    m = m + tot[:, D:]
                    xc_early = x - tile_d(m)
                    tot = None
                for cp in cps:
                    cp.wait()
                for h in range(GI // HI):
                    a = None
                    for i in range(max(i0, h * HI), min(i1, (h + 1) * HI)):
                        vv = v_chunk(s, i, j)
                        w = wl_f[j, i]
                        if final:
                            w = jnp.concatenate([w, wl2_f[i - IA]], axis=1)
                        else:
                            vf[g * GP + i // PI, (i % PI) * NJ + j] = vv
                        cc = vpu_out(pv_chunk(head_probs(i), vv), w)
                        a = cc if a is None else a + cc
                    if a is not None:
                        a = a * linvs[h // 2][(h % 2) * 8:(h % 2) * 8 + 8]
                        tot = a if tot is None else tot + a
            tot = jnp.sum(tot, axis=0, keepdims=True)
            x = x + tot[:, 0:D]
            m = m + tot[:, D:D + 128]

            x, m = ffn(x, m, wr, nv1, nr1, (xc_early, tot[:, D + 128:]))
            x, m = attention3(x, m)
            x, _ = ffn(x, m, wr, nv, nr)
            xs = jnp.where(lax.broadcasted_iota(jnp.int32, (8, D), 0) == b, x, xs_v[...])
            xs_v[...] = xs
            o_ref[...] = xs[0:B].astype(o_ref.dtype)
            return 0

        lax.fori_loop(0, B, batch, 0)

    any_spec = pl.BlockSpec(memory_space=pl.ANY)
    out = pl.pallas_call(
        kernel,
        in_specs=[any_spec] * 9,
        out_specs=pl.BlockSpec(memory_space=pltpu.VMEM),
        out_shape=jax.ShapeDtypeStruct((B, D), A_x.dtype),
        scratch_shapes=[
            pltpu.VMEM((NS, GI, RT, 8, W), _BF16),
            pltpu.VMEM((NS, GI, RT, 8, W), _BF16),
            pltpu.VMEM((NC, DP // 2, W), _U32),
            pltpu.VMEM((NC, PT, 16, W), _F32),
            pltpu.VMEM((D, H * Dh), _BF16),
            pltpu.VMEM((H * Dh, D), _BF16),
            pltpu.VMEM((D, F), _BF16),
            pltpu.VMEM((D, F), _BF16),
            pltpu.VMEM((F, D), _BF16),
            pltpu.VMEM((D // 2, H * Dh), _U32),
            pltpu.VMEM((H * Dh // 2, D), _U32),
            pltpu.VMEM((D // 2, F), _U32),
            pltpu.VMEM((D // 2, F), _U32),
            pltpu.VMEM((F // 2, D), _U32),
            pltpu.VMEM((max(len(wqf_slot), 1), 128, DP), _F32),
            pltpu.VMEM((max(len(wof_slot), 1), 128, D + 128), _F32),
            pltpu.VMEM((NJ, GI, 16, D + 128), _F32),
            pltpu.VMEM((GI - IA, 16, 2 * FM1), _F32),
            pltpu.VMEM((max(NR, 1) * 128, D + 128), _F32),
            pltpu.VMEM((max(len(wt_slot), 1), 128, D), _F32),
            pltpu.VMEM((B, D), _BF16),
            pltpu.VMEM((D,), _BF16),
            pltpu.VMEM((8, D), _F32),
            pltpu.VMEM((8, H * Dh), _F32),
            pltpu.VMEM((GP, 16, W), _F32),
            pltpu.VMEM((8, H * Dh), _F32),
            pltpu.VMEM((8, F), _F32),
            pltpu.SemaphoreType.DMA((NS,)),
            pltpu.SemaphoreType.DMA((NS,)),
            pltpu.SemaphoreType.DMA((len(last_parts),)),
        ],
        compiler_params=_compiler_params(),
    )(
        A_x.reshape(B, D),
        jnp.swapaxes(A_k_cache, 2, 3).reshape(B, NG, GI, RT, 8, Sk),
        jnp.swapaxes(A_v_cache, 2, 3).reshape(B, NG, GI, RT, 8, Sk),
        A_wq, A_wo, B_w_r, B_w_gate, B_w_up, B_w_down,
    )
    return out.reshape(B, Sq, D)


@jax.jit
def pallas_interleave_layers__sliding_block_cached__moe_arch_mod__decode_kernel(
    A_x: jax.Array,
    A_k_cache: jax.Array,
    A_v_cache: jax.Array,
    A_wq: jax.Array,
    A_wo: jax.Array,
    B_x: jax.Array,
    B_w_r: jax.Array,
    B_w_gate: jax.Array,
    B_w_up: jax.Array,
    B_w_down: jax.Array,
):
    return _forward(_CFG, A_x, A_k_cache, A_v_cache, A_wq, A_wo,
                    B_w_r, B_w_gate, B_w_up, B_w_down)
```

```python
import jax
import jax.numpy as jnp
from jax import lax
import jax.experimental.pallas as pl
import jax.experimental.pallas.tpu as pltpu

_F32 = jnp.float32
_BF16 = jnp.bfloat16
_U32 = jnp.uint32
_LOG2E = 1.4426950408889634

_CFG = dict(
    SA=4, SB=3, SM=2, SS=0, order="MSCADB",
    rot=14,
    ka="0212021001211001",
    bd="2112022211121103",
    sd="3331381504532353",
    LM=3,
    cuts=(0, 7, 12),
    nv=5, nr=2, fgrp=3,
    nv1=2, nr1=3,
)


def _pack(x):
    return pltpu.bitcast(x, _U32)


def _unpack(x):
    return pltpu.bitcast(x, _BF16)


def _dot(a, b):
    return jnp.dot(a, b, preferred_element_type=_F32)


def _dot_t(a, b):
    return lax.dot_general(a, b, (((1,), (1,)), ((), ())), preferred_element_type=_F32)


def _lhs(x8):
    return jnp.concatenate([x8, x8], axis=0).astype(_BF16)


def _lane_fold(x):
    a = x[:, 0:128]
    for j in range(1, x.shape[1] // 128):
        a = a + x[:, j * 128:(j + 1) * 128]
    return a


def _row_sums(parts):
    return jnp.sum(jnp.concatenate(parts, axis=0).T, axis=0, keepdims=True)


def _row_sums8(parts):
    t = jnp.concatenate(parts, axis=0).T
    a = t[0:8]
    for i in range(1, 16):
        a = a + t[i * 8:(i + 1) * 8]
    return a


def _rstd(xc):
    return lax.rsqrt(jnp.mean(xc * xc, axis=-1, keepdims=True) + 1e-5)


def _compiler_params():
    limit = 120 * 1024 * 1024
    try:
        return pltpu.CompilerParams(vmem_limit_bytes=limit, disable_semaphore_checks=True)
    except TypeError:
        return pltpu.CompilerParams(vmem_limit_bytes=limit)


def _forward(cfg, A_x, A_k_cache, A_v_cache, A_wq, A_wo, B_w_r, B_w_gate, B_w_up, B_w_down):
    B, Sq, D = A_x.shape
    _, H, Sk, Dh = A_k_cache.shape
    F = B_w_gate.shape[1]
    W = min(4096, max(256, Sk // 4))
    assert Sq == 1 and H == 32 and Dh == 192 and B <= 8 and D % 128 == 0 and F % 128 == 0
    DP = 2 * Dh
    NC = H // 2
    DT = D // 128
    FT = F // 128
    RT = 8
    NJ = RT // 2
    GP = 2
    NG = NC // GP
    GI = GP * DP // (8 * RT)
    PI = GI // GP
    HI = PI // 2
    PT = DP // 16
    NS = 4
    cuts = cfg["cuts"]
    IA = cuts[-2]
    last_parts = [(j, 0, GI) for j in range(NJ - 1)]
    last_parts += [(NJ - 1, i0, i1) for i0, i1 in zip(cuts[:-1], cuts[1:])]
    qscale = float(Dh) ** -0.5 * _LOG2E

    perm = [(cfg["rot"] + n) % NC for n in range(NC)]
    ka = {perm[n]: int(c) for n, c in enumerate(cfg["ka"])}
    bd = {perm[n]: int(c) for n, c in enumerate(cfg["bd"])}
    dpos = [n + int(c, 16) for n, c in enumerate(cfg["sd"])]
    nv, nr, nv1, nr1 = cfg["nv"], cfg["nr"], cfg["nv1"], cfg["nr1"]
    NR = max(nr, nr1)
    FM1 = (FT - nv1 - nr1) * 128

    def slots(keys):
        return {key: n for n, key in enumerate(keys)}
    wqf_slot = slots((c, i) for c in range(NC) for i in range(DT - ka[c], DT))
    wof_slot = slots((c, i) for c in range(NC) for i in range(3 - bd[c], 3))
    wt_slot = slots((w, n) for n in range(FT - max(nv + nr, nv1 + nr1), FT) for w in "gu")

    def kernel(x_hbm, k_hbm, v_hbm, wq_hbm, wo_hbm, wr_hbm, wg_hbm, wu_hbm, wd_hbm,
               o_ref,
               kraw, vraw, kp, vf,
               wq_r, wo_r, wg_r, wu_r, wd_r,
               wq_p, wo_p, wg_p, wu_p, wd_p, wq_f, wo_f, wl_f, wl2_f, wd_f, w_t,
               x_v, wr_v, xs_v, q1_v, p_v, rmo_v, rmd_v,
               ksem, vsem, lsem):

        def k_copies(b, g):
            s = g % NS
            return [pltpu.make_async_copy(
                k_hbm.at[b, g, :, j, :, pl.ds(Sk - W, W)], kraw.at[s, :, j],
                ksem.at[s]) for j in range(RT)]

        def v_copies(b, g):
            s = g % NS
            return [pltpu.make_async_copy(
                v_hbm.at[b, g, :, j, :, pl.ds(Sk - W, W)], vraw.at[s, :, j],
                vsem.at[s]) for j in range(RT)]

        def v_last_copies(b):
            g = NG - 1
            return [[pltpu.make_async_copy(
                v_hbm.at[b, g, pl.ds(i0, i1 - i0), t, :, pl.ds(Sk - W, W)],
                vraw.at[g % NS, pl.ds(i0, i1 - i0), t], lsem.at[e]) for t in (2 * j, 2 * j + 1)]
                for e, (j, i0, i1) in enumerate(last_parts)]

        def v_chunk(s, i, j):
            return jnp.concatenate([vraw[s, i, t].astype(_F32) for t in (2 * j, 2 * j + 1)], axis=0)

        def start_next(copies, b, g):
            n = b * NG + g + NS

            @pl.when(n < B * NG)
            def _():
                for cp in copies(n // NG, n % NG):
                    cp.start()

        w_sets = [
            [(wq_hbm, wq_r), (x_hbm, x_v), (wr_hbm, wr_v)],
            [(wo_hbm, wo_r)],
            [(wg_hbm, wg_r), (wu_hbm, wu_r), (wd_hbm, wd_r)],
        ]
        w_copies = [[pltpu.make_async_copy(src, dst, lsem.at[i]) for src, dst in ws]
                    for i, ws in enumerate(w_sets)]
        for ws in w_copies:
            for cp in ws:
                cp.start()

        def start0(g, _):
            for cp in k_copies(0, g) + v_copies(0, g):
                cp.start()
            return 0
        lax.fori_loop(0, NS, start0, 0)

        def repack(raw, packed, rows):
            def go(i, _):
                r = pl.multiple_of(i * rows, rows)
                r2 = pl.multiple_of(i * (rows // 2), rows // 2)
                packed[pl.ds(r2, rows // 2), :] = _pack(raw[pl.ds(r, rows), :])
                return 0
            lax.fori_loop(0, raw.shape[0] // rows, go, 0)

        def transpose_blocks(raw, name):
            keys = [key for key in wt_slot if key[0] == name]
            if keys:
                def go(i, _):
                    r = pl.multiple_of(i * 128, 128)
                    for key in keys:
                        blk = raw[pl.ds(r, 128), key[1] * 128:(key[1] + 1) * 128]
                        w_t[wt_slot[key], :, pl.ds(r, 128)] = blk.astype(_F32).T
                    return 0
                lax.fori_loop(0, DT, go, 0)

        def row_means(raw, dst):
            ones = jnp.ones((16, D), _BF16)

            def go(i, _):
                r = pl.multiple_of(i * 512, 512)
                dst[:, pl.ds(r, 512)] = _dot_t(ones, raw[pl.ds(r, 512), :])[0:8] * (1.0 / D)
                return 0
            lax.fori_loop(0, raw.shape[0] // 512, go, 0)

        def with_mean(rows):
            w = rows.astype(_F32)
            m = jnp.mean(w, axis=-1, keepdims=True)
            return jnp.concatenate([w, jnp.broadcast_to(m, (w.shape[0], 128))], axis=1)

        low_half = lax.broadcasted_iota(jnp.int32, (8, 128), 1) < 64

        def tile_d(m):
            return jnp.concatenate([m] * DT, axis=1)

        def lane_mean_part(x):
            return jnp.broadcast_to(jnp.sum(_lane_fold(x), axis=-1, keepdims=True), (8, 128))

        def scores(q, kk):
            mid = q[:, 128:256]
            mid = jnp.concatenate([jnp.where(low_half, mid, 0.0), jnp.where(low_half, 0.0, mid)],
                                  axis=0).astype(_BF16)
            s0 = _dot(_lhs(q[:, 0:128]), kk[0:128])
            s1 = _dot(mid, kk[128:256])
            s2 = _dot(_lhs(q[:, 256:384]), kk[256:384])
            return s1 + jnp.concatenate([s0[0:8], s2[8:16]], axis=0)

        def probs(s):
            return jnp.exp2(s - jnp.max(s, axis=-1, keepdims=True))

        def inv_sum(p):
            l = jnp.sum(p, axis=-1, keepdims=True)
            r = pl.reciprocal(l, approx=True)
            return r * (2.0 - l * r)

        def pair_scale(linv):
            l0 = jnp.broadcast_to(linv[0:8], (8, 128))
            l1 = jnp.broadcast_to(linv[8:16], (8, 128))
            return jnp.concatenate([l0, jnp.where(low_half, l0, l1), l1], axis=1)

        def pv_chunk(pp, vv):
            return _lane_fold(vv * jnp.concatenate([pp, pp], axis=0))

        def vpu_out(part, w):
            cc = jnp.sum(part, axis=1, keepdims=True) * w
            return cc[0:8] + cc[8:16]

        def vpu_cols(xc, key):
            parts = [_lane_fold(w_t[wt_slot[key], t * 8:(t + 1) * 8, :] * xc) for t in range(16)]
            return jnp.broadcast_to(_row_sums(parts), (8, 128))

        def ffn(x, m, wr, nv, nr, early=None):
            xc = x - tile_d(m)
            rstd = _rstd(xc)
            half = 0.5 * rstd
            gate = jax.nn.sigmoid(jnp.sum(xc * wr, axis=-1, keepdims=True) * rstd)

            def hidden(g, u):
                a = g * half
                return (a + a * jnp.tanh(a)) * u

            xb = _lhs(xc if early is None else early[0])
            nm = FT - nv - nr
            hs = []
            for n0 in range(0, nm, cfg["fgrp"]):
                n1 = min(nm, n0 + cfg["fgrp"])
                g = _dot(xb, _unpack(wg_p[:, n0 * 128:n1 * 128]))[0:8]
                u = _dot(xb, _unpack(wu_p[:, n0 * 128:n1 * 128]))[0:8]
                if early is not None:
                    g = g + early[1][:, n0 * 128:n1 * 128]
                    u = u + early[1][:, FM1 + n0 * 128:FM1 + n1 * 128]
                hs.append((n0, n1, _lhs(hidden(g, u))))
            for n in range(nm, nm + nv):
                hs.append((n, n + 1, _lhs(hidden(vpu_cols(xc, ("g", n)), vpu_cols(xc, ("u", n))))))
            yv = None
            for n in range(FT - nr, FT):
                for t in range(16):
                    g, u = [jnp.sum(w_t[wt_slot[w, n], t * 8:(t + 1) * 8, :] * xc,
                                    axis=-1, keepdims=True) for w in "gu"]
                    r = (n - FT + NR) * 128 + t * 8
                    cc = hidden(g, u) * wd_f[r:r + 8, :]
                    yv = cc if yv is None else yv + cc
            y = None
            for n0, n1, h in hs:
                d = _dot(h, _unpack(wd_p[n0 * 64:n1 * 64, :]))[0:8]
                y = d if y is None else y + d
            hall = jnp.concatenate([h[0:8].astype(_F32) for _, _, h in hs], axis=1)
            my = lane_mean_part(hall * rmd_v[:, 0:(FT - nr) * 128])
            if yv is not None:
                yv = jnp.sum(yv, axis=0, keepdims=True)
                y = y + yv[:, 0:D]
                my = my + yv[:, D:]
            gate = gate * rstd
            return x + xc * rstd + y * gate, m + my * gate

        for cp in w_copies[0]:
            cp.wait()
        repack(wq_r, wq_p, 16)

        def wqf_go(t, _):
            for (c, i), n in wqf_slot.items():
                r = pl.multiple_of(i * 128 + t * 16, 16)
                wq_f[n, pl.ds(pl.multiple_of(t * 16, 16), 16), :] = (
                    wq_r[pl.ds(r, 16), c * DP:(c + 1) * DP].astype(_F32))
            return 0
        lax.fori_loop(0, 8, wqf_go, 0)

        xs_v[...] = jnp.zeros(xs_v.shape, _F32)
        xs_v[0:B, :] = x_v[...].astype(_F32)
        wr = wr_v[...].astype(_F32).reshape(1, D)
        xc0 = xs_v[...] - jnp.mean(xs_v[...], axis=-1, keepdims=True)
        qs0 = _rstd(xc0) * qscale
        xb0 = _lhs(xc0)

        def q1_go(g, _):
            col = pl.ds(pl.multiple_of(g * GP * DP, 128), GP * DP)
            q1_v[:, col] = _dot(xb0, _unpack(wq_p[:, col]))[0:8] * qs0
            return 0
        lax.fori_loop(0, NG, q1_go, 0)

        for cp in w_copies[1]:
            cp.wait()

        repack(wo_r, wo_p, 128)

        def wof_go(t, _):
            for (c, i), n in wof_slot.items():
                r = pl.multiple_of(c * DP + i * 128 + t * 16, 16)
                wo_f[n, pl.ds(pl.multiple_of(t * 16, 16), 16), :] = with_mean(wo_r[pl.ds(r, 16), :])
            return 0
        lax.fori_loop(0, 8, wof_go, 0)

        def wlf_go(i, _):
            for j in range(NJ):
                r = pl.multiple_of((((NG - 1) * GI + i) * NJ + j) * 16, 16)
                wl_f[j, i] = with_mean(wo_r[pl.ds(r, 16), :])
            return 0
        lax.fori_loop(0, GI, wlf_go, 0)
        row_means(wo_r, rmo_v)

        for cp in w_copies[2]:
            cp.wait()
        repack(wg_r, wg_p, 64)
        repack(wu_r, wu_p, 64)
        repack(wd_r, wd_p, 128)
        transpose_blocks(wg_r, "g")
        transpose_blocks(wu_r, "u")
        row_means(wd_r, rmd_v)

        def wdf_go(i, _):
            r = pl.multiple_of(i * 128, 128)
            wd_f[pl.ds(r, 128), :] = with_mean(wd_r[pl.ds(F - NR * 128 + r, 128), :])
            return 0
        lax.fori_loop(0, NR, wdf_go, 0)

        rows = [wo_r[pl.ds((((NG - 1) * GI + i) * NJ + NJ - 1) * 16, 16), :] for i in range(IA, GI)]
        rows = jnp.concatenate(rows + [jnp.ones((16, D), _BF16)], axis=0)

        def wl2_go(n, _):
            col = pl.multiple_of(n * 128, 128)
            for e, w_p in enumerate((wg_p, wu_p)):
                prod = _dot(rows, _unpack(w_p[:, pl.ds(col, 128)]))
                for i in range(GI - IA):
                    wl2_f[i, :, pl.ds(pl.multiple_of(e * FM1 + col, 128), 128)] = (
                        prod[i * 16:(i + 1) * 16]
                        - wl_f[NJ - 1, IA + i, :, D:] * prod[(GI - IA) * 16:])
            return 0
        lax.fori_loop(0, FM1 // 128, wl2_go, 0)

        def attention3(x, m):
            xc = x - tile_d(m)
            qs8 = _rstd(xc) * qscale
            xb = _lhs(xc)
            xcol = {i: jnp.broadcast_to(xc[0:1, i * 128:(i + 1) * 128], (128, 128)).T
                    for i in range(DT - max(ka.values()), DT)}

            def stage_a(c):
                km = (DT - ka[c]) * 128
                q = _dot(xb[:, 0:km], _unpack(wq_p[0:km // 2, c * DP:(c + 1) * DP]))[0:8]
                if ka[c]:
                    a = None
                    for i in range(DT - ka[c], DT):
                        for t in range(16):
                            xx = xcol[i][t * 8:(t + 1) * 8, :]
                            cc = (jnp.concatenate([xx] * (DP // 128), axis=1)
                                  * wq_f[wqf_slot[c, i], t * 8:(t + 1) * 8, :])
                            a = cc if a is None else a + cc
                    q = q + jnp.sum(a, axis=0, keepdims=True)
                return q * qs8

            def v_rows(c, t):
                i = (c % GP) * PI + t // NJ
                if c // GP == NG - 1 and t % NJ == NJ - 1 and i >= IA:
                    return v_chunk((NG - 1) % NS, i, NJ - 1)
                return vf[c, t]

            def stage_c(p, linv, c, wide):
                nt = (3 - bd[c]) * 8
                head = lambda t: t // (PT // 2)
                chunk = lambda t: pv_chunk(p[head(t) * 8:head(t) * 8 + 8], v_rows(c, t))
                o = None
                if nt:
                    o = _lhs(_row_sums8([chunk(t) for t in range(nt)])
                             * pair_scale(linv)[:, 0:nt * 16])
                tot = None
                for hh in range(2):
                    a = None
                    for t in range(nt, PT):
                        if head(t) != hh:
                            continue
                        r = (t % 8) * 16
                        cc = vpu_out(chunk(t), wo_f[wof_slot[c, t // 8], r:r + 16, 0:wide])
                        a = cc if a is None else a + cc
                    if a is not None:
                        a = a * linv[hh * 8:hh * 8 + 8]
                        tot = a if tot is None else tot + a
                return o, tot

            def stage_d(o, c):
                r = c * DP // 2
                return _dot(o, _unpack(wo_p[r:r + o.shape[1] // 2, :]))[0:8]

            def add(a, b):
                return b if a is None else a + b

            acc = accl = accm = accw = None
            qs, ss, ps, ls, os_ = {}, {}, {}, {}, {}
            off = dict(A=cfg["SA"], B=cfg["SB"], M=cfg["SM"], S=cfg["SS"], C=0)
            for step in range(-cfg["SA"], max(dpos) + 1):
                for st in cfg["order"]:
                    if st == "D":
                        for n in range(NC):
                            if dpos[n] == step and os_[n] is not None:
                                o, c = os_[n], perm[n]
                                accl = add(accl, stage_d(o, c))
                                rm = rmo_v[:, c * DP:c * DP + o.shape[1]]
                                accm = add(accm, _lane_fold(o[0:8].astype(_F32) * rm))
                        continue
                    n = step + off[st]
                    if not 0 <= n < NC:
                        continue
                    c = perm[n]
                    if st == "A":
                        qs[n] = stage_a(c)
                    elif st == "B":
                        ss[n] = scores(qs[n], _unpack(kp[c]))
                    elif st == "M":
                        ps[n] = probs(ss[n])
                    elif st == "S":
                        ls[n] = inv_sum(ps[n])
                    elif st == "C":
                        late = n >= NC - cfg["LM"]
                        os_[n], part = stage_c(ps[n], ls[n], c, D + 128 if late else D)
                        if part is not None and late:
                            accw = add(accw, part)
                        elif part is not None:
                            acc = add(acc, part)
            if acc is not None:
                accm = accm + _lane_fold(acc) * (1.0 / D)
                accl = accl + acc
            tot = jnp.concatenate([accl, lane_mean_part(accm)], axis=1)
            if accw is not None:
                tot = tot + accw
            tot = jnp.sum(tot, axis=0, keepdims=True)
            return x + tot[:, 0:D], m + tot[:, D:]

        def batch(b, _):
            @pl.when(b > 0)
            def _():
                for cp in v_copies(b, (NG - 1 + NS) % NG):
                    cp.start()

            def group_probs(g, s, static):
                for cp in k_copies(b, g):
                    cp.wait()
                for i in range(GP):
                    c = g * GP + i
                    col = c * DP if static else pl.multiple_of(c * DP, 128)
                    q = jnp.broadcast_to(q1_v[pl.ds(b, 1), pl.ds(col, DP)], (8, DP))
                    kk = kraw[s, i * PI:(i + 1) * PI].reshape(DP, W)
                    kp[c] = _pack(kk)
                    p = probs(scores(q, kk))
                    p_v[i] = p * inv_sum(p)
                start_next(k_copies, b, g)

            def head_probs(i):
                h = i // HI
                return p_v[h // 2, (h % 2) * 8:(h % 2) * 8 + 8, :]

            def group(g, acc):
                s = g % NS
                group_probs(g, s, False)
                for cp in v_copies(b, g):
                    cp.wait()
                for e in range(GP):
                    c = g * GP + e
                    parts = []
                    for t in range(PT):
                        i = e * PI + t // NJ
                        vv = v_chunk(s, i, t % NJ)
                        vf[c, t] = vv
                        parts.append(pv_chunk(head_probs(i), vv))
                    o = _lhs(jnp.broadcast_to(_row_sums(parts), (8, DP)))
                    r = pl.multiple_of(c * (DP // 2), 8)
                    acc = acc + _dot(o, _unpack(wo_p[pl.ds(r, DP // 2), :]))[0:8]

                @pl.when(g == NG - 1 - NS)
                def _():
                    for cps in v_last_copies(b):
                        for cp in cps:
                            cp.start()

                @pl.when(g != NG - 1 - NS)
                def _():
                    start_next(v_copies, b, g)
                return acc

            x = lax.fori_loop(0, NG - 1, group, jnp.broadcast_to(xs_v[pl.ds(b, 1), :], (8, D)))
            g = NG - 1
            s = g % NS
            m = lane_mean_part(x) * (1.0 / D)
            group_probs(g, s, True)
            tot = None
            for cps, (j, i0, i1) in zip(v_last_copies(b), last_parts):
                final = j == NJ - 1 and i0 == IA
                if final:
                    tot = jnp.sum(tot, axis=0, keepdims=True)
                    x = x + tot[:, 0:D]
                    m = m + tot[:, D:]
                    xc_early = x - tile_d(m)
                    tot = None
                for cp in cps:
                    cp.wait()
                for i in range(i0, i1):
                    vv = v_chunk(s, i, j)
                    w = wl_f[j, i]
                    if final:
                        w = jnp.concatenate([w, wl2_f[i - IA]], axis=1)
                    else:
                        vf[g * GP + i // PI, (i % PI) * NJ + j] = vv
                    cc = vpu_out(pv_chunk(head_probs(i), vv), w)
                    tot = cc if tot is None else tot + cc
            tot = jnp.sum(tot, axis=0, keepdims=True)
            x = x + tot[:, 0:D]
            m = m + tot[:, D:D + 128]

            x, m = ffn(x, m, wr, nv1, nr1, (xc_early, tot[:, D + 128:]))
            x, m = attention3(x, m)
            x, _ = ffn(x, m, wr, nv, nr)
            xs = jnp.where(lax.broadcasted_iota(jnp.int32, (8, D), 0) == b, x, xs_v[...])
            xs_v[...] = xs
            o_ref[...] = xs[0:B].astype(o_ref.dtype)
            return 0

        lax.fori_loop(0, B, batch, 0)

    any_spec = pl.BlockSpec(memory_space=pl.ANY)
    out = pl.pallas_call(
        kernel,
        in_specs=[any_spec] * 9,
        out_specs=pl.BlockSpec(memory_space=pltpu.VMEM),
        out_shape=jax.ShapeDtypeStruct((B, D), A_x.dtype),
        scratch_shapes=[
            pltpu.VMEM((NS, GI, RT, 8, W), _BF16),
            pltpu.VMEM((NS, GI, RT, 8, W), _BF16),
            pltpu.VMEM((NC, DP // 2, W), _U32),
            pltpu.VMEM((NC, PT, 16, W), _F32),
            pltpu.VMEM((D, H * Dh), _BF16),
            pltpu.VMEM((H * Dh, D), _BF16),
            pltpu.VMEM((D, F), _BF16),
            pltpu.VMEM((D, F), _BF16),
            pltpu.VMEM((F, D), _BF16),
            pltpu.VMEM((D // 2, H * Dh), _U32),
            pltpu.VMEM((H * Dh // 2, D), _U32),
            pltpu.VMEM((D // 2, F), _U32),
            pltpu.VMEM((D // 2, F), _U32),
            pltpu.VMEM((F // 2, D), _U32),
            pltpu.VMEM((max(len(wqf_slot), 1), 128, DP), _F32),
            pltpu.VMEM((max(len(wof_slot), 1), 128, D + 128), _F32),
            pltpu.VMEM((NJ, GI, 16, D + 128), _F32),
            pltpu.VMEM((GI - IA, 16, 2 * FM1), _F32),
            pltpu.VMEM((max(NR, 1) * 128, D + 128), _F32),
            pltpu.VMEM((max(len(wt_slot), 1), 128, D), _F32),
            pltpu.VMEM((B, D), _BF16),
            pltpu.VMEM((D,), _BF16),
            pltpu.VMEM((8, D), _F32),
            pltpu.VMEM((8, H * Dh), _F32),
            pltpu.VMEM((GP, 16, W), _F32),
            pltpu.VMEM((8, H * Dh), _F32),
            pltpu.VMEM((8, F), _F32),
            pltpu.SemaphoreType.DMA((NS,)),
            pltpu.SemaphoreType.DMA((NS,)),
            pltpu.SemaphoreType.DMA((len(last_parts),)),
        ],
        compiler_params=_compiler_params(),
    )(
        A_x.reshape(B, D),
        jnp.swapaxes(A_k_cache, 2, 3).reshape(B, NG, GI, RT, 8, Sk),
        jnp.swapaxes(A_v_cache, 2, 3).reshape(B, NG, GI, RT, 8, Sk),
        A_wq, A_wo, B_w_r, B_w_gate, B_w_up, B_w_down,
    )
    return out.reshape(B, Sq, D)


@jax.jit
def pallas_interleave_layers__sliding_block_cached__moe_arch_mod__decode_kernel(
    A_x: jax.Array,
    A_k_cache: jax.Array,
    A_v_cache: jax.Array,
    A_wq: jax.Array,
    A_wo: jax.Array,
    B_x: jax.Array,
    B_w_r: jax.Array,
    B_w_gate: jax.Array,
    B_w_up: jax.Array,
    B_w_down: jax.Array,
):
    return _forward(_CFG, A_x, A_k_cache, A_v_cache, A_wq, A_wo,
                    B_w_r, B_w_gate, B_w_up, B_w_down)
```

```python
import jax
import jax.numpy as jnp
from jax import lax
import jax.experimental.pallas as pl
import jax.experimental.pallas.tpu as pltpu

_F32 = jnp.float32
_BF16 = jnp.bfloat16
_U32 = jnp.uint32
_LOG2E = 1.4426950408889634

_CFG = dict(
    SA=4, SB=3, SM=2, SS=0, order="MSCADB",
    rot=14,
    ka="0212021001211001",
    bd="2112022211121103",
    sd="3331381504532353",
    LM=3,
    cuts=(0, 7, 12),
    nv=5, nr=2, fgrp=3,
    nv1=2, nr1=3,
)


def _pack(x):
    return pltpu.bitcast(x, _U32)


def _unpack(x):
    return pltpu.bitcast(x, _BF16)


def _dot(a, b):
    return jnp.dot(a, b, preferred_element_type=_F32)


def _dot_t(a, b):
    return lax.dot_general(a, b, (((1,), (1,)), ((), ())), preferred_element_type=_F32)


def _lhs(x8):
    return jnp.concatenate([x8, x8], axis=0).astype(_BF16)


def _lane_fold(x):
    a = x[:, 0:128]
    for j in range(1, x.shape[1] // 128):
        a = a + x[:, j * 128:(j + 1) * 128]
    return a


def _row_sums(parts):
    return jnp.sum(jnp.concatenate(parts, axis=0).T, axis=0, keepdims=True)


def _row_sums8(parts):
    t = jnp.concatenate(parts, axis=0).T
    a = t[0:8]
    for i in range(1, 16):
        a = a + t[i * 8:(i + 1) * 8]
    return a


def _rstd(xc):
    return lax.rsqrt(jnp.mean(xc * xc, axis=-1, keepdims=True) + 1e-5)


def _forward(cfg, A_x, A_k_cache, A_v_cache, A_wq, A_wo, B_w_r, B_w_gate, B_w_up, B_w_down):
    B, Sq, D = A_x.shape
    _, H, Sk, Dh = A_k_cache.shape
    F = B_w_gate.shape[1]
    W = min(4096, max(256, Sk // 4))
    assert Sq == 1 and H == 32 and Dh == 192 and B <= 8 and D % 128 == 0 and F % 128 == 0
    DP = 2 * Dh
    NC = H // 2
    DT = D // 128
    FT = F // 128
    RT = 8
    NJ = RT // 2
    GP = 2
    NG = NC // GP
    GI = GP * DP // (8 * RT)
    PI = GI // GP
    HI = PI // 2
    PT = DP // 16
    NS = 4
    cuts = cfg["cuts"]
    IA = cuts[-2]
    last_parts = [(j, 0, GI) for j in range(NJ - 1)]
    last_parts += [(NJ - 1, i0, i1) for i0, i1 in zip(cuts[:-1], cuts[1:])]
    qscale = float(Dh) ** -0.5 * _LOG2E

    perm = [(cfg["rot"] + n) % NC for n in range(NC)]
    ka = {perm[n]: int(c) for n, c in enumerate(cfg["ka"])}
    bd = {perm[n]: int(c) for n, c in enumerate(cfg["bd"])}
    dpos = [n + int(c, 16) for n, c in enumerate(cfg["sd"])]
    nv, nr, nv1, nr1 = cfg["nv"], cfg["nr"], cfg["nv1"], cfg["nr1"]
    NR = max(nr, nr1)
    FM1 = (FT - nv1 - nr1) * 128

    def slots(keys):
        return {key: n for n, key in enumerate(keys)}
    wqf_slot = slots((c, i) for c in range(NC) for i in range(DT - ka[c], DT))
    wof_slot = slots((c, i) for c in range(NC) for i in range(3 - bd[c], 3))
    wt_slot = slots((w, n) for n in range(FT - max(nv + nr, nv1 + nr1), FT) for w in "gu")

    def kernel(*refs):
        *refs, o_v, osem = refs
        out_copy = pltpu.make_async_copy(o_v, refs[9], osem)

        def scoped(ksem, vsem, lsem):
            body(*refs[:9], o_v, *refs[10:], ksem, vsem, lsem)
            out_copy.start()

        pl.run_scoped(scoped, pltpu.SemaphoreType.DMA((NS,)), pltpu.SemaphoreType.DMA((NS,)),
                      pltpu.SemaphoreType.DMA((len(last_parts),)))
        out_copy.wait()

    def body(x_hbm, k_hbm, v_hbm, wq_hbm, wo_hbm, wr_hbm, wg_hbm, wu_hbm, wd_hbm,
             o_ref,
             kraw, vraw, kp, vf,
             wq_r, wo_r, wg_r, wu_r, wd_r,
             wq_p, wo_p, wg_p, wu_p, wd_p, wq_f, wo_f, wl_f, wl2_f, wd_f, w_t,
             x_v, wr_v, xs_v, q1_v, p_v, rmo_v, rmd_v,
             ksem, vsem, lsem):

        def k_copies(b, g):
            s = g % NS
            return [pltpu.make_async_copy(
                k_hbm.at[b, g, :, j, :, pl.ds(Sk - W, W)], kraw.at[s, :, j],
                ksem.at[s]) for j in range(RT)]

        def v_copies(b, g):
            s = g % NS
            return [pltpu.make_async_copy(
                v_hbm.at[b, g, :, j, :, pl.ds(Sk - W, W)], vraw.at[s, :, j],
                vsem.at[s]) for j in range(RT)]

        def v_last_copies(b):
            g = NG - 1
            return [[pltpu.make_async_copy(
                v_hbm.at[b, g, pl.ds(i0, i1 - i0), t, :, pl.ds(Sk - W, W)],
                vraw.at[g % NS, pl.ds(i0, i1 - i0), t], lsem.at[e]) for t in (2 * j, 2 * j + 1)]
                for e, (j, i0, i1) in enumerate(last_parts)]

        def v_chunk(s, i, j):
            return jnp.concatenate([vraw[s, i, t].astype(_F32) for t in (2 * j, 2 * j + 1)], axis=0)

        def start_next(copies, b, g):
            n = b * NG + g + NS

            @pl.when(n < B * NG)
            def _():
                for cp in copies(n // NG, n % NG):
                    cp.start()

        w_sets = [
            [(wq_hbm, wq_r), (x_hbm, x_v), (wr_hbm, wr_v)],
            [(wo_hbm, wo_r)],
            [(wg_hbm, wg_r), (wu_hbm, wu_r), (wd_hbm, wd_r)],
        ]
        w_copies = [[pltpu.make_async_copy(src, dst, lsem.at[i]) for src, dst in ws]
                    for i, ws in enumerate(w_sets)]
        for ws in w_copies:
            for cp in ws:
                cp.start()

        def start0(g, _):
            for cp in k_copies(0, g) + v_copies(0, g):
                cp.start()
            return 0
        lax.fori_loop(0, NS, start0, 0)

        def repack(raw, packed, rows):
            def go(i, _):
                r = pl.multiple_of(i * rows, rows)
                r2 = pl.multiple_of(i * (rows // 2), rows // 2)
                packed[pl.ds(r2, rows // 2), :] = _pack(raw[pl.ds(r, rows), :])
                return 0
            lax.fori_loop(0, raw.shape[0] // rows, go, 0)

        def transpose_blocks(raw, name):
            keys = [key for key in wt_slot if key[0] == name]
            if keys:
                def go(i, _):
                    r = pl.multiple_of(i * 128, 128)
                    for key in keys:
                        blk = raw[pl.ds(r, 128), key[1] * 128:(key[1] + 1) * 128]
                        w_t[wt_slot[key], :, pl.ds(r, 128)] = blk.astype(_F32).T
                    return 0
                lax.fori_loop(0, DT, go, 0)

        def row_means(raw, dst):
            ones = jnp.ones((16, D), _BF16)

            def go(i, _):
                r = pl.multiple_of(i * 512, 512)
                dst[:, pl.ds(r, 512)] = _dot_t(ones, raw[pl.ds(r, 512), :])[0:8] * (1.0 / D)
                return 0
            lax.fori_loop(0, raw.shape[0] // 512, go, 0)

        def with_mean(rows):
            w = rows.astype(_F32)
            m = jnp.mean(w, axis=-1, keepdims=True)
            return jnp.concatenate([w, jnp.broadcast_to(m, (w.shape[0], 128))], axis=1)

        low_half = lax.broadcasted_iota(jnp.int32, (8, 128), 1) < 64

        def tile_d(m):
            return jnp.concatenate([m] * DT, axis=1)

        def lane_mean_part(x):
            return jnp.broadcast_to(jnp.sum(_lane_fold(x), axis=-1, keepdims=True), (8, 128))

        def scores(q, kk):
            mid = q[:, 128:256]
            mid = jnp.concatenate([jnp.where(low_half, mid, 0.0), jnp.where(low_half, 0.0, mid)],
                                  axis=0).astype(_BF16)
            s0 = _dot(_lhs(q[:, 0:128]), kk[0:128])
            s1 = _dot(mid, kk[128:256])
            s2 = _dot(_lhs(q[:, 256:384]), kk[256:384])
            return s1 + jnp.concatenate([s0[0:8], s2[8:16]], axis=0)

        def probs(s):
            return jnp.exp2(s - jnp.max(s, axis=-1, keepdims=True))

        def inv_sum(p):
            l = jnp.sum(p, axis=-1, keepdims=True)
            r = pl.reciprocal(l, approx=True)
            return r * (2.0 - l * r)

        def pair_scale(linv):
            l0 = jnp.broadcast_to(linv[0:8], (8, 128))
            l1 = jnp.broadcast_to(linv[8:16], (8, 128))
            return jnp.concatenate([l0, jnp.where(low_half, l0, l1), l1], axis=1)

        def pv_chunk(pp, vv):
            return _lane_fold(vv * jnp.concatenate([pp, pp], axis=0))

        def vpu_out(part, w):
            cc = jnp.sum(part, axis=1, keepdims=True) * w
            return cc[0:8] + cc[8:16]

        def vpu_cols(xc, key):
            parts = [_lane_fold(w_t[wt_slot[key], t * 8:(t + 1) * 8, :] * xc) for t in range(16)]
            return jnp.broadcast_to(_row_sums(parts), (8, 128))

        def ffn(x, m, wr, nv, nr, early=None):
            xc = x - tile_d(m)
            rstd = _rstd(xc)
            half = 0.5 * rstd
            gate = jax.nn.sigmoid(jnp.sum(xc * wr, axis=-1, keepdims=True) * rstd)

            def hidden(g, u):
                a = g * half
                return (a + a * jnp.tanh(a)) * u

            xb = _lhs(xc if early is None else early[0])
            nm = FT - nv - nr
            hs = []
            for n0 in range(0, nm, cfg["fgrp"]):
                n1 = min(nm, n0 + cfg["fgrp"])
                g = _dot(xb, _unpack(wg_p[:, n0 * 128:n1 * 128]))[0:8]
                u = _dot(xb, _unpack(wu_p[:, n0 * 128:n1 * 128]))[0:8]
                if early is not None:
                    g = g + early[1][:, n0 * 128:n1 * 128]
                    u = u + early[1][:, FM1 + n0 * 128:FM1 + n1 * 128]
                hs.append((n0, n1, _lhs(hidden(g, u))))
            for n in range(nm, nm + nv):
                hs.append((n, n + 1, _lhs(hidden(vpu_cols(xc, ("g", n)), vpu_cols(xc, ("u", n))))))
            yv = None
            for n in range(FT - nr, FT):
                for t in range(16):
                    g, u = [jnp.sum(w_t[wt_slot[w, n], t * 8:(t + 1) * 8, :] * xc,
                                    axis=-1, keepdims=True) for w in "gu"]
                    r = (n - FT + NR) * 128 + t * 8
                    cc = hidden(g, u) * wd_f[r:r + 8, :]
                    yv = cc if yv is None else yv + cc
            y = None
            for n0, n1, h in hs:
                d = _dot(h, _unpack(wd_p[n0 * 64:n1 * 64, :]))[0:8]
                y = d if y is None else y + d
            hall = jnp.concatenate([h[0:8].astype(_F32) for _, _, h in hs], axis=1)
            my = lane_mean_part(hall * rmd_v[:, 0:(FT - nr) * 128])
            if yv is not None:
                yv = jnp.sum(yv, axis=0, keepdims=True)
                y = y + yv[:, 0:D]
                my = my + yv[:, D:]
            gate = gate * rstd
            return x + xc * rstd + y * gate, m + my * gate

        for cp in w_copies[0]:
            cp.wait()
        repack(wq_r, wq_p, 16)

        def wqf_go(t, _):
            for (c, i), n in wqf_slot.items():
                r = pl.multiple_of(i * 128 + t * 16, 16)
                wq_f[n, pl.ds(pl.multiple_of(t * 16, 16), 16), :] = (
                    wq_r[pl.ds(r, 16), c * DP:(c + 1) * DP].astype(_F32))
            return 0
        lax.fori_loop(0, 8, wqf_go, 0)

        xs_v[...] = jnp.zeros(xs_v.shape, _F32)
        xs_v[0:B, :] = x_v[...].astype(_F32)
        wr = wr_v[...].astype(_F32).reshape(1, D)
        xc0 = xs_v[...] - jnp.mean(xs_v[...], axis=-1, keepdims=True)
        qs0 = _rstd(xc0) * qscale
        xb0 = _lhs(xc0)

        def q1_go(g, _):
            col = pl.ds(pl.multiple_of(g * GP * DP, 128), GP * DP)
            q1_v[:, col] = _dot(xb0, _unpack(wq_p[:, col]))[0:8] * qs0
            return 0
        lax.fori_loop(0, NG, q1_go, 0)

        for cp in w_copies[1]:
            cp.wait()

        repack(wo_r, wo_p, 128)

        def wof_go(t, _):
            for (c, i), n in wof_slot.items():
                r = pl.multiple_of(c * DP + i * 128 + t * 16, 16)
                wo_f[n, pl.ds(pl.multiple_of(t * 16, 16), 16), :] = with_mean(wo_r[pl.ds(r, 16), :])
            return 0
        lax.fori_loop(0, 8, wof_go, 0)

        def wlf_go(i, _):
            for j in range(NJ):
                r = pl.multiple_of((((NG - 1) * GI + i) * NJ + j) * 16, 16)
                wl_f[j, i] = with_mean(wo_r[pl.ds(r, 16), :])
            return 0
        lax.fori_loop(0, GI, wlf_go, 0)
        row_means(wo_r, rmo_v)

        for cp in w_copies[2]:
            cp.wait()
        repack(wg_r, wg_p, 64)
        repack(wu_r, wu_p, 64)
        repack(wd_r, wd_p, 128)
        transpose_blocks(wg_r, "g")
        transpose_blocks(wu_r, "u")
        row_means(wd_r, rmd_v)

        def wdf_go(i, _):
            r = pl.multiple_of(i * 128, 128)
            wd_f[pl.ds(r, 128), :] = with_mean(wd_r[pl.ds(F - NR * 128 + r, 128), :])
            return 0
        lax.fori_loop(0, NR, wdf_go, 0)

        rows = [wo_r[pl.ds((((NG - 1) * GI + i) * NJ + NJ - 1) * 16, 16), :] for i in range(IA, GI)]
        rows = jnp.concatenate(rows + [jnp.ones((16, D), _BF16)], axis=0)

        def wl2_go(n, _):
            col = pl.multiple_of(n * 128, 128)
            for e, w_p in enumerate((wg_p, wu_p)):
                prod = _dot(rows, _unpack(w_p[:, pl.ds(col, 128)]))
                for i in range(GI - IA):
                    wl2_f[i, :, pl.ds(pl.multiple_of(e * FM1 + col, 128), 128)] = (
                        prod[i * 16:(i + 1) * 16]
                        - wl_f[NJ - 1, IA + i, :, D:] * prod[(GI - IA) * 16:])
            return 0
        lax.fori_loop(0, FM1 // 128, wl2_go, 0)

        def attention3(x, m):
            xc = x - tile_d(m)
            qs8 = _rstd(xc) * qscale
            xb = _lhs(xc)
            xcol = {i: jnp.broadcast_to(xc[0:1, i * 128:(i + 1) * 128], (128, 128)).T
                    for i in range(DT - max(ka.values()), DT)}

            def stage_a(c):
                km = (DT - ka[c]) * 128
                q = _dot(xb[:, 0:km], _unpack(wq_p[0:km // 2, c * DP:(c + 1) * DP]))[0:8]
                if ka[c]:
                    a = None
                    for i in range(DT - ka[c], DT):
                        for t in range(16):
                            xx = xcol[i][t * 8:(t + 1) * 8, :]
                            cc = (jnp.concatenate([xx] * (DP // 128), axis=1)
                                  * wq_f[wqf_slot[c, i], t * 8:(t + 1) * 8, :])
                            a = cc if a is None else a + cc
                    q = q + jnp.sum(a, axis=0, keepdims=True)
                return q * qs8

            def v_rows(c, t):
                i = (c % GP) * PI + t // NJ
                if c // GP == NG - 1 and t % NJ == NJ - 1 and i >= IA:
                    return v_chunk((NG - 1) % NS, i, NJ - 1)
                return vf[c, t]

            def stage_c(p, linv, c, wide):
                nt = (3 - bd[c]) * 8
                head = lambda t: t // (PT // 2)
                chunk = lambda t: pv_chunk(p[head(t) * 8:head(t) * 8 + 8], v_rows(c, t))
                o = None
                if nt:
                    o = _lhs(_row_sums8([chunk(t) for t in range(nt)])
                             * pair_scale(linv)[:, 0:nt * 16])
                tot = None
                for hh in range(2):
                    a = None
                    for t in range(nt, PT):
                        if head(t) != hh:
                            continue
                        r = (t % 8) * 16
                        cc = vpu_out(chunk(t), wo_f[wof_slot[c, t // 8], r:r + 16, 0:wide])
                        a = cc if a is None else a + cc
                    if a is not None:
                        a = a * linv[hh * 8:hh * 8 + 8]
                        tot = a if tot is None else tot + a
                return o, tot

            def stage_d(o, c):
                r = c * DP // 2
                return _dot(o, _unpack(wo_p[r:r + o.shape[1] // 2, :]))[0:8]

            def add(a, b):
                return b if a is None else a + b

            acc = accl = accm = accw = None
            qs, ss, ps, ls, os_ = {}, {}, {}, {}, {}
            off = dict(A=cfg["SA"], B=cfg["SB"], M=cfg["SM"], S=cfg["SS"], C=0)
            for step in range(-cfg["SA"], max(dpos) + 1):
                for st in cfg["order"]:
                    if st == "D":
                        for n in range(NC):
                            if dpos[n] == step and os_[n] is not None:
                                o, c = os_[n], perm[n]
                                accl = add(accl, stage_d(o, c))
                                rm = rmo_v[:, c * DP:c * DP + o.shape[1]]
                                accm = add(accm, _lane_fold(o[0:8].astype(_F32) * rm))
                        continue
                    n = step + off[st]
                    if not 0 <= n < NC:
                        continue
                    c = perm[n]
                    if st == "A":
                        qs[n] = stage_a(c)
                    elif st == "B":
                        ss[n] = scores(qs[n], _unpack(kp[c]))
                    elif st == "M":
                        ps[n] = probs(ss[n])
                    elif st == "S":
                        ls[n] = inv_sum(ps[n])
                    elif st == "C":
                        late = n >= NC - cfg["LM"]
                        os_[n], part = stage_c(ps[n], ls[n], c, D + 128 if late else D)
                        if part is not None and late:
                            accw = add(accw, part)
                        elif part is not None:
                            acc = add(acc, part)
            if acc is not None:
                accm = accm + _lane_fold(acc) * (1.0 / D)
                accl = accl + acc
            tot = jnp.concatenate([accl, lane_mean_part(accm)], axis=1)
            if accw is not None:
                tot = tot + accw
            tot = jnp.sum(tot, axis=0, keepdims=True)
            return x + tot[:, 0:D], m + tot[:, D:]

        def batch(b, _):
            @pl.when(b > 0)
            def _():
                for cp in v_copies(b, (NG - 1 + NS) % NG):
                    cp.start()

            def group_probs(g, s, static):
                for cp in k_copies(b, g):
                    cp.wait()
                for i in range(GP):
                    c = g * GP + i
                    col = c * DP if static else pl.multiple_of(c * DP, 128)
                    q = jnp.broadcast_to(q1_v[pl.ds(b, 1), pl.ds(col, DP)], (8, DP))
                    kk = kraw[s, i * PI:(i + 1) * PI].reshape(DP, W)
                    kp[c] = _pack(kk)
                    p = probs(scores(q, kk))
                    p_v[i] = p * inv_sum(p)
                start_next(k_copies, b, g)

            def head_probs(i):
                h = i // HI
                return p_v[h // 2, (h % 2) * 8:(h % 2) * 8 + 8, :]

            def group(g, acc):
                s = g % NS
                group_probs(g, s, False)
                for cp in v_copies(b, g):
                    cp.wait()
                for e in range(GP):
                    c = g * GP + e
                    parts = []
                    for t in range(PT):
                        i = e * PI + t // NJ
                        vv = v_chunk(s, i, t % NJ)
                        vf[c, t] = vv
                        parts.append(pv_chunk(head_probs(i), vv))
                    o = _lhs(jnp.broadcast_to(_row_sums(parts), (8, DP)))
                    r = pl.multiple_of(c * (DP // 2), 8)
                    acc = acc + _dot(o, _unpack(wo_p[pl.ds(r, DP // 2), :]))[0:8]

                @pl.when(g == NG - 1 - NS)
                def _():
                    for cps in v_last_copies(b):
                        for cp in cps:
                            cp.start()

                @pl.when(g != NG - 1 - NS)
                def _():
                    start_next(v_copies, b, g)
                return acc

            x = lax.fori_loop(0, NG - 1, group, jnp.broadcast_to(xs_v[pl.ds(b, 1), :], (8, D)))
            g = NG - 1
            s = g % NS
            m = lane_mean_part(x) * (1.0 / D)
            group_probs(g, s, True)
            tot = None
            for cps, (j, i0, i1) in zip(v_last_copies(b), last_parts):
                final = j == NJ - 1 and i0 == IA
                if final:
                    tot = jnp.sum(tot, axis=0, keepdims=True)
                    x = x + tot[:, 0:D]
                    m = m + tot[:, D:]
                    xc_early = x - tile_d(m)
                    tot = None
                for cp in cps:
                    cp.wait()
                for i in range(i0, i1):
                    vv = v_chunk(s, i, j)
                    w = wl_f[j, i]
                    if final:
                        w = jnp.concatenate([w, wl2_f[i - IA]], axis=1)
                    else:
                        vf[g * GP + i // PI, (i % PI) * NJ + j] = vv
                    cc = vpu_out(pv_chunk(head_probs(i), vv), w)
                    tot = cc if tot is None else tot + cc
            tot = jnp.sum(tot, axis=0, keepdims=True)
            x = x + tot[:, 0:D]
            m = m + tot[:, D:D + 128]

            x, m = ffn(x, m, wr, nv1, nr1, (xc_early, tot[:, D + 128:]))
            x, m = attention3(x, m)
            x, _ = ffn(x, m, wr, nv, nr)
            xs = jnp.where(lax.broadcasted_iota(jnp.int32, (8, D), 0) == b, x, xs_v[...])
            xs_v[...] = xs
            o_ref[...] = xs[0:B].astype(o_ref.dtype)
            return 0

        lax.fori_loop(0, B, batch, 0)

    any_spec = pl.BlockSpec(memory_space=pl.ANY)
    out = pl.pallas_call(
        kernel,
        in_specs=[any_spec] * 9,
        out_specs=any_spec,
        out_shape=jax.ShapeDtypeStruct((B, D), A_x.dtype),
        scratch_shapes=[
            pltpu.VMEM((NS, GI, RT, 8, W), _BF16),
            pltpu.VMEM((NS, GI, RT, 8, W), _BF16),
            pltpu.VMEM((NC, DP // 2, W), _U32),
            pltpu.VMEM((NC, PT, 16, W), _F32),
            pltpu.VMEM((D, H * Dh), _BF16),
            pltpu.VMEM((H * Dh, D), _BF16),
            pltpu.VMEM((D, F), _BF16),
            pltpu.VMEM((D, F), _BF16),
            pltpu.VMEM((F, D), _BF16),
            pltpu.VMEM((D // 2, H * Dh), _U32),
            pltpu.VMEM((H * Dh // 2, D), _U32),
            pltpu.VMEM((D // 2, F), _U32),
            pltpu.VMEM((D // 2, F), _U32),
            pltpu.VMEM((F // 2, D), _U32),
            pltpu.VMEM((max(len(wqf_slot), 1), 128, DP), _F32),
            pltpu.VMEM((max(len(wof_slot), 1), 128, D + 128), _F32),
            pltpu.VMEM((NJ, GI, 16, D + 128), _F32),
            pltpu.VMEM((GI - IA, 16, 2 * FM1), _F32),
            pltpu.VMEM((max(NR, 1) * 128, D + 128), _F32),
            pltpu.VMEM((max(len(wt_slot), 1), 128, D), _F32),
            pltpu.VMEM((B, D), _BF16),
            pltpu.VMEM((D,), _BF16),
            pltpu.VMEM((8, D), _F32),
            pltpu.VMEM((8, H * Dh), _F32),
            pltpu.VMEM((GP, 16, W), _F32),
            pltpu.VMEM((8, H * Dh), _F32),
            pltpu.VMEM((8, F), _F32),
            pltpu.VMEM((B, D), A_x.dtype),
            pltpu.SemaphoreType.DMA(()),
        ],
        compiler_params=pltpu.CompilerParams(vmem_limit_bytes=120 * 1024 * 1024),
    )(
        A_x.reshape(B, D),
        jnp.swapaxes(A_k_cache, 2, 3).reshape(B, NG, GI, RT, 8, Sk),
        jnp.swapaxes(A_v_cache, 2, 3).reshape(B, NG, GI, RT, 8, Sk),
        A_wq, A_wo, B_w_r, B_w_gate, B_w_up, B_w_down,
    )
    return out.reshape(B, Sq, D)


@jax.jit
def pallas_interleave_layers__sliding_block_cached__moe_arch_mod__decode_kernel(
    A_x: jax.Array,
    A_k_cache: jax.Array,
    A_v_cache: jax.Array,
    A_wq: jax.Array,
    A_wo: jax.Array,
    B_x: jax.Array,
    B_w_r: jax.Array,
    B_w_gate: jax.Array,
    B_w_up: jax.Array,
    B_w_down: jax.Array,
):
    return _forward(_CFG, A_x, A_k_cache, A_v_cache, A_wq, A_wo,
                    B_w_r, B_w_gate, B_w_up, B_w_down)
```
